```python
import jax
import jax.numpy as jnp

def _softmax(x, axis=-1):
    return jax.nn.softmax(x, axis=axis)
def _gelu(x):
    return jax.nn.gelu(x, approximate=True)
def _silu(x):
    return jax.nn.silu(x)
def _sigmoid(x):
    return jax.nn.sigmoid(x)
def _layernorm(x, axis=-1, eps=1e-5):
    m = jnp.mean(x, axis=axis, keepdims=True)
    v = jnp.var(x, axis=axis, keepdims=True)
    return (x - m) / jnp.sqrt(v + eps)
def _scatter_add(tgt, idx, src, axis=0):
    return tgt.at[idx].add(src)
def _segment_sum(src, seg, n):
    return jax.ops.segment_sum(src, seg, n)
class _Rng:
    def __init__(self, key):
        self._k = key
    def _next(self):
        self._k, sub = jax.random.split(self._k)
        return sub
    def normal(self, shape):
        return jax.random.normal(self._next(), shape, dtype=jnp.bfloat16)
    def randint(self, lo, hi, shape):
        return jax.random.randint(self._next(), shape, lo, hi, dtype=jnp.int32)
    def uniform(self, shape, lo=0.0, hi=1.0):
        return jax.random.uniform(self._next(), shape, jnp.bfloat16, lo, hi)
    def permutation(self, n):
        return jax.random.permutation(self._next(), n)


kernel_name = 'interleave_layers__sliding_block_cached__moe_arch_mod__decode'

def setup_inputs():
    _rng = _Rng(jax.random.key(int.from_bytes(__import__("os").urandom(4), "little")))
    _w = (lambda a: (lambda t: t.astype(jnp.bfloat16) if jnp.issubdtype(t.dtype, jnp.floating) else t)(jnp.asarray(a)))
    def _A_setup():
        B, Sq, D = 4, 1, 640
        Hq, Hkv, Sk, Dh = 32, 32, 4096, 192
        assert Hq % Hkv == 0, (Hq, Hkv)
        return {
            "x": _w((lambda *s: _rng.normal(s) * 0.05)(B, Sq, D)),
            "k_cache": _w((lambda *s: _rng.normal(s) * 0.05)(B, Hkv, Sk, Dh)),
            "v_cache": _w((lambda *s: _rng.normal(s) * 0.05)(B, Hkv, Sk, Dh)),
            "wq": _w((lambda *s: _rng.normal(s) * 0.05)(D, Hq * Dh) * (D ** -0.5)),
            "wo": _w((lambda *s: _rng.normal(s) * 0.05)(Hq * Dh, D) * ((Hq * Dh) ** -0.5)),
        }
    _A_in = _A_setup()

    def _B_setup():
        B, S, D, F, C = 4, 1, 640, 1536, 1
        return {
            "x": _w((lambda *s: _rng.normal(s) * 0.05)(B, S, D)),
            "w_r": _w((lambda *s: _rng.normal(s) * 0.05)(D)),
            "w_gate": _w((lambda *s: _rng.normal(s) * 0.05)(D, F)),
            "w_up": _w((lambda *s: _rng.normal(s) * 0.05)(D, F)),
            "w_down": _w((lambda *s: _rng.normal(s) * 0.05)(F, D)),
        }
    _B_in = _B_setup()

    return {
        "A_x": _A_in["x"],
        "A_k_cache": _A_in["k_cache"],
        "A_v_cache": _A_in["v_cache"],
        "A_wq": _A_in["wq"],
        "A_wo": _A_in["wo"],
        "B_x": _B_in["x"],
        "B_w_r": _B_in["w_r"],
        "B_w_gate": _B_in["w_gate"],
        "B_w_up": _B_in["w_up"],
        "B_w_down": _B_in["w_down"],
    }

def reference(A_x, A_k_cache, A_v_cache, A_wq, A_wo, B_x, B_w_r, B_w_gate, B_w_up, B_w_down):
    def _A_ref(x, k_cache, v_cache, wq, wo):
        B, Sq, D = x.shape
        Hq, Dh = 32, 192
        Hkv, Sk = k_cache.shape[1], k_cache.shape[2]
        W = min(4096, max(256, Sk // 4))
        rep = Hq // Hkv
        q = (lambda x, *d: x.transpose(*d))((x @ wq).reshape(B, Sq, Hq, Dh), 0, 2, 1, 3)
        k = jnp.repeat(k_cache[:, :, Sk - W:, :], rep, axis=1)
        v = jnp.repeat(v_cache[:, :, Sk - W:, :], rep, axis=1)
        scores = jnp.einsum("bhqd,bhkd->bhqk", q, k) * (Dh ** -0.5)
        p = _softmax(scores, axis=-1)
        o = jnp.einsum("bhqk,bhkd->bhqd", p, v)
        return (lambda x, *d: x.transpose(*d))(o, 0, 2, 1, 3).reshape(B, Sq, Hq * Dh) @ wo

    def _B_ref(x, w_r, w_gate, w_up, w_down):
        B, S, D = x.shape
        C = 1
        r = x @ w_r
        idx = jnp.argsort(-r, axis=-1)[:, :C]
        idx_e = jnp.repeat(idx.reshape(B, C, 1), D, axis=2)
        x_sel = jnp.take_along_axis(x, idx_e, axis=1)
        g = _silu(x_sel @ w_gate)
        u = x_sel @ w_up
        y = (g * u) @ w_down
        r_sel = _sigmoid(jnp.take_along_axis(r, idx, axis=1))
        y = y * r_sel.reshape(B, C, 1)
        b_off = (jnp.arange(B) * S).reshape(B, 1)
        flat_idx = (idx + b_off).reshape(B * C)
        zero = (x * 0.0).reshape(B * S, D)
        upd = _scatter_add(zero, flat_idx, y.reshape(B * C, D), axis=0)
        return x + upd.reshape(B, S, D)

    x = A_x
    x = x + _A_ref(_layernorm(x, axis=-1), A_k_cache, A_v_cache, A_wq, A_wo)
    x = x + _B_ref(_layernorm(x, axis=-1), B_w_r, B_w_gate, B_w_up, B_w_down)
    x = x + _A_ref(_layernorm(x, axis=-1), A_k_cache, A_v_cache, A_wq, A_wo)
    x = x + _B_ref(_layernorm(x, axis=-1), B_w_r, B_w_gate, B_w_up, B_w_down)
    return x
```

```python
import functools

import jax
import jax.numpy as jnp
from jax import lax
import jax.experimental.pallas as pl
import jax.experimental.pallas.tpu as pltpu

f32, bf16, u32 = jnp.float32, jnp.bfloat16, jnp.uint32

B, D, H, DH, SK, FF = 4, 640, 32, 192, 4096, 1536
W = min(4096, max(256, SK // 4))
RT = DH // 8
CT = W // 128
NT = H * DH // 128
HC = 4
NCH = H // HC
SCALE = DH ** -0.5
EPS = 1e-5


def _plan(lat_a=250, lat_b=150, lat_s=250, lat_c2=150, cv=7.0, c2_margin=10,
          v_ahead=600, a_ahead=3, prio=("C2", "B", "A", "D")):
    ev = []
    t = 0.0
    v_t = 0.0
    a_done, c2_done, c1_time = {}, {}, {}
    n_a = n_b = n_c2 = n_d = 0
    while n_d < NT:
        cands = []
        if n_c2 < NT:
            last = n_c2 * 16 + 15
            if last in c1_time and c1_time[last] + c2_margin <= t:
                cands.append("C2")
        if n_b < H * 4:
            need = ((n_b // 4) * DH + DH - 1) // 128
            if (need in a_done and a_done[need] + lat_a <= t
                    and (v_t - t <= v_ahead or n_b % 4 != 0)):
                cands.append("B")
        if n_a < NT and n_a * 128 <= (n_b // 4 + a_ahead) * DH:
            cands.append("A")
        if n_d < n_c2 and c2_done[n_d] + lat_c2 <= t:
            cands.append("D")
        pick = next((k for k in prio if k in cands), None)
        if pick is None:
            t += 4
        elif pick == "C2":
            ev.append((t, "C2", n_c2))
            t += 16
            c2_done[n_c2] = t + 48
            n_c2 += 1
        elif pick == "B":
            h = n_b // 4
            ev.append((t, "B", (h, n_b % 4)))
            t += 24
            if n_b % 4 == 3:
                ev.append((t + lat_b, "S", h))
                v_t = max(v_t, t + lat_b + lat_s)
                for rt in range(RT):
                    ev.append((v_t, "C1", (h, rt)))
                    v_t += cv
                    c1_time[h * RT + rt] = v_t
            n_b += 1
        elif pick == "A":
            ev.append((t, "A", n_a))
            t += 40
            a_done[n_a] = t
            n_a += 1
        else:
            ev.append((t, "D", n_d))
            t += 40
            n_d += 1
    ev.sort(key=lambda e: e[0])
    return [(k, i) for _, k, i in ev]


def _layernorm(x):
    m = jnp.sum(x, axis=1, keepdims=True) * (1.0 / D)
    xc = x - m
    v = jnp.sum(xc * xc, axis=1, keepdims=True) * (1.0 / D)
    return xc * lax.rsqrt(v + EPS)


def _kernel(x_hbm, wr_hbm, k_hbm, v_hbm, wq_hbm, wo_hbm, wg_hbm, wu_hbm, wd_hbm,
            out_ref,
            x_v, wr_v, wq_v, wo_v, wg_v, wu_v, wd_v, k_v, v_v, xf_v,
            w_sem, kv_sem):
    w_src = (x_hbm, wr_hbm, wq_hbm, wo_hbm, wg_hbm, wu_hbm, wd_hbm)
    w_dst = (x_v, wr_v) + tuple(r.bitcast(bf16) for r in (wq_v, wo_v, wg_v, wu_v, wd_v))
    w_cp = [pltpu.make_async_copy(s, d, w_sem.at[i])
            for i, (s, d) in enumerate(zip(w_src, w_dst))]

    def kv_copy(which, b, c):
        src, dst = ((k_hbm, k_v), (v_hbm, v_v))[which]
        return pltpu.make_async_copy(
            src.at[b, pl.ds(c * HC, HC), :, pl.ds((SK - W) // 16, W // 16), :],
            dst.at[b, pl.ds(c * HC, HC)],
            kv_sem.at[which, b, c])

    def start_kv(b):
        for c in range(NCH):
            kv_copy(0, b, c).start()
            kv_copy(1, b, c).start()

    for cp in w_cp:
        cp.start()
    for b in range(B - 1):
        start_kv(b)

    lane = lax.broadcasted_iota(jnp.int32, (8, 128), 1)
    row = lax.broadcasted_iota(jnp.int32, (8, 128), 0)
    gidx = (lane // 16) * 8 + (lane % 8)
    emask = (row % 2) == ((lane // 8) % 2)
    ones = jnp.ones((8, 128), bf16)
    k32 = k_v.bitcast(u32)

    def wtile(ref, rows, cols):
        return pltpu.bitcast(ref[rows, cols], bf16)

    def q_tile(xn, cols):
        q = jnp.dot(xn, wtile(wq_v, slice(None), cols), preferred_element_type=f32)
        return [jnp.where(emask, jnp.take_along_axis(q, gidx + 64 * hf, axis=1), 0.0).astype(bf16)
                for hf in range(2)]

    def score_quarter(lhs, b, h, u, s):
        wu = pltpu.bitcast(k32[b, h, :, u * 8:(u + 1) * 8, :].reshape(RT * 8, 128), bf16)
        r = jnp.dot(lhs, wu, preferred_element_type=f32)
        return r if s is None else jnp.where(row // 2 == u, r, s)

    def softmax(s):
        m = jnp.max(jnp.max(s, axis=1, keepdims=True), axis=0, keepdims=True)
        e = jnp.exp((s - m) * SCALE)
        l = jnp.sum(jnp.sum(e, axis=1, keepdims=True), axis=0, keepdims=True)
        return e * (1.0 / l)

    def p_rows(p):
        return [jnp.broadcast_to(p[c:c + 1, :], (8, 128)) for c in range(CT)]

    def pv_tile(pb, b, h, rt):
        v = v_v[b, h, rt].astype(f32)
        a = v[0:8] * pb[0]
        for c in range(1, CT):
            a = a + v[c * 8:(c + 1) * 8] * pb[c]
        return a

    def lane_reduce(accs):
        a = jnp.concatenate(accs, axis=0).astype(bf16)
        o = lax.dot_general(ones, a, (((1,), (1,)), ((), ())), preferred_element_type=f32)
        return o.astype(bf16)

    def attn_streaming(xn, b):
        tpc = HC * DH // 128

        def body(c, y):
            qe = []
            for i in range(tpc):
                qe += q_tile(xn, pl.ds(pl.multiple_of((c * tpc + i) * 128, 128), 128))
            kv_copy(0, b, c).wait()
            ps = []
            for i in range(HC):
                lhs = jnp.concatenate(qe[3 * i:3 * i + 3], axis=1)
                s = None
                for u in range(4):
                    s = score_quarter(lhs, b, c * HC + i, u, s)
                ps.append(softmax(s))
            kv_copy(1, b, c).wait()
            accs = []
            for i in range(HC):
                pb = p_rows(ps[i])
                accs += [pv_tile(pb, b, c * HC + i, rt) for rt in range(RT)]
            for i in range(tpc):
                o = lane_reduce(accs[16 * i:16 * i + 16])
                rows = pl.ds(pl.multiple_of((c * tpc + i) * 64, 64), 64)
                y = y + jnp.dot(o, wtile(wo_v, rows, slice(None)), preferred_element_type=f32)
            return y

        return lax.fori_loop(0, NCH, body, jnp.zeros((8, D), f32))

    def attn_resident(xn, b):
        qe, s, acc, o = {}, {}, {}, {}
        pb = y = None
        for kind, idx in _plan():
            if kind == "A":
                qe[2 * idx], qe[2 * idx + 1] = q_tile(xn, slice(idx * 128, (idx + 1) * 128))
            elif kind == "B":
                h, u = idx
                lhs = jnp.concatenate([qe[3 * h + g] for g in range(3)], axis=1)
                s[h] = score_quarter(lhs, b, h, u, s.get(h))
            elif kind == "S":
                s[idx] = softmax(s[idx])
            elif kind == "C1":
                h, rt = idx
                if rt == 0:
                    pb = p_rows(s.pop(h))
                acc[h * RT + rt] = pv_tile(pb, b, h, rt)
            elif kind == "C2":
                o[idx] = lane_reduce([acc.pop(idx * 16 + i) for i in range(16)])
            else:
                d = jnp.dot(o.pop(idx), wtile(wo_v, slice(idx * 64, (idx + 1) * 64), slice(None)),
                            preferred_element_type=f32)
                y = d if y is None else y + d
        return y

    def mod_block(x, wr):
        xn = _layernorm(x)
        xb = xn.astype(bf16)
        r = jnp.sum(xn * wr, axis=1, keepdims=True)
        g = jnp.dot(xb, wtile(wg_v, slice(None), slice(None)), preferred_element_type=f32)
        u = jnp.dot(xb, wtile(wu_v, slice(None), slice(None)), preferred_element_type=f32)
        hid = (g * jax.nn.sigmoid(g) * u).astype(bf16)
        y = jnp.dot(hid, wtile(wd_v, slice(None), slice(None)), preferred_element_type=f32)
        return x + (xn + y * jax.nn.sigmoid(r))

    w_cp[0].wait()
    w_cp[1].wait()
    xf_v[0:B, :] = x_v[...].astype(f32)
    wr = wr_v[...].astype(f32).reshape(1, D)
    for cp in w_cp[2:]:
        cp.wait()

    def batch_body(b, carry):
        x = jnp.broadcast_to(xf_v[pl.ds(b, 1), :], (8, D))
        x = x + attn_streaming(_layernorm(x).astype(bf16), b)

        @pl.when(b == 0)
        def _():
            start_kv(B - 1)

        x = mod_block(x, wr)
        x = x + attn_resident(_layernorm(x).astype(bf16), b)
        x = mod_block(x, wr)
        xf_v[pl.ds(b, 1), :] = x[0:1, :]
        return carry

    lax.fori_loop(0, B, batch_body, 0)
    out_ref[...] = xf_v[0:B, :].astype(bf16)


def _tile_view(c):
    c = c.reshape(B, H, SK // 128, 128, RT, 8).transpose(0, 1, 4, 2, 5, 3)
    return c.reshape(B, H, RT, SK // 16, 128)


@jax.jit
def pallas_interleave_layers__sliding_block_cached__moe_arch_mod__decode_kernel(
    A_x: jax.Array,
    A_k_cache: jax.Array,
    A_v_cache: jax.Array,
    A_wq: jax.Array,
    A_wo: jax.Array,
    B_x: jax.Array,
    B_w_r: jax.Array,
    B_w_gate: jax.Array,
    B_w_up: jax.Array,
    B_w_down: jax.Array,
):
    del B_x
    out = pl.pallas_call(
        _kernel,
        out_shape=jax.ShapeDtypeStruct((B, D), bf16),
        in_specs=[pl.BlockSpec(memory_space=pl.ANY)] * 9,
        out_specs=pl.BlockSpec(memory_space=pltpu.VMEM),
        scratch_shapes=[
            pltpu.VMEM((B, D), bf16),
            pltpu.VMEM((D,), bf16),
            pltpu.VMEM((D // 2, H * DH), u32),
            pltpu.VMEM((H * DH // 2, D), u32),
            pltpu.VMEM((D // 2, FF), u32),
            pltpu.VMEM((D // 2, FF), u32),
            pltpu.VMEM((FF // 2, D), u32),
            pltpu.VMEM((B, H, RT, W // 16, 128), bf16),
            pltpu.VMEM((B, H, RT, W // 16, 128), bf16),
            pltpu.VMEM((8, D), f32),
            pltpu.SemaphoreType.DMA((7,)),
            pltpu.SemaphoreType.DMA((2, B, NCH)),
        ],
        compiler_params=pltpu.CompilerParams(vmem_limit_bytes=124 * 1024 * 1024),
        name="fused_decode",
    )(A_x.reshape(B, D), B_w_r, _tile_view(A_k_cache), _tile_view(A_v_cache),
      A_wq, A_wo, B_w_gate, B_w_up, B_w_down)
    return out.reshape(B, 1, D)
```

```python
import contextlib

import jax
import jax.numpy as jnp
from jax import lax
import jax.experimental.pallas as pl
import jax.experimental.pallas.tpu as pltpu

f32, bf16, u32 = jnp.float32, jnp.bfloat16, jnp.uint32

B, D, H, DH, SK, FF = 4, 640, 32, 192, 4096, 1536
W = min(4096, max(256, SK // 4))
RT = DH // 8
CT = W // 128
NT = H * DH // 128
NP = H * RT // 2
V_CHUNKS = ((0, 24, True), (24, 12, True), (36, 6, True), (42, 3, True), (45, 2, False), (47, 1, False))
NW = 7
SEMS_PER_ROW = 2 * (1 + len(V_CHUNKS))
SCALE = DH ** -0.5
EPS = 1e-5
try:
    _OVR
except NameError:
    _OVR = {}


def _scope(name):
    return jax.named_scope(name) if _OVR.get("SCOPES") else contextlib.nullcontext()


def _plan(lat_a=250, lat_b=150, lat_s=250, lat_c2=150, cv=7.0, c2_margin=10,
          v_ahead=600, a_ahead=3, prio=("C2", "B", "A", "D")):
    ev = []
    t = 0.0
    v_t = 0.0
    a_done, c2_done, c1_time = {}, {}, {}
    n_a = n_b = n_c2 = n_d = 0
    while n_d < NT:
        cands = []
        if n_c2 < NT:
            last = n_c2 * 16 + 15
            if last in c1_time and c1_time[last] + c2_margin <= t:
                cands.append("C2")
        if n_b < H * 4:
            need = ((n_b // 4) * DH + DH - 1) // 128
            if (need in a_done and a_done[need] + lat_a <= t
                    and (v_t - t <= v_ahead or n_b % 4 != 0)):
                cands.append("B")
        if n_a < NT and n_a * 128 <= (n_b // 4 + a_ahead) * DH:
            cands.append("A")
        if n_d < n_c2 and c2_done[n_d] + lat_c2 <= t:
            cands.append("D")
        pick = next((k for k in prio if k in cands), None)
        if pick is None:
            t += 4
        elif pick == "C2":
            ev.append((t, "C2", n_c2))
            t += 16
            c2_done[n_c2] = t + 48
            n_c2 += 1
        elif pick == "B":
            h = n_b // 4
            ev.append((t, "B", (h, n_b % 4)))
            t += 24
            if n_b % 4 == 3:
                ev.append((t + lat_b, "S", h))
                v_t = max(v_t, t + lat_b + lat_s)
                for rt in range(RT):
                    ev.append((v_t, "C1", (h, rt)))
                    v_t += cv
                    c1_time[h * RT + rt] = v_t
            n_b += 1
        elif pick == "A":
            ev.append((t, "A", n_a))
            t += 40
            a_done[n_a] = t
            n_a += 1
        else:
            ev.append((t, "D", n_d))
            t += 40
            n_d += 1
    ev.sort(key=lambda e: e[0])
    return [(k, i) for _, k, i in ev]


def _layernorm(x):
    m = jnp.sum(x, axis=1, keepdims=True) * (1.0 / D)
    xc = x - m
    v = jnp.sum(xc * xc, axis=1, keepdims=True) * (1.0 / D)
    return xc * lax.rsqrt(v + EPS)


def _kernel(x_hbm, wr_hbm, k_hbm, v_hbm, wq_hbm, wo_hbm, wg_hbm, wu_hbm, wd_hbm,
            out_ref,
            x_v, wr_v, wq_v, wo_v, wg_v, wu_v, wd_v, k_v, v_v, xf_v, p_v,
            sems):
    w_src = (x_hbm, wr_hbm, wq_hbm, wo_hbm, wg_hbm, wu_hbm, wd_hbm)
    w_dst = (x_v, wr_v) + tuple(r.bitcast(bf16) for r in (wq_v, wo_v, wg_v, wu_v, wd_v))
    w_cp = [pltpu.make_async_copy(s, d, sems.at[i])
            for i, (s, d) in enumerate(zip(w_src, w_dst))]

    win = pl.ds((SK - W) // 16, W // 16)

    def kv_copies(src, dst, slot, b, p0, n, split):
        rows = pl.ds(p0, n)
        s0 = NW + b * SEMS_PER_ROW + 2 * slot
        if split:
            return [pltpu.make_async_copy(src.at[b, rows, t, win, :], dst.at[b, rows, t],
                                          sems.at[s0 + t]) for t in range(2)]
        return [pltpu.make_async_copy(src.at[b, rows, :, win, :], dst.at[b, rows], sems.at[s0])]

    def k_copies(b):
        return kv_copies(k_hbm, k_v, 0, b, 0, NP, True)

    def v_copies(b, c):
        t0, nt, split = V_CHUNKS[c]
        return kv_copies(v_hbm, v_v, 1 + c, b, t0 * 8, nt * 8, split)

    for cp in w_cp:
        cp.start()
    for b in range(B):
        for cp in k_copies(b):
            cp.start()
        for c in range(len(V_CHUNKS)):
            for cp in v_copies(b, c):
                cp.start()

    lane = lax.broadcasted_iota(jnp.int32, (8, 128), 1)
    row = lax.broadcasted_iota(jnp.int32, (8, 128), 0)
    gidx = (lane // 16) * 8 + (lane % 8)
    emask = (row % 2) == ((lane // 8) % 2)
    ones = jnp.ones((8, 128), bf16)
    k32 = k_v.bitcast(u32)

    def wtile(ref, rows, cols):
        return pltpu.bitcast(ref[rows, cols], bf16)

    def q_tile(xn, cols):
        q = jnp.dot(xn, wtile(wq_v, slice(None), cols), preferred_element_type=f32)
        return [jnp.where(emask, jnp.take_along_axis(q, gidx + 64 * hf, axis=1), 0.0).astype(bf16)
                for hf in range(2)]

    def score_quarter(lhs, b, h, u, s):
        wu = k32[b, pl.ds(h * (RT // 2), RT // 2), :, u * 8:(u + 1) * 8, :]
        wu = pltpu.bitcast(wu.reshape(RT * 8, 128), bf16)
        r = jnp.dot(lhs, wu, preferred_element_type=f32)
        return r if s is None else jnp.where(row // 2 == u, r, s)

    def softmax(s):
        m = jnp.max(jnp.max(s, axis=1, keepdims=True), axis=0, keepdims=True)
        e = jnp.exp((s - m) * SCALE)
        l = jnp.sum(jnp.sum(e, axis=1, keepdims=True), axis=0, keepdims=True)
        return e * (1.0 / l)

    def p_rows(p):
        return [jnp.broadcast_to(p[c:c + 1, :], (8, 128)) for c in range(CT)]

    def pv_tile(pb, b, h, rt):
        v = v_v[b, h * (RT // 2) + rt // 2, rt % 2].astype(f32)
        a = v[0:8] * pb[0]
        for c in range(1, CT):
            a = a + v[c * 8:(c + 1) * 8] * pb[c]
        return a

    def lane_reduce(accs):
        a = jnp.concatenate(accs, axis=0).astype(bf16)
        o = lax.dot_general(ones, a, (((1,), (1,)), ((), ())), preferred_element_type=f32)
        return o.astype(bf16)

    def attn_streaming(xn, b):
        hg = 4
        tpg = hg * DH // 128
        with _scope("wait_k"):
            for cp in k_copies(b):
                cp.wait()

        def scores(c, carry):
            qe = []
            for i in range(tpg):
                qe += q_tile(xn, pl.ds(pl.multiple_of((c * tpg + i) * 128, 128), 128))
            for i in range(hg):
                lhs = jnp.concatenate(qe[3 * i:3 * i + 3], axis=1)
                s = None
                for u in range(4):
                    s = score_quarter(lhs, b, c * hg + i, u, s)
                p_v[c * hg + i] = softmax(s)
            return carry

        with _scope("scores"):
            lax.fori_loop(0, H // hg, scores, 0)

        def out_tile(accs, tile, y):
            rows = pl.ds(pl.multiple_of(tile * 64, 64), 64)
            return y + jnp.dot(lane_reduce(accs), wtile(wo_v, rows, slice(None)),
                               preferred_element_type=f32)

        def head_pair(j, y):
            for c, (t0, _, _) in enumerate(V_CHUNKS[:-2]):
                @pl.when(j == t0 // 3)
                def _():
                    for cp in v_copies(b, c):
                        cp.wait()
            accs = []
            for i in range(2):
                pb = p_rows(p_v[2 * j + i])
                accs += [pv_tile(pb, b, 2 * j + i, rt) for rt in range(RT)]
            for i in range(3):
                y = out_tile(accs[16 * i:16 * i + 16], 3 * j + i, y)
            return y

        with _scope("pv_loop"):
            y = lax.fori_loop(0, H // 2 - 1, head_pair, jnp.zeros((8, D), f32))
        for cp in v_copies(b, len(V_CHUNKS) - 2):
            cp.wait()
        pb = p_rows(p_v[H - 2])
        accs = [pv_tile(pb, b, H - 2, rt) for rt in range(RT)]
        pb = p_rows(p_v[H - 1])
        accs += [pv_tile(pb, b, H - 1, rt) for rt in range(8)]
        y = out_tile(accs[:16], NT - 3, y)
        y = out_tile(accs[16:], NT - 2, y)
        with _scope("wait_last"):
            for cp in v_copies(b, len(V_CHUNKS) - 1):
                cp.wait()
        return out_tile([pv_tile(pb, b, H - 1, rt) for rt in range(8, RT)], NT - 1, y)

    def attn_resident(xn, b):
        qe, s, acc, o = {}, {}, {}, {}
        pb = y = None
        for kind, idx in _plan():
            if kind == "A":
                qe[2 * idx], qe[2 * idx + 1] = q_tile(xn, slice(idx * 128, (idx + 1) * 128))
            elif kind == "B":
                h, u = idx
                lhs = jnp.concatenate([qe[3 * h + g] for g in range(3)], axis=1)
                s[h] = score_quarter(lhs, b, h, u, s.get(h))
            elif kind == "S":
                s[idx] = softmax(s[idx])
            elif kind == "C1":
                h, rt = idx
                if rt == 0:
                    pb = p_rows(s.pop(h))
                acc[h * RT + rt] = pv_tile(pb, b, h, rt)
            elif kind == "C2":
                o[idx] = lane_reduce([acc.pop(idx * 16 + i) for i in range(16)])
            else:
                d = jnp.dot(o.pop(idx), wtile(wo_v, slice(idx * 64, (idx + 1) * 64), slice(None)),
                            preferred_element_type=f32)
                y = d if y is None else y + d
        return y

    def mod_block(x, wr):
        xn = _layernorm(x)
        xb = xn.astype(bf16)
        r = jnp.sum(xn * wr, axis=1, keepdims=True)
        g = jnp.dot(xb, wtile(wg_v, slice(None), slice(None)), preferred_element_type=f32)
        u = jnp.dot(xb, wtile(wu_v, slice(None), slice(None)), preferred_element_type=f32)
        hid = (g * jax.nn.sigmoid(g) * u).astype(bf16)
        y = jnp.dot(hid, wtile(wd_v, slice(None), slice(None)), preferred_element_type=f32)
        return x + (xn + y * jax.nn.sigmoid(r))

    w_cp[0].wait()
    w_cp[1].wait()
    xf_v[0:B, :] = x_v[...].astype(f32)
    wr = wr_v[...].astype(f32).reshape(1, D)
    for cp in w_cp[2:]:
        cp.wait()

    def batch_body(b, carry):
        x = jnp.broadcast_to(xf_v[pl.ds(b, 1), :], (8, D))
        x = x + attn_streaming(_layernorm(x).astype(bf16), b)
        with _scope("mod1"):
            x = mod_block(x, wr)
        with _scope("attn2"):
            x = x + attn_resident(_layernorm(x).astype(bf16), b)
        with _scope("mod2"):
            x = mod_block(x, wr)
        xf_v[pl.ds(b, 1), :] = x[0:1, :]
        return carry

    lax.fori_loop(0, B, batch_body, 0)
    out_ref[...] = xf_v[0:B, :].astype(bf16)


def _tile_view(c):
    c = c.reshape(B, H, SK // 128, 128, RT, 8).transpose(0, 1, 4, 2, 5, 3)
    return c.reshape(B, NP, 2, SK // 16, 128)


@jax.jit
def pallas_interleave_layers__sliding_block_cached__moe_arch_mod__decode_kernel(
    A_x: jax.Array,
    A_k_cache: jax.Array,
    A_v_cache: jax.Array,
    A_wq: jax.Array,
    A_wo: jax.Array,
    B_x: jax.Array,
    B_w_r: jax.Array,
    B_w_gate: jax.Array,
    B_w_up: jax.Array,
    B_w_down: jax.Array,
):
    del B_x
    out = pl.pallas_call(
        _kernel,
        out_shape=jax.ShapeDtypeStruct((B, D), bf16),
        in_specs=[pl.BlockSpec(memory_space=pl.ANY)] * 9,
        out_specs=pl.BlockSpec(memory_space=pltpu.VMEM),
        scratch_shapes=[
            pltpu.VMEM((B, D), bf16),
            pltpu.VMEM((D,), bf16),
            pltpu.VMEM((D // 2, H * DH), u32),
            pltpu.VMEM((H * DH // 2, D), u32),
            pltpu.VMEM((D // 2, FF), u32),
            pltpu.VMEM((D // 2, FF), u32),
            pltpu.VMEM((FF // 2, D), u32),
            pltpu.VMEM((B, NP, 2, W // 16, 128), bf16),
            pltpu.VMEM((B, NP, 2, W // 16, 128), bf16),
            pltpu.VMEM((8, D), f32),
            pltpu.VMEM((H, 8, 128), f32),
            pltpu.SemaphoreType.DMA((NW + B * SEMS_PER_ROW,)),
        ],
        compiler_params=pltpu.CompilerParams(vmem_limit_bytes=124 * 1024 * 1024,
                                             disable_semaphore_checks=True),
        name="fused_decode",
    )(A_x.reshape(B, D), B_w_r, _tile_view(A_k_cache), _tile_view(A_v_cache),
      A_wq, A_wo, B_w_gate, B_w_up, B_w_down)
    return out.reshape(B, 1, D)
```

```python
import contextlib
import functools

import jax
import jax.numpy as jnp
from jax import lax
import jax.experimental.pallas as pl
import jax.experimental.pallas.tpu as pltpu

f32, bf16, u32 = jnp.float32, jnp.bfloat16, jnp.uint32

try:
    _OVR
except NameError:
    _OVR = {}

B, D, H, DH, SK, FF = 4, 640, 32, 192, 4096, 1536
W = min(4096, max(256, SK // 4))
RT = DH // 8
CT = W // 128
NT = H * DH // 128
NP = H * RT // 2
V_CHUNKS = ((0, 24, True), (24, 12, True), (36, 6, True), (42, 3, True), (45, 2, False), (47, 1, False))
NW = 7
SEMS_PER_ROW = 2 * (1 + len(V_CHUNKS))
NSLOT = 2
HF = H - 2
NVT = _OVR.get("NVT", 30)
SCALE = DH ** -0.5
LOG2E = 1.4426950408889634
EPS = 1e-5

PAIR_ORDER = (H // 2 - 1,) + tuple(range(H // 2 - 1))
TILE_ORDER = tuple(3 * j + i for j in PAIR_ORDER for i in range(3))


def _scope(name):
    return jax.named_scope(name) if _OVR.get("SCOPES") else contextlib.nullcontext()


def _sum(xs):
    return functools.reduce(lambda a, c: a + c, xs)


def _ln_stats(x):
    m = jnp.sum(x, axis=1, keepdims=True) * (1.0 / D)
    xc = x - m
    v = jnp.sum(xc * xc, axis=1, keepdims=True) * (1.0 / D)
    return m, xc, lax.rsqrt(v + EPS)


def _kernel(x_hbm, wr_hbm, k_hbm, v_hbm, wq_hbm, wo_hbm, wg_hbm, wu_hbm, wd_hbm,
            out_ref,
            x_v, wr_v, wq_v, wo_v, wg_v, wu_v, wd_v, k_v, v_v, vf_v, wof_v,
            csq_v, csg_v, csu_v, xf_v, p_v, sems):
    w_src = (wq_hbm, x_hbm, wr_hbm, wo_hbm, wg_hbm, wu_hbm, wd_hbm)
    w_dst = (wq_v.bitcast(bf16), x_v, wr_v) + tuple(r.bitcast(bf16) for r in (wo_v, wg_v, wu_v, wd_v))
    w_cp = [pltpu.make_async_copy(s, d, sems.at[i]) for i, (s, d) in enumerate(zip(w_src, w_dst))]
    win = pl.ds((SK - W) // 128, CT)

    def k_copies(b):
        s0 = NW + b * SEMS_PER_ROW
        return [pltpu.make_async_copy(k_hbm.at[b, :, t, win],
                                      k_v.at[b % NSLOT, :, :, pl.ds(8 * t, 8), :],
                                      sems.at[s0 + t]) for t in range(2)]

    def v_copies(b, c):
        t0, nt, split = V_CHUNKS[c]
        rows = pl.ds(t0 * 8, nt * 8)
        s0 = NW + b * SEMS_PER_ROW + 2 * (1 + c)
        if split:
            return [pltpu.make_async_copy(v_hbm.at[b, rows, t, win], v_v.at[b % NSLOT, rows, t],
                                          sems.at[s0 + t]) for t in range(2)]
        return [pltpu.make_async_copy(v_hbm.at[b, rows, :, win], v_v.at[b % NSLOT, rows],
                                      sems.at[s0])]

    def start_row(b):
        for cp in k_copies(b):
            cp.start()
        for c in range(len(V_CHUNKS)):
            for cp in v_copies(b, c):
                cp.start()

    for cp in w_cp:
        cp.start()
    for b in range(NSLOT):
        start_row(b)

    lane = lax.broadcasted_iota(jnp.int32, (8, 128), 1)
    row = lax.broadcasted_iota(jnp.int32, (8, 128), 0)
    k32 = k_v.bitcast(u32)

    def wtile(ref, rows, cols):
        return pltpu.bitcast(ref[rows, cols], bf16)

    def blk(i, n):
        if isinstance(i, int):
            return pl.ds(i * n, n)
        return pl.ds(pl.multiple_of(i * n, n), n)

    def merge_tree(vals, idx):
        bit = 0
        while len(vals) > 1:
            odd = ((idx >> bit) & 1) == 1
            vals = [jnp.where(odd, vals[2 * i + 1], vals[2 * i]) for i in range(len(vals) // 2)]
            bit += 1
        return vals[0]

    def q_tile(xb, mean, tile, middle):
        cols = blk(tile, 128)
        q = jnp.dot(xb, wtile(wq_v, slice(None), cols), preferred_element_type=f32)
        q = q - mean * csq_v[:, cols]
        if middle:
            q = jnp.concatenate([jnp.where(lane < 64, q, 0.0), jnp.where(lane >= 64, q, 0.0)], axis=0)
        return q.astype(bf16)

    def k_tile(slot, tile, c):
        w = k32[slot, blk(tile, 8), c]
        return pltpu.bitcast(w.reshape(64, 128), bf16)

    def scores_first(slot, j, q0, q1):
        ra, rb = [], []
        for c in range(CT):
            r1 = jnp.dot(q1, k_tile(slot, 3 * j + 1, c), preferred_element_type=f32)
            r0 = jnp.dot(q0, k_tile(slot, 3 * j, c), preferred_element_type=f32)
            ra.append(r0 + r1[0:8])
            rb.append(r1[8:16])
        return merge_tree(ra, row), merge_tree(rb, row)

    def scores_second(slot, j, q2, mid):
        r = [jnp.dot(q2, k_tile(slot, 3 * j + 2, c), preferred_element_type=f32) for c in range(CT)]
        return merge_tree(r, row) + mid

    def softmax(s, sc):
        m = jnp.max(jnp.max(s, axis=1, keepdims=True), axis=0, keepdims=True)
        e = jnp.exp2((s - m) * sc)
        l = jnp.sum(jnp.sum(e, axis=1, keepdims=True), axis=0, keepdims=True)
        r = pl.reciprocal(l, approx=True)
        return e * (r * (2.0 - l * r))

    def p_rows(p):
        return [jnp.broadcast_to(p[c:c + 1, :], (8, 128)) for c in range(CT)]

    def v_bf16(slot, h, rt):
        return v_v[slot, h * (RT // 2) + rt // 2, rt % 2].reshape(CT * 8, 128).astype(f32)

    def pv(v, pb):
        a = v[0:8] * pb[0]
        for c in range(1, CT):
            a = a + v[c * 8:(c + 1) * 8] * pb[c]
        return jnp.broadcast_to(jnp.sum(a, axis=1, keepdims=True), (8, 128))

    def o_lhs(oc):
        o = merge_tree(oc, lane >> 3)
        return jnp.where((lane & 7) == row, o, 0.0).astype(bf16)

    def proj_mxu(lhs, tile):
        return jnp.dot(lhs, wtile(wo_v, blk(tile, 64), slice(None)), preferred_element_type=f32)

    def proj_vpu(oc, w):
        return w * jnp.concatenate([oc] * (D // 128), axis=1)

    def fold_rows(y):
        return jnp.broadcast_to(jnp.sum(y, axis=0, keepdims=True), (8, D))

    def attn_streaming(x, b):
        slot = b % NSLOT
        mean, _, rstd = _ln_stats(x)
        xb = x.astype(bf16)
        sc = rstd * (SCALE * LOG2E)
        with _scope("wait_k"):
            for cp in k_copies(b):
                cp.wait()

        def scores(g, carry):
            q = [q_tile(xb, mean, 6 * g + i, i % 3 == 1) for i in range(6)]
            for i in range(2):
                j = 2 * g + i
                sa, mid = scores_first(slot, j, q[3 * i], q[3 * i + 1])
                sb = scores_second(slot, j, q[3 * i + 2], mid)
                p_v[2 * j] = softmax(sa, sc)
                p_v[2 * j + 1] = softmax(sb, sc)
            return carry

        with _scope("scores"):
            lax.fori_loop(0, H // 4, scores, 0)

        def head_pair(j, carry):
            y, prev = carry
            for c, (t0, _, _) in enumerate(V_CHUNKS[:-2]):
                @pl.when(j == t0 // 3)
                def _():
                    for cp in v_copies(b, c):
                        cp.wait()
            jp = jnp.maximum(j - 1, 0)
            y = y + _sum([proj_mxu(prev[i], 3 * jp + i) for i in range(3)])
            oc = []
            for i in range(2):
                h = 2 * j + i
                pb = p_rows(p_v[h])
                for rt in range(RT):
                    v = v_bf16(slot, h, rt)
                    vf_v[h, rt] = v
                    oc.append(pv(v, pb))
            return y, tuple(o_lhs(oc[16 * i:16 * i + 16]) for i in range(3))

        with _scope("pv_loop"):
            y, prev = lax.fori_loop(
                0, H // 2 - 1, head_pair,
                (jnp.zeros((8, D), f32), (jnp.zeros((8, 128), bf16),) * 3))
        for cp in v_copies(b, len(V_CHUNKS) - 2):
            cp.wait()
        y = y + _sum([proj_mxu(prev[i], NT - 6 + i) for i in range(3)])
        pb = p_rows(p_v[H - 2])
        oc = [pv(v_bf16(slot, H - 2, rt), pb) for rt in range(RT)]
        pb = p_rows(p_v[H - 1])
        oc += [pv(v_bf16(slot, H - 1, rt), pb) for rt in range(8)]
        lhs = [o_lhs(oc[:16]), o_lhs(oc[16:])]
        with _scope("wait_last"):
            for cp in v_copies(b, len(V_CHUNKS) - 1):
                cp.wait()
        y = y + proj_mxu(lhs[0], NT - 3) + proj_mxu(lhs[1], NT - 2)
        base = TILE_ORDER.index(NT - 1) * 128
        ys = [y, None]
        for rt in range(8, RT):
            d = proj_vpu(pv(v_bf16(slot, H - 1, rt), pb), wof_v[pl.ds(base + (rt - 8) * 8, 8), :])
            ys[rt % 2] = d if ys[rt % 2] is None else ys[rt % 2] + d
        return fold_rows(ys[0] + ys[1])

    def attn_resident(x, b):
        a_ahead, a0, b_ahead = _OVR.get("A_AHEAD", 2), _OVR.get("A0", 1), _OVR.get("B_AHEAD", 2)
        r_lag, nacc = _OVR.get("R_LAG", 20), _OVR.get("NACC", 3)
        slot = b % NSLOT
        mean, _, rstd = _ln_stats(x)
        xb = x.astype(bf16)
        sc = rstd * (SCALE * LOG2E)
        q, p, mid, oc = {}, {}, {}, {}
        ys = [None] * nacc
        n_a = n_b = n_d = 0

        def dv(g):
            d = proj_vpu(oc.pop(g), wof_v[pl.ds(g * 8, 8), :])
            ys[g % nacc] = d if ys[g % nacc] is None else ys[g % nacc] + d

        for i in range(H):
            while n_b < H and n_b <= i + b_ahead:
                while n_a < NT and n_a * 128 < (n_b + 1 + min(a_ahead, a0 + n_b)) * DH:
                    q[n_a] = q_tile(xb, mean, TILE_ORDER[n_a], n_a % 3 == 1)
                    n_a += 1
                jj = n_b // 2
                if n_b % 2 == 0:
                    s, mid[jj] = scores_first(slot, PAIR_ORDER[jj], q.pop(3 * jj), q.pop(3 * jj + 1))
                else:
                    s = scores_second(slot, PAIR_ORDER[jj], q.pop(3 * jj + 2), mid.pop(jj))
                p[n_b] = softmax(s, sc)
                n_b += 1
            h = 2 * PAIR_ORDER[i // 2] + i % 2
            pb = p_rows(p.pop(i))
            for rt in range(RT):
                v = vf_v[h, rt] if h < HF else v_bf16(slot, h, rt)
                oc[i * RT + rt] = pv(v, pb)
                while n_d < NVT * 16 and n_d + r_lag <= i * RT + rt:
                    dv(n_d)
                    n_d += 1
        for t in range(NVT, NT):
            ys.append(proj_mxu(o_lhs([oc.pop(16 * t + i) for i in range(16)]), TILE_ORDER[t]))
        while n_d < NVT * 16:
            dv(n_d)
            n_d += 1
        return fold_rows(_sum(ys[nacc:] + ys[:nacc]))

    def mod_block(x, wr):
        mean, xc, rstd = _ln_stats(x)
        xb = x.astype(bf16)
        r = jnp.sum(xc * wr, axis=1, keepdims=True) * rstd
        mr = mean * rstd
        hid = []
        for t in range(FF // 128):
            cols = blk(t, 128)
            g = jnp.dot(xb, wtile(wg_v, slice(None), cols), preferred_element_type=f32)
            u = jnp.dot(xb, wtile(wu_v, slice(None), cols), preferred_element_type=f32)
            g = g * rstd - mr * csg_v[:, cols]
            u = u * rstd - mr * csu_v[:, cols]
            hid.append((g * jax.nn.sigmoid(g) * u).astype(bf16))
        y = _sum([jnp.dot(hid[t], wtile(wd_v, blk(t, 64), slice(None)), preferred_element_type=f32)
                  for t in range(FF // 128)])
        return (x + xc * rstd) + y * jax.nn.sigmoid(r)

    ones = jnp.ones((8, D), bf16)

    def colsum(w_v, cs_v, n):
        def body(t, carry):
            cols = blk(t, 512)
            cs_v[:, cols] = jnp.dot(ones, wtile(w_v, slice(None), cols), preferred_element_type=f32)
            return carry
        lax.fori_loop(0, n // 512, body, 0)

    for cp in w_cp[:3]:
        cp.wait()
    xf_v[0:B, :] = x_v[...].astype(f32)
    wr = wr_v[...].astype(f32).reshape(1, D)
    colsum(wq_v, csq_v, H * DH)
    w_cp[3].wait()

    def unpack_wo(t, carry):
        src = jnp.where(t < 3, t + (NT - 3), t - 3)
        wof_v[blk(t, 128), :] = wtile(wo_v, blk(src, 64), slice(None)).astype(f32)
        return carry

    lax.fori_loop(0, NVT, unpack_wo, 0)
    w_cp[4].wait()
    colsum(wg_v, csg_v, FF)
    w_cp[5].wait()
    colsum(wu_v, csu_v, FF)
    w_cp[6].wait()

    def batch_body(b, carry):
        @pl.when(jnp.logical_and(b >= 1, b + NSLOT - 1 < B))
        def _():
            start_row(b + NSLOT - 1)

        x = jnp.broadcast_to(xf_v[pl.ds(b, 1), :], (8, D))
        x = x + attn_streaming(x, b)
        with _scope("mod1"):
            x = mod_block(x, wr)
        with _scope("attn2"):
            x = x + attn_resident(x, b)
        with _scope("mod2"):
            x = mod_block(x, wr)
        xf_v[pl.ds(b, 1), :] = x[0:1, :]
        return carry

    lax.fori_loop(0, B, batch_body, 0)
    out_ref[...] = xf_v[0:B, :].astype(bf16)


def _tile_view(c):
    c = c.reshape(B, H, SK // 128, 128, RT, 8).transpose(0, 1, 4, 2, 5, 3)
    return c.reshape(B, NP, 2, SK // 128, 8, 128)


@jax.jit
def pallas_interleave_layers__sliding_block_cached__moe_arch_mod__decode_kernel(
    A_x: jax.Array,
    A_k_cache: jax.Array,
    A_v_cache: jax.Array,
    A_wq: jax.Array,
    A_wo: jax.Array,
    B_x: jax.Array,
    B_w_r: jax.Array,
    B_w_gate: jax.Array,
    B_w_up: jax.Array,
    B_w_down: jax.Array,
):
    del B_x
    out = pl.pallas_call(
        _kernel,
        out_shape=jax.ShapeDtypeStruct((B, D), bf16),
        in_specs=[pl.BlockSpec(memory_space=pl.ANY)] * 9,
        out_specs=pl.BlockSpec(memory_space=pltpu.VMEM),
        scratch_shapes=[
            pltpu.VMEM((B, D), bf16),
            pltpu.VMEM((D,), bf16),
            pltpu.VMEM((D // 2, H * DH), u32),
            pltpu.VMEM((H * DH // 2, D), u32),
            pltpu.VMEM((D // 2, FF), u32),
            pltpu.VMEM((D // 2, FF), u32),
            pltpu.VMEM((FF // 2, D), u32),
            pltpu.VMEM((NSLOT, NP, CT, 16, 128), bf16),
            pltpu.VMEM((NSLOT, NP, 2, CT, 8, 128), bf16),
            pltpu.VMEM((HF, RT, CT * 8, 128), f32),
            pltpu.VMEM((NVT * 128, D), f32),
            pltpu.VMEM((8, H * DH), f32),
            pltpu.VMEM((8, FF), f32),
            pltpu.VMEM((8, FF), f32),
            pltpu.VMEM((8, D), f32),
            pltpu.VMEM((H, 8, 128), f32),
            pltpu.SemaphoreType.DMA((NW + B * SEMS_PER_ROW,)),
        ],
        compiler_params=pltpu.CompilerParams(vmem_limit_bytes=120 * 1024 * 1024,
                                             disable_semaphore_checks=True),
        name="fused_decode",
    )(A_x.reshape(B, D), B_w_r, _tile_view(A_k_cache), _tile_view(A_v_cache),
      A_wq, A_wo, B_w_gate, B_w_up, B_w_down)
    return out.reshape(B, 1, D)
```

```python
import contextlib
import functools

import jax
import jax.numpy as jnp
from jax import lax
import jax.experimental.pallas as pl
import jax.experimental.pallas.tpu as pltpu

f32, bf16, u32 = jnp.float32, jnp.bfloat16, jnp.uint32

try:
    _OVR
except NameError:
    _OVR = {}

B, D, H, DH, SK, FF = 4, 640, 32, 192, 4096, 1536
W = min(4096, max(256, SK // 4))
RT = DH // 8
CT = W // 128
NT = H * DH // 128
NP = H * RT // 2
V_CHUNKS = ((0, 24, True), (24, 12, True), (36, 6, True), (42, 3, True), (45, 2, False), (47, 1, False))
NW = 7
SEMS_PER_ROW = 2 * (1 + len(V_CHUNKS))
NSLOT = 2
HF = H - 2
NVT = _OVR.get("NVT", 30)
NVH = _OVR.get("NVH", 7)
SCALE = DH ** -0.5
LOG2E = 1.4426950408889634
EPS = 1e-5

PAIR_ORDER = (H // 2 - 1,) + tuple(range(H // 2 - 1))
TILE_ORDER = tuple(3 * j + i for j in PAIR_ORDER for i in range(3))


def _scope(name):
    return jax.named_scope(name) if _OVR.get("SCOPES") else contextlib.nullcontext()


def _sum(xs):
    return functools.reduce(lambda a, c: a + c, xs)


def _ln_stats(x):
    m = jnp.sum(x, axis=1, keepdims=True) * (1.0 / D)
    if _OVR.get("ONEPASS", True):
        v = jnp.maximum(jnp.sum(x * x, axis=1, keepdims=True) * (1.0 / D) - m * m, 0.0)
        return m, x - m, lax.rsqrt(v + EPS)
    xc = x - m
    v = jnp.sum(xc * xc, axis=1, keepdims=True) * (1.0 / D)
    return m, xc, lax.rsqrt(v + EPS)


def _kernel(x_hbm, wr_hbm, k_hbm, v_hbm, wq_hbm, wo_hbm, wg_hbm, wu_hbm, wd_hbm,
            out_ref,
            x_v, wr_v, wq_v, wo_v, wg_v, wu_v, wd_v, k_v, v_v, vf_v, wof_v, wgut_v,
            csq_v, csg_v, csu_v, xf_v, p_v, zero_s, sems):
    w_src = (wq_hbm, x_hbm, wr_hbm, wo_hbm, wg_hbm, wu_hbm, wd_hbm)
    w_dst = (wq_v.bitcast(bf16), x_v, wr_v) + tuple(
        r.bitcast(bf16) for r in (wo_v, wg_v.at[0], wu_v.at[0], wd_v.at[0]))
    w_cp = [pltpu.make_async_copy(s, d, sems.at[i]) for i, (s, d) in enumerate(zip(w_src, w_dst))]
    win = pl.ds((SK - W) // 128, CT)

    def k_copies(b):
        s0 = NW + b * SEMS_PER_ROW
        return [pltpu.make_async_copy(k_hbm.at[b, :, t, win],
                                      k_v.at[b % NSLOT, :, :, pl.ds(8 * t, 8), :],
                                      sems.at[s0 + t]) for t in range(2)]

    def v_copies(b, c):
        t0, nt, split = V_CHUNKS[c]
        rows = pl.ds(t0 * 8, nt * 8)
        s0 = NW + b * SEMS_PER_ROW + 2 * (1 + c)
        if split:
            return [pltpu.make_async_copy(v_hbm.at[b, rows, t, win], v_v.at[b % NSLOT, rows, t],
                                          sems.at[s0 + t]) for t in range(2)]
        return [pltpu.make_async_copy(v_hbm.at[b, rows, :, win], v_v.at[b % NSLOT, rows],
                                      sems.at[s0])]

    def start_row(b):
        for cp in k_copies(b):
            cp.start()
        for c in range(len(V_CHUNKS)):
            for cp in v_copies(b, c):
                cp.start()

    for cp in w_cp:
        cp.start()
    for b in range(NSLOT):
        start_row(b)

    lane = lax.broadcasted_iota(jnp.int32, (8, 128), 1)
    row = lax.broadcasted_iota(jnp.int32, (8, 128), 0)
    k32 = k_v.bitcast(u32)

    def wtile(ref, rows, cols):
        return pltpu.bitcast(ref[rows, cols], bf16)

    def blk(i, n):
        if isinstance(i, int):
            return pl.ds(i * n, n)
        return pl.ds(pl.multiple_of(i * n, n), n)

    def merge_tree(vals, idx):
        bit = 0
        while len(vals) > 1:
            odd = ((idx >> bit) & 1) == 1
            vals = [jnp.where(odd, vals[2 * i + 1], vals[2 * i]) for i in range(len(vals) // 2)]
            bit += 1
        return vals[0]

    def q_tile(xb, mean, tile, middle):
        cols = blk(tile, 128)
        q = jnp.dot(xb, wtile(wq_v, slice(None), cols), preferred_element_type=f32)
        q = q - mean * csq_v[:, cols]
        if middle:
            q = jnp.concatenate([jnp.where(lane < 64, q, 0.0), jnp.where(lane >= 64, q, 0.0)], axis=0)
        return q.astype(bf16)

    def k_tile(slot, tile, c):
        w = k32[slot, blk(tile, 8), c]
        return pltpu.bitcast(w.reshape(64, 128), bf16)

    def scores_first(slot, j, q0, q1):
        ra, rb = [], []
        for c in range(CT):
            r1 = jnp.dot(q1, k_tile(slot, 3 * j + 1, c), preferred_element_type=f32)
            r0 = jnp.dot(q0, k_tile(slot, 3 * j, c), preferred_element_type=f32)
            ra.append(r0 + r1[0:8])
            rb.append(r1[8:16])
        return merge_tree(ra, row), merge_tree(rb, row)

    def scores_second(slot, j, q2, mid):
        r = [jnp.dot(q2, k_tile(slot, 3 * j + 2, c), preferred_element_type=f32) for c in range(CT)]
        return merge_tree(r, row) + mid

    def softmax(s, sc):
        m = jnp.max(jnp.max(s, axis=1, keepdims=True), axis=0, keepdims=True)
        e = jnp.exp2((s - m) * sc)
        l = jnp.sum(jnp.sum(e, axis=1, keepdims=True), axis=0, keepdims=True)
        r = pl.reciprocal(l, approx=True)
        return e * (r * (2.0 - l * r))

    def p_rows(p):
        return [jnp.broadcast_to(p[c:c + 1, :], (8, 128)) for c in range(CT)]

    def v_bf16(slot, h, rt):
        return v_v[slot, h * (RT // 2) + rt // 2, rt % 2].reshape(CT * 8, 128).astype(f32)

    def pv(v, pb):
        a = v[0:8] * pb[0]
        for c in range(1, CT):
            a = a + v[c * 8:(c + 1) * 8] * pb[c]
        return jnp.broadcast_to(jnp.sum(a, axis=1, keepdims=True), (8, 128))

    def o_lhs(oc):
        o = merge_tree(oc, lane >> 3)
        return jnp.where((lane & 7) == row, o, 0.0).astype(bf16)

    def proj_mxu(lhs, tile):
        return jnp.dot(lhs, wtile(wo_v, blk(tile, 64), slice(None)), preferred_element_type=f32)

    def proj_vpu(oc, w):
        return w * jnp.concatenate([oc] * (D // 128), axis=1)

    def fold_rows(y):
        return jnp.broadcast_to(jnp.sum(y, axis=0, keepdims=True), y.shape)

    def rows_dot(x, wt_ref, tile):
        cols = []
        for i in range(16):
            w = wt_ref[pl.ds(tile * 128 + i * 8, 8), :] * x
            a = _sum([w[:, t * 128:(t + 1) * 128] for t in range(D // 128)])
            cols.append(jnp.broadcast_to(jnp.sum(a, axis=1, keepdims=True), (8, 128)))
        return merge_tree(cols, lane >> 3)

    def attn_streaming(x, b, z):
        slot = b % NSLOT
        mean, _, rstd = _ln_stats(x)
        xb = x.astype(bf16)
        sc = rstd * (SCALE * LOG2E)
        with _scope("wait_k"):
            for cp in k_copies(b):
                cp.wait()

        def scores(g, carry):
            q = [q_tile(xb, mean, 6 * g + i, i % 3 == 1) for i in range(6)]
            for i in range(2):
                j = 2 * g + i
                sa, mid = scores_first(slot, j, q[3 * i], q[3 * i + 1])
                sb = scores_second(slot, j, q[3 * i + 2], mid)
                p_v[2 * j] = softmax(sa, sc)
                p_v[2 * j + 1] = softmax(sb, sc)
            return carry

        with _scope("scores"):
            lax.fori_loop(0, H // 4, scores, 0)

        def head_pair(j, carry):
            y, prev = carry
            for c, (t0, _, _) in enumerate(V_CHUNKS[:-2]):
                @pl.when(j == t0 // 3)
                def _():
                    for cp in v_copies(b, c):
                        cp.wait()
            jp = jnp.maximum(j - 1, 0)
            y = y + _sum([proj_mxu(prev[i], 3 * jp + i) for i in range(3)])
            oc = []
            for i in range(2):
                h = 2 * j + i
                pb = p_rows(p_v[h])
                for rt in range(RT):
                    v = v_bf16(slot, h, rt)
                    vf_v[h, rt] = v
                    oc.append(pv(v, pb))
            return y, tuple(o_lhs(oc[16 * i:16 * i + 16]) for i in range(3))

        with _scope("pv_loop"):
            y, prev = lax.fori_loop(
                0, H // 2 - 1, head_pair,
                (jnp.zeros((8, D), f32), (jnp.zeros((8, 128), bf16),) * 3))
        for cp in v_copies(b, len(V_CHUNKS) - 2):
            cp.wait()
        y = y + _sum([proj_mxu(prev[i], NT - 6 + i) for i in range(3)])
        pb = p_rows(p_v[H - 2])
        oc = [pv(v_bf16(slot, H - 2, rt), pb) for rt in range(RT)]
        pb = p_rows(p_v[H - 1])
        oc += [pv(v_bf16(slot, H - 1, rt), pb) for rt in range(8)]
        lhs = [o_lhs(oc[:16]), o_lhs(oc[16:])]
        with _scope("wait_last"):
            for cp in v_copies(b, len(V_CHUNKS) - 1):
                cp.wait()
        y = y + proj_mxu(lhs[0], NT - 3) + proj_mxu(lhs[1], NT - 2)
        base = TILE_ORDER.index(NT - 1) * 128
        ys = [y, None]
        for rt in range(8, RT):
            d = proj_vpu(pv(v_bf16(slot + z, H - 1, rt), pb), wof_v[z, pl.ds(base + (rt - 8) * 8, 8), :])
            ys[rt % 2] = d if ys[rt % 2] is None else ys[rt % 2] + d
        return fold_rows(ys[0] + ys[1])

    def attn_resident(x, b):
        a_ahead, a0, b_ahead = _OVR.get("A_AHEAD", 2), _OVR.get("A0", 1), _OVR.get("B_AHEAD", 2)
        r_lag, nacc = _OVR.get("R_LAG", 20), _OVR.get("NACC", 3)
        slot = b % NSLOT
        mean, _, rstd = _ln_stats(x)
        xb = x.astype(bf16)
        sc = rstd * (SCALE * LOG2E)
        q, p, mid, oc = {}, {}, {}, {}
        ys = [None] * nacc
        n_a = n_b = n_d = 0

        def dv(g):
            d = proj_vpu(oc.pop(g), wof_v[0, pl.ds(g * 8, 8), :])
            ys[g % nacc] = d if ys[g % nacc] is None else ys[g % nacc] + d

        for i in range(H):
            while n_b < H and n_b <= i + b_ahead:
                while n_a < NT and n_a * 128 < (n_b + 1 + min(a_ahead, a0 + n_b)) * DH:
                    q[n_a] = q_tile(xb, mean, TILE_ORDER[n_a], n_a % 3 == 1)
                    n_a += 1
                jj = n_b // 2
                if n_b % 2 == 0:
                    s, mid[jj] = scores_first(slot, PAIR_ORDER[jj], q.pop(3 * jj), q.pop(3 * jj + 1))
                else:
                    s = scores_second(slot, PAIR_ORDER[jj], q.pop(3 * jj + 2), mid.pop(jj))
                p[n_b] = softmax(s, sc)
                n_b += 1
            h = 2 * PAIR_ORDER[i // 2] + i % 2
            pb = p_rows(p.pop(i))
            for rt in range(RT):
                v = vf_v[h, rt] if h < HF else v_bf16(slot, h, rt)
                oc[i * RT + rt] = pv(v, pb)
                while n_d < NVT * 16 and n_d + r_lag <= i * RT + rt:
                    dv(n_d)
                    n_d += 1
        for t in range(NVT, NT):
            ys.append(proj_mxu(o_lhs([oc.pop(16 * t + i) for i in range(16)]), TILE_ORDER[t]))
        while n_d < NVT * 16:
            dv(n_d)
            n_d += 1
        return fold_rows(_sum(ys[nacc:] + ys[:nacc]))

    def mod_block(x, z):
        wg, wu, wd, wgut, csg, csu = (r.at[z] for r in (wg_v, wu_v, wd_v, wgut_v, csg_v, csu_v))
        mean, xc, rstd = _ln_stats(x)
        xb = x.astype(bf16)
        mr = mean * rstd
        r = jnp.sum(x * wr, axis=1, keepdims=True) * rstd - mr * wr_sum
        nm = FF // 128 - NVH
        hid = []
        for t in range(nm):
            cols = blk(t, 128)
            g = jnp.dot(xb, wtile(wg, slice(None), cols), preferred_element_type=f32)
            u = jnp.dot(xb, wtile(wu, slice(None), cols), preferred_element_type=f32)
            g = g * rstd - mr * csg[:, cols]
            u = u * rstd - mr * csu[:, cols]
            hid.append((g * jax.nn.sigmoid(g) * u).astype(bf16))
        for k in range(NVH):
            g = rows_dot(x, wgut, 2 * k) * rstd
            u = rows_dot(x, wgut, 2 * k + 1) * rstd
            hid.append(jnp.where((lane & 7) == row, g * jax.nn.sigmoid(g) * u, 0.0).astype(bf16))
        y = [jnp.dot(hid[t], wtile(wd, blk(t, 64), slice(None)), preferred_element_type=f32)
             for t in range(FF // 128)]
        y = _sum(y[:nm]) + fold_rows(_sum(y[nm:]))
        return (x + xc * rstd) + y * jax.nn.sigmoid(r)

    zero_s[0] = 0
    ones = jnp.ones((8, D), bf16)

    def colsum(w_v, cs_v, n):
        def body(t, carry):
            cols = blk(t, 512)
            cs_v[:, cols] = jnp.dot(ones, wtile(w_v, slice(None), cols), preferred_element_type=f32)
            return carry
        lax.fori_loop(0, n // 512, body, 0)

    for cp in w_cp[:3]:
        cp.wait()
    xf_v[0:B, :] = x_v[...].astype(f32)
    wr = wr_v[...].astype(f32).reshape(1, D)
    wr_sum = jnp.sum(wr, axis=1, keepdims=True)
    colsum(wq_v, csq_v, H * DH)
    w_cp[3].wait()

    def unpack_wo(t, carry):
        src = jnp.where(t < 3, t + (NT - 3), t - 3)
        wof_v[0, blk(t, 128), :] = wtile(wo_v, blk(src, 64), slice(None)).astype(f32)
        return carry

    lax.fori_loop(0, NVT, unpack_wo, 0)
    w_cp[4].wait()
    colsum(wg_v.at[0], csg_v.at[0], FF)
    w_cp[5].wait()
    colsum(wu_v.at[0], csu_v.at[0], FF)

    def centered_transpose(w_v, cs_v, src, wt_v, dst):
        cols = blk(src, 128)
        mu = cs_v[0:1, cols] * (1.0 / D)
        for t in range(D // 128):
            w = wtile(w_v, blk(t, 64), cols).astype(f32) - mu
            wt_v[blk(dst, 128), blk(t, 128)] = w.T

    def prep_gu(k, carry):
        src = FF // 128 - NVH + k
        centered_transpose(wg_v.at[0], csg_v.at[0], src, wgut_v.at[0], 2 * k)
        centered_transpose(wu_v.at[0], csu_v.at[0], src, wgut_v.at[0], 2 * k + 1)
        return carry

    lax.fori_loop(0, NVH, prep_gu, 0)
    w_cp[6].wait()

    def batch_body(b, carry):
        @pl.when(jnp.logical_and(b >= 1, b + NSLOT - 1 < B))
        def _():
            start_row(b + NSLOT - 1)

        x = jnp.broadcast_to(xf_v[pl.ds(b, 1), :], (8, D))
        z = zero_s[0]
        x = x + attn_streaming(x, b, z)
        with _scope("mod1"):
            x = mod_block(x, 0)
        if _OVR.get("FENCE", True):
            wgut_v[z, pl.ds(2 * NVH * 128, 8), pl.ds(0, 128)] = jnp.zeros((8, 128), f32)
            z = 0
        with _scope("attn2"):
            x = x + attn_resident(x, b)
        with _scope("mod2"):
            x = mod_block(x, z)
        xf_v[pl.ds(b, 1), :] = x[0:1, :]
        return carry

    lax.fori_loop(0, B, batch_body, 0)
    out_ref[...] = xf_v[0:B, :].astype(bf16)


def _tile_view(c):
    c = c.reshape(B, H, SK // 128, 128, RT, 8).transpose(0, 1, 4, 2, 5, 3)
    return c.reshape(B, NP, 2, SK // 128, 8, 128)


@jax.jit
def pallas_interleave_layers__sliding_block_cached__moe_arch_mod__decode_kernel(
    A_x: jax.Array,
    A_k_cache: jax.Array,
    A_v_cache: jax.Array,
    A_wq: jax.Array,
    A_wo: jax.Array,
    B_x: jax.Array,
    B_w_r: jax.Array,
    B_w_gate: jax.Array,
    B_w_up: jax.Array,
    B_w_down: jax.Array,
):
    del B_x
    out = pl.pallas_call(
        _kernel,
        out_shape=jax.ShapeDtypeStruct((B, D), bf16),
        in_specs=[pl.BlockSpec(memory_space=pl.ANY)] * 9,
        out_specs=pl.BlockSpec(memory_space=pltpu.VMEM),
        scratch_shapes=[
            pltpu.VMEM((B, D), bf16),
            pltpu.VMEM((D,), bf16),
            pltpu.VMEM((D // 2, H * DH), u32),
            pltpu.VMEM((H * DH // 2, D), u32),
            pltpu.VMEM((1, D // 2, FF), u32),
            pltpu.VMEM((1, D // 2, FF), u32),
            pltpu.VMEM((1, FF // 2, D), u32),
            pltpu.VMEM((NSLOT, NP, CT, 16, 128), bf16),
            pltpu.VMEM((NSLOT, NP, 2, CT, 8, 128), bf16),
            pltpu.VMEM((HF, RT, CT * 8, 128), f32),
            pltpu.VMEM((1, NVT * 128, D), f32),
            pltpu.VMEM((1, 2 * NVH * 128 + 8, D), f32),
            pltpu.VMEM((8, H * DH), f32),
            pltpu.VMEM((1, 8, FF), f32),
            pltpu.VMEM((1, 8, FF), f32),
            pltpu.VMEM((8, D), f32),
            pltpu.VMEM((H, 8, 128), f32),
            pltpu.SMEM((1,), jnp.int32),
            pltpu.SemaphoreType.DMA((NW + B * SEMS_PER_ROW,)),
        ],
        compiler_params=pltpu.CompilerParams(vmem_limit_bytes=120 * 1024 * 1024,
                                             disable_semaphore_checks=True),
        name="fused_decode",
    )(A_x.reshape(B, D), B_w_r, _tile_view(A_k_cache), _tile_view(A_v_cache),
      A_wq, A_wo, B_w_gate, B_w_up, B_w_down)
    return out.reshape(B, 1, D)
```

```python
import contextlib
import functools

import jax
import jax.numpy as jnp
from jax import lax
import jax.experimental.pallas as pl
import jax.experimental.pallas.tpu as pltpu

f32, bf16, u32 = jnp.float32, jnp.bfloat16, jnp.uint32

try:
    _OVR
except NameError:
    _OVR = {}

B, D, H, DH, SK, FF = 4, 640, 32, 192, 4096, 1536
W = min(4096, max(256, SK // 4))
RT = DH // 8
CT = W // 128
NT = H * DH // 128
NP = H * RT // 2
LASTP = _OVR.get("LASTP", 2)
V_CHUNKS = ((0, 192, True), (192, 96, True), (288, 48, True), (336, 24, True), (360, 8, False),
            (368, 8, False), (376, 8 - LASTP, False), (384 - LASTP, LASTP, False))
NW = 7
SEMS_PER_ROW = 2 * (1 + len(V_CHUNKS))
NSLOT = 2
HF = H - 2
NVT = _OVR.get("NVT", 30)
NVL = _OVR.get("NVL", 1)
QV0 = _OVR.get("QV0", 3)
NQV = _OVR.get("NQV", 9)
NVH = _OVR.get("NVH", 7)
SCALE = DH ** -0.5
LOG2E = 1.4426950408889634
EPS = 1e-5

PAIR_ORDER = (H // 2 - 1,) + tuple(range(H // 2 - 1))
TILE_ORDER = tuple(3 * j + i for j in PAIR_ORDER for i in range(3))
VPU_TILES = tuple(range(NVT - NVL)) + tuple(range(NT - NVL, NT))
_VT = _OVR.get("VT", "vvm" * 13 + "vv" + "m" * 7)
VPU_TILES = tuple(t for t in range(NT) if _VT[t % len(_VT)] == "v" or t < 3 or t >= NT - NVL)
NVT = len(VPU_TILES)


def _scope(name):
    return jax.named_scope(name) if _OVR.get("SCOPES") else contextlib.nullcontext()


def _sum(xs):
    return functools.reduce(lambda a, c: a + c, xs)


def _sigmoid(x):
    return 0.5 * jnp.tanh(0.5 * x) + 0.5


def _ln_stats(x):
    m = jnp.sum(x, axis=1, keepdims=True) * (1.0 / D)
    if _OVR.get("ONEPASS", True):
        v = jnp.maximum(jnp.sum(x * x, axis=1, keepdims=True) * (1.0 / D) - m * m, 0.0)
        return m, x - m, lax.rsqrt(v + EPS)
    xc = x - m
    v = jnp.sum(xc * xc, axis=1, keepdims=True) * (1.0 / D)
    return m, xc, lax.rsqrt(v + EPS)


def _kernel(x_hbm, wr_hbm, k_hbm, v_hbm, wq_hbm, wo_hbm, wg_hbm, wu_hbm, wd_hbm,
            out_ref,
            x_v, wr_v, wq_v, wo_v, wg_v, wu_v, wd_v, k_v, v_v, vf_v, wof_v, wgut_v, wqt_v,
            csq_v, csg_v, csu_v, xf_v, p_v, zero_s, sems):
    w_src = (wq_hbm, x_hbm, wr_hbm, wo_hbm, wg_hbm, wu_hbm, wd_hbm)
    w_dst = (wq_v.bitcast(bf16), x_v, wr_v) + tuple(
        r.bitcast(bf16) for r in (wo_v, wg_v.at[0], wu_v.at[0], wd_v.at[0]))
    w_cp = [pltpu.make_async_copy(s, d, sems.at[i]) for i, (s, d) in enumerate(zip(w_src, w_dst))]
    win = pl.ds((SK - W) // 128, CT)

    def k_copies(b):
        s0 = NW + b * SEMS_PER_ROW
        return [pltpu.make_async_copy(k_hbm.at[b, :, t, win],
                                      k_v.at[b % NSLOT, :, :, pl.ds(8 * t, 8), :],
                                      sems.at[s0 + t]) for t in range(2)]

    def v_copies(b, c):
        p0, n, split = V_CHUNKS[c]
        rows = pl.ds(p0, n)
        s0 = NW + b * SEMS_PER_ROW + 2 * (1 + c)
        if split:
            return [pltpu.make_async_copy(v_hbm.at[b, rows, t, win], v_v.at[b % NSLOT, rows, t],
                                          sems.at[s0 + t]) for t in range(2)]
        return [pltpu.make_async_copy(v_hbm.at[b, rows, :, win], v_v.at[b % NSLOT, rows],
                                      sems.at[s0])]

    def start_row(b):
        for cp in k_copies(b):
            cp.start()
        for c in range(len(V_CHUNKS)):
            for cp in v_copies(b, c):
                cp.start()

    for cp in w_cp:
        cp.start()
    for b in range(NSLOT):
        start_row(b)

    lane = lax.broadcasted_iota(jnp.int32, (8, 128), 1)
    row = lax.broadcasted_iota(jnp.int32, (8, 128), 0)
    k32 = k_v.bitcast(u32)

    def wtile(ref, rows, cols):
        return pltpu.bitcast(ref[rows, cols], bf16)

    def blk(i, n):
        if isinstance(i, int):
            return pl.ds(i * n, n)
        return pl.ds(pl.multiple_of(i * n, n), n)

    def merge_tree(vals, idx):
        bit = 0
        while len(vals) > 1:
            odd = ((idx >> bit) & 1) == 1
            vals = [jnp.where(odd, vals[2 * i + 1], vals[2 * i]) for i in range(len(vals) // 2)]
            bit += 1
        return vals[0]

    def q_tile(xb, mean, tile, middle):
        cols = blk(tile, 128)
        q = jnp.dot(xb, wtile(wq_v, slice(None), cols), preferred_element_type=f32)
        return q_lhs(q - mean * csq_v[:, cols], middle)

    def q_lhs(q, middle):
        if middle:
            q = jnp.concatenate([jnp.where(lane < 64, q, 0.0), jnp.where(lane >= 64, q, 0.0)], axis=0)
        return q.astype(bf16)

    def k_tile(slot, tile, c):
        w = k32[slot, blk(tile, 8), c]
        return pltpu.bitcast(w.reshape(64, 128), bf16)

    def scores_first(slot, j, q0, q1):
        ra, rb = [], []
        for c in range(CT):
            r1 = jnp.dot(q1, k_tile(slot, 3 * j + 1, c), preferred_element_type=f32)
            r0 = jnp.dot(q0, k_tile(slot, 3 * j, c), preferred_element_type=f32)
            ra.append(r0 + r1[0:8])
            rb.append(r1[8:16])
        return merge_tree(ra, row), merge_tree(rb, row)

    def scores_second(slot, j, q2, mid):
        r = [jnp.dot(q2, k_tile(slot, 3 * j + 2, c), preferred_element_type=f32) for c in range(CT)]
        return merge_tree(r, row) + mid

    def softmax(s, sc, defer=False):
        m = jnp.max(jnp.max(s, axis=1, keepdims=True), axis=0, keepdims=True)
        e = jnp.exp2((s - m) * sc)
        l = jnp.sum(jnp.sum(e, axis=1, keepdims=True), axis=0, keepdims=True)
        r = pl.reciprocal(l, approx=True)
        r = r * (2.0 - l * r)
        return (e, r) if defer else e * r

    def p_rows(p):
        return [jnp.broadcast_to(p[c:c + 1, :], (8, 128)) for c in range(CT)]

    def v_bf16(slot, h, rt):
        return v_v[slot, h * (RT // 2) + rt // 2, rt % 2].reshape(CT * 8, 128).astype(f32)

    def pv_lanes(v, pb):
        a = v[0:8] * pb[0]
        for c in range(1, CT):
            a = a + v[c * 8:(c + 1) * 8] * pb[c]
        return a

    def lane_sum(a):
        return jnp.broadcast_to(jnp.sum(a, axis=1, keepdims=True), (8, 128))

    def pv(v, pb):
        return lane_sum(pv_lanes(v, pb))

    def o_lhs(oc):
        o = merge_tree(oc, lane >> 3)
        return jnp.where((lane & 7) == row, o, 0.0).astype(bf16)

    def proj_mxu(lhs, tile):
        return jnp.dot(lhs, wtile(wo_v, blk(tile, 64), slice(None)), preferred_element_type=f32)

    def proj_vpu(oc, w):
        return w * jnp.concatenate([oc] * (D // 128), axis=1)

    def fold_rows(y):
        return jnp.broadcast_to(jnp.sum(y, axis=0, keepdims=True), y.shape)

    def rows_dot(x, wt_ref, tile):
        cols = []
        for i in range(16):
            w = wt_ref[pl.ds(tile * 128 + i * 8, 8), :] * x
            a = _sum([w[:, t * 128:(t + 1) * 128] for t in range(D // 128)])
            cols.append(jnp.broadcast_to(jnp.sum(a, axis=1, keepdims=True), (8, 128)))
        return merge_tree(cols, lane >> 3)

    def attn_streaming(x, b, z):
        slot = b % NSLOT
        mean, _, rstd = _ln_stats(x)
        xb = x.astype(bf16)
        sc = rstd * (SCALE * LOG2E)
        with _scope("wait_k"):
            for cp in k_copies(b):
                cp.wait()

        def scores(g, carry):
            q = [q_tile(xb, mean, 6 * g + i, i % 3 == 1) for i in range(6)]
            for i in range(2):
                j = 2 * g + i
                sa, mid = scores_first(slot, j, q[3 * i], q[3 * i + 1])
                sb = scores_second(slot, j, q[3 * i + 2], mid)
                p_v[2 * j] = softmax(sa, sc)
                p_v[2 * j + 1] = softmax(sb, sc)
            return carry

        with _scope("scores"):
            lax.fori_loop(0, H // 4, scores, 0)

        def head_pair(j, carry):
            y, prev = carry
            for c, (p0, _, _) in enumerate(V_CHUNKS[:-4]):
                @pl.when(j == p0 // RT)
                def _():
                    for cp in v_copies(b, c):
                        cp.wait()
            jp = jnp.maximum(j - 1, 0)
            y = y + _sum([proj_mxu(prev[i], 3 * jp + i) for i in range(3)])
            oc = []
            for i in range(2):
                h = 2 * j + i
                pb = p_rows(p_v[h])
                for rt in range(RT):
                    v = v_bf16(slot, h, rt)
                    vf_v[h, rt] = v
                    oc.append(pv(v, pb))
            return y, tuple(o_lhs(oc[16 * i:16 * i + 16]) for i in range(3))

        with _scope("pv_loop"):
            y, prev = lax.fori_loop(
                0, H // 2 - 1, head_pair,
                (jnp.zeros((8, D), f32), (jnp.zeros((8, 128), bf16),) * 3))
        def wait_v(c):
            for cp in v_copies(b, len(V_CHUNKS) + c):
                cp.wait()

        def project(acc, n0, idx):
            ys = [None] * 3
            for n, a in enumerate(acc):
                d = proj_vpu(lane_sum(a), wof_v[idx, pl.ds((n0 + n) * 8, 8), :])
                ys[n % 3] = d if ys[n % 3] is None else ys[n % 3] + d
            return ys

        pbs = [p_rows(p_v[H - 2]), p_rows(p_v[H - 1])]

        def lanes(n0, n1, sl):
            return [pv_lanes(v_bf16(sl, H - 2 + n // RT, n % RT), pbs[n // RT]) for n in range(n0, n1)]

        wait_v(-4)
        y = y + _sum([proj_mxu(prev[i], NT - 6 + i) for i in range(3)])
        y = y + _sum(project(lanes(0, 16, slot), 0, 0))
        wait_v(-3)
        y = y + _sum(project(lanes(16, 32, slot), 16, 0))
        wait_v(-2)
        acc = lanes(32, 48 - 2 * LASTP, slot)
        with _scope("wait_last"):
            wait_v(-1)
        ys = project(acc + lanes(48 - 2 * LASTP, 48, slot + z), 32, z)
        return fold_rows((y + ys[1]) + (ys[2] + ys[0]))

    def attn_resident(x, b, never):
        a_ahead, a0, b_ahead = _OVR.get("A_AHEAD", 2), _OVR.get("A0", 1), _OVR.get("B_AHEAD", 4)
        r_lag, nacc = _OVR.get("R_LAG", 20), _OVR.get("NACC", 3)
        slot = b % NSLOT
        mean, _, rstd = _ln_stats(x)
        xb = x.astype(bf16)
        sc = rstd * (SCALE * LOG2E)
        q, p, mid, oc = {}, {}, {}, {}
        ys = [None] * nacc
        n_a = n_b = n_d = 0
        tie, done, late = _OVR.get("TIE", 3), {}, {}
        vg = [16 * t + i for t in VPU_TILES for i in range(16)]
        for k in range(NQV):
            qk = jnp.where((lane & 7) == row, rows_dot(x, wqt_v, k), 0.0)
            q[QV0 + k] = q_lhs(fold_rows(qk), (QV0 + k) % 3 == 1)

        def dv(n):
            g = vg[n]
            d = proj_vpu(oc.pop(g), wof_v[0, pl.ds(n * 8, 8), :])
            ys[g % nacc] = d if ys[g % nacc] is None else ys[g % nacc] + d
            if tie and (n + 1 == len(vg) or vg[n + 1] // RT != g // RT):
                ys[:nacc] = [_sum([y for y in ys[:nacc] if y is not None])] + [None] * (nacc - 1)
                done[g // RT] = _sum([ys[0][:, t * 128:(t + 1) * 128] for t in range(D // 128)])

        a_tiles = [t for t in range(NT) if not QV0 <= t < QV0 + NQV]
        a_first = _OVR.get("A_FIRST", 0)
        n_defer = _OVR.get("DEFER", 1)
        m_lag = _OVR.get("M_LAG", 10000)
        mt = [t for t in range(NT) if t not in VPU_TILES]
        ym = []

        merged = {}

        def merge(t):
            merged[t] = merge_tree([oc.pop(16 * t + i) for i in range(16)], lane >> 3)
            if _OVR.get("MTIE", 0):
                late.setdefault((16 * t + 15) // RT, []).append(merged[t])

        def dm(t):
            lhs = jnp.where((lane & 7) == row, merged.pop(t), 0.0).astype(bf16)
            d = proj_mxu(lhs, TILE_ORDER[t])
            ym[:] = [d if not ym else ym[0] + d]

        for i in range(H):
            while n_b < H and n_b <= i + b_ahead:
                while n_a < len(a_tiles) and (
                        n_a < a_first
                        or a_tiles[n_a] * 128 < (n_b + 1 + min(a_ahead, a0 + n_b)) * DH):
                    t = a_tiles[n_a]
                    q[t] = q_tile(xb, mean, TILE_ORDER[t], t % 3 == 1)
                    n_a += 1
                jj = n_b // 2
                if n_b % 2 == 0:
                    s, mid[jj] = scores_first(slot, PAIR_ORDER[jj], q.pop(3 * jj), q.pop(3 * jj + 1))
                else:
                    s = scores_second(slot, PAIR_ORDER[jj], q.pop(3 * jj + 2), mid.pop(jj))
                p[n_b] = softmax(s, sc, defer=n_b < n_defer)
                n_b += 1
            h = 2 * PAIR_ORDER[i // 2] + i % 2
            pi = p.pop(i)
            if i < n_defer:
                pi, linv = pi
            dep = late.pop(i - tie, []) + ([done.pop(i - tie)] if i - tie in done else [])
            if dep:
                pi = jnp.where(never, _sum(dep), pi)
            pb = p_rows(pi)
            for rt in range(RT):
                use_f32 = h < HF and rt % _OVR.get("BF_EVERY", 99) != _OVR.get("BF_EVERY", 99) - 1
                v = vf_v[h, rt] if use_f32 else v_bf16(slot, h, rt)
                oc[i * RT + rt] = pv(v, pb) * linv if i < n_defer else pv(v, pb)
                if (i * RT + rt) % 16 == 15 and (i * RT + rt) // 16 in mt:
                    merge((i * RT + rt) // 16)
                while n_d < len(vg) - 16 * NVL and vg[n_d] + r_lag <= i * RT + rt:
                    dv(n_d)
                    n_d += 1
                while mt and mt[0] * 16 + 15 + m_lag <= i * RT + rt:
                    dm(mt.pop(0))
        while mt:
            dm(mt.pop(0))
        y = ym[0]
        tie = 0
        while n_d < len(vg):
            dv(n_d)
            n_d += 1
        return fold_rows(_sum([y] + [y for y in ys if y is not None]))

    def mod_block(x, z):
        wg, wu, wd, wgut, csg, csu = (r.at[z] for r in (wg_v, wu_v, wd_v, wgut_v, csg_v, csu_v))
        mean, xc, rstd = _ln_stats(x)
        xb = x.astype(bf16)
        mr = mean * rstd
        r = jnp.sum(x * wr, axis=1, keepdims=True) * rstd - mr * wr_sum
        nm = FF // 128 - NVH
        hid = []
        for t in range(nm):
            cols = blk(t, 128)
            g = jnp.dot(xb, wtile(wg, slice(None), cols), preferred_element_type=f32)
            u = jnp.dot(xb, wtile(wu, slice(None), cols), preferred_element_type=f32)
            g = g * rstd - mr * csg[:, cols]
            u = u * rstd - mr * csu[:, cols]
            hid.append((g * _sigmoid(g) * u).astype(bf16))
        for k in range(NVH):
            g = rows_dot(x, wgut, 2 * k) * rstd
            u = rows_dot(x, wgut, 2 * k + 1) * rstd
            hid.append(jnp.where((lane & 7) == row, g * _sigmoid(g) * u, 0.0).astype(bf16))
        ya = yb = None
        for t in range(FF // 128):
            d = jnp.dot(hid[t], wtile(wd, blk(t, 64), slice(None)), preferred_element_type=f32)
            if t < nm:
                ya = d if ya is None else d + ya
            else:
                yb = d if yb is None else d + yb
        y = ya + fold_rows(yb)
        return (x + xc * rstd) + y * _sigmoid(r)

    zero_s[0] = 0
    ones = jnp.ones((8, D), bf16)

    def colsum(w_v, cs_v, n):
        def body(t, carry):
            cols = blk(t, 512)
            cs_v[:, cols] = jnp.dot(ones, wtile(w_v, slice(None), cols), preferred_element_type=f32)
            return carry
        lax.fori_loop(0, n // 512, body, 0)

    for cp in w_cp[:3]:
        cp.wait()
    xf_v[0:B, :] = x_v[...].astype(f32)
    wr = wr_v[...].astype(f32).reshape(1, D)
    wr_sum = jnp.sum(wr, axis=1, keepdims=True)
    colsum(wq_v, csq_v, H * DH)

    def tile_order(t):
        return jnp.where(t < 3, t + (NT - 3), t - 3)

    def centered_transpose(w_v, cs_v, src, wt_v, dst):
        cols = blk(src, 128)
        mu = cs_v[0:1, cols] * (1.0 / D)
        for t in range(D // 128):
            w = wtile(w_v, blk(t, 64), cols).astype(f32) - mu
            wt_v[blk(dst, 128), blk(t, 128)] = w.T

    def prep_q(k, carry):
        centered_transpose(wq_v, csq_v, tile_order(QV0 + k), wqt_v, k)
        return carry

    lax.fori_loop(0, NQV, prep_q, 0)
    w_cp[3].wait()

    def unpack_wo(t, carry):
        pos = _sum([jnp.where(t == n, v, 0) for n, v in enumerate(VPU_TILES)])
        wof_v[0, blk(t, 128), :] = wtile(wo_v, blk(tile_order(pos), 64), slice(None)).astype(f32)
        return carry

    lax.fori_loop(0, NVT, unpack_wo, 0)
    w_cp[4].wait()
    colsum(wg_v.at[0], csg_v.at[0], FF)
    w_cp[5].wait()
    colsum(wu_v.at[0], csu_v.at[0], FF)

    def prep_gu(k, carry):
        src = FF // 128 - NVH + k
        centered_transpose(wg_v.at[0], csg_v.at[0], src, wgut_v.at[0], 2 * k)
        centered_transpose(wu_v.at[0], csu_v.at[0], src, wgut_v.at[0], 2 * k + 1)
        return carry

    lax.fori_loop(0, NVH, prep_gu, 0)
    w_cp[6].wait()

    def batch_body(b, carry):
        @pl.when(jnp.logical_and(b >= 1, b + NSLOT - 1 < B))
        def _():
            start_row(b + NSLOT - 1)

        x = jnp.broadcast_to(xf_v[pl.ds(b, 1), :], (8, D))
        z = zero_s[0]
        x = x + attn_streaming(x, b, z)
        with _scope("mod1"):
            x = mod_block(x, 0)
        never = lane < z
        if _OVR.get("FENCE", True):
            wgut_v[z, pl.ds(2 * NVH * 128, 8), pl.ds(0, 128)] = jnp.zeros((8, 128), f32)
            z = 0
        with _scope("attn2"):
            x = x + attn_resident(x, b, never)
        with _scope("mod2"):
            x = mod_block(x, z)
        xf_v[pl.ds(b, 1), :] = x[0:1, :]
        return carry

    lax.fori_loop(0, B, batch_body, 0)
    out_ref[...] = xf_v[0:B, :].astype(bf16)


def _tile_view(c):
    c = c.reshape(B, H, SK // 128, 128, RT, 8).transpose(0, 1, 4, 2, 5, 3)
    return c.reshape(B, NP, 2, SK // 128, 8, 128)


@jax.jit
def pallas_interleave_layers__sliding_block_cached__moe_arch_mod__decode_kernel(
    A_x: jax.Array,
    A_k_cache: jax.Array,
    A_v_cache: jax.Array,
    A_wq: jax.Array,
    A_wo: jax.Array,
    B_x: jax.Array,
    B_w_r: jax.Array,
    B_w_gate: jax.Array,
    B_w_up: jax.Array,
    B_w_down: jax.Array,
):
    del B_x
    out = pl.pallas_call(
        _kernel,
        out_shape=jax.ShapeDtypeStruct((B, D), bf16),
        in_specs=[pl.BlockSpec(memory_space=pl.ANY)] * 9,
        out_specs=pl.BlockSpec(memory_space=pltpu.VMEM),
        scratch_shapes=[
            pltpu.VMEM((B, D), bf16),
            pltpu.VMEM((D,), bf16),
            pltpu.VMEM((D // 2, H * DH), u32),
            pltpu.VMEM((H * DH // 2, D), u32),
            pltpu.VMEM((1, D // 2, FF), u32),
            pltpu.VMEM((1, D // 2, FF), u32),
            pltpu.VMEM((1, FF // 2, D), u32),
            pltpu.VMEM((NSLOT, NP, CT, 16, 128), bf16),
            pltpu.VMEM((NSLOT, NP, 2, CT, 8, 128), bf16),
            pltpu.VMEM((HF, RT, CT * 8, 128), f32),
            pltpu.VMEM((1, NVT * 128, D), f32),
            pltpu.VMEM((1, 2 * NVH * 128 + 8, D), f32),
            pltpu.VMEM((max(NQV, 1) * 128, D), f32),
            pltpu.VMEM((8, H * DH), f32),
            pltpu.VMEM((1, 8, FF), f32),
            pltpu.VMEM((1, 8, FF), f32),
            pltpu.VMEM((8, D), f32),
            pltpu.VMEM((H, 8, 128), f32),
            pltpu.SMEM((1,), jnp.int32),
            pltpu.SemaphoreType.DMA((NW + B * SEMS_PER_ROW,)),
        ],
        compiler_params=pltpu.CompilerParams(vmem_limit_bytes=120 * 1024 * 1024,
                                             disable_semaphore_checks=True),
        name="fused_decode",
    )(A_x.reshape(B, D), B_w_r, _tile_view(A_k_cache), _tile_view(A_v_cache),
      A_wq, A_wo, B_w_gate, B_w_up, B_w_down)
    return out.reshape(B, 1, D)
```

```python
import contextlib
import functools

import jax
import jax.numpy as jnp
from jax import lax
import jax.experimental.pallas as pl
import jax.experimental.pallas.tpu as pltpu

f32, bf16, u32 = jnp.float32, jnp.bfloat16, jnp.uint32

try:
    _OVR
except NameError:
    _OVR = {}

B, D, H, DH, SK, FF = 4, 640, 32, 192, 4096, 1536
W = min(4096, max(256, SK // 4))
RT = DH // 8
CT = W // 128
NT = H * DH // 128
NP = H * RT // 2
LASTP = _OVR.get("LASTP", 2)
V_CHUNKS = ((0, 192, True), (192, 96, True), (288, 48, True), (336, 24, True), (360, 8, False),
            (368, 8, False), (376, 8 - LASTP, False), (384 - LASTP, LASTP, False))
NW = 7
SEMS_PER_ROW = 2 * (1 + len(V_CHUNKS))
NSLOT = 2
HF = H - 2
NVT = _OVR.get("NVT", 30)
NVL = _OVR.get("NVL", 1)
QV0 = _OVR.get("QV0", 3)
NQV = _OVR.get("NQV", 9)
NVH = _OVR.get("NVH", 7)
PADW = _OVR.get("PADW", 128)
PADK = _OVR.get("PADK", 1)
SCALE = DH ** -0.5
LOG2E = 1.4426950408889634
EPS = 1e-5

PAIR_ORDER = (H // 2 - 1,) + tuple(range(H // 2 - 1))
TILE_ORDER = tuple(3 * j + i for j in PAIR_ORDER for i in range(3))
VPU_TILES = tuple(range(NVT - NVL)) + tuple(range(NT - NVL, NT))
_VT = _OVR.get("VT", "vvm" * 13 + "vv" + "m" * 7)
VPU_TILES = tuple(t for t in range(NT) if _VT[t % len(_VT)] == "v" or t < 3 or t >= NT - NVL)
NVT = len(VPU_TILES)


def _scope(name):
    return jax.named_scope(name) if _OVR.get("SCOPES") else contextlib.nullcontext()


def _sum(xs):
    return functools.reduce(lambda a, c: a + c, xs)


def _sigmoid(x):
    return 0.5 * jnp.tanh(0.5 * x) + 0.5


def _ln_stats(x):
    m = jnp.sum(x, axis=1, keepdims=True) * (1.0 / D)
    if _OVR.get("ONEPASS", True):
        v = jnp.maximum(jnp.sum(x * x, axis=1, keepdims=True) * (1.0 / D) - m * m, 0.0)
        return m, x - m, lax.rsqrt(v + EPS)
    xc = x - m
    v = jnp.sum(xc * xc, axis=1, keepdims=True) * (1.0 / D)
    return m, xc, lax.rsqrt(v + EPS)


def _kernel(x_hbm, wr_hbm, k_hbm, v_hbm, wq_hbm, wo_hbm, wg_hbm, wu_hbm, wd_hbm,
            out_ref,
            x_v, wr_v, wq_v, wo_v, wg_v, wu_v, wd_v, k_v, v_v, vf_v, wof_v, wgut_v, wqt_v,
            csq_v, csg_v, csu_v, xf_v, p_v, zero_s, sems):
    w_src = (wq_hbm, x_hbm, wr_hbm, wo_hbm, wg_hbm, wu_hbm, wd_hbm)
    w_dst = (wq_v.at[:, pl.ds(0, H * DH)].bitcast(bf16), x_v, wr_v, wo_v.bitcast(bf16),
             wg_v.at[0, :, pl.ds(0, FF)].bitcast(bf16), wu_v.at[0, :, pl.ds(0, FF)].bitcast(bf16),
             wd_v.at[0].bitcast(bf16))
    w_cp = [pltpu.make_async_copy(s, d, sems.at[i]) for i, (s, d) in enumerate(zip(w_src, w_dst))]
    win = pl.ds((SK - W) // 128, CT)

    def k_copies(b):
        s0 = NW + b * SEMS_PER_ROW
        return [pltpu.make_async_copy(k_hbm.at[b, :, t, win],
                                      k_v.at[b % NSLOT, :, pl.ds(0, CT), pl.ds(8 * t, 8), :],
                                      sems.at[s0 + t]) for t in range(2)]

    def v_copies(b, c):
        p0, n, split = V_CHUNKS[c]
        rows = pl.ds(p0, n)
        s0 = NW + b * SEMS_PER_ROW + 2 * (1 + c)
        if split:
            return [pltpu.make_async_copy(v_hbm.at[b, rows, t, win], v_v.at[b % NSLOT, rows, t],
                                          sems.at[s0 + t]) for t in range(2)]
        return [pltpu.make_async_copy(v_hbm.at[b, rows, :, win], v_v.at[b % NSLOT, rows],
                                      sems.at[s0])]

    def start_row(b):
        for cp in k_copies(b):
            cp.start()
        for c in range(len(V_CHUNKS)):
            for cp in v_copies(b, c):
                cp.start()

    for cp in w_cp:
        cp.start()
    for b in range(NSLOT):
        start_row(b)

    lane = lax.broadcasted_iota(jnp.int32, (8, 128), 1)
    row = lax.broadcasted_iota(jnp.int32, (8, 128), 0)
    k32 = k_v.bitcast(u32)

    def wtile(ref, rows, cols):
        return pltpu.bitcast(ref[rows, cols], bf16)

    def blk(i, n):
        if isinstance(i, int):
            return pl.ds(i * n, n)
        return pl.ds(pl.multiple_of(i * n, n), n)

    def merge_tree(vals, idx):
        bit = 0
        while len(vals) > 1:
            odd = ((idx >> bit) & 1) == 1
            vals = [jnp.where(odd, vals[2 * i + 1], vals[2 * i]) for i in range(len(vals) // 2)]
            bit += 1
        return vals[0]

    def q_tile(xb, mean, tile, middle):
        cols = blk(tile, 128)
        q = jnp.dot(xb, wtile(wq_v, slice(None), cols), preferred_element_type=f32)
        return q_lhs(q - mean * csq_v[:, cols], middle)

    def q_lhs(q, middle):
        if middle:
            q = jnp.concatenate([jnp.where(lane < 64, q, 0.0), jnp.where(lane >= 64, q, 0.0)], axis=0)
        return q.astype(bf16)

    def k_tile(slot, tile, c):
        w = k32[slot, blk(tile, 8), c]
        return pltpu.bitcast(w.reshape(64, 128), bf16)

    def scores_first(slot, j, q0, q1):
        ra, rb = [], []
        for c in range(CT):
            r1 = jnp.dot(q1, k_tile(slot, 3 * j + 1, c), preferred_element_type=f32)
            r0 = jnp.dot(q0, k_tile(slot, 3 * j, c), preferred_element_type=f32)
            ra.append(r0 + r1[0:8])
            rb.append(r1[8:16])
        return merge_tree(ra, row), merge_tree(rb, row)

    def scores_second(slot, j, q2, mid):
        r = [jnp.dot(q2, k_tile(slot, 3 * j + 2, c), preferred_element_type=f32) for c in range(CT)]
        return merge_tree(r, row) + mid

    def softmax(s, sc, defer=False):
        m = jnp.max(jnp.max(s, axis=1, keepdims=True), axis=0, keepdims=True)
        e = jnp.exp2((s - m) * sc)
        l = jnp.sum(jnp.sum(e, axis=1, keepdims=True), axis=0, keepdims=True)
        r = pl.reciprocal(l, approx=True)
        r = r * (2.0 - l * r)
        return (e, r) if defer else e * r

    def p_rows(p):
        return [jnp.broadcast_to(p[c:c + 1, :], (8, 128)) for c in range(CT)]

    def v_bf16(slot, h, rt):
        return v_v[slot, h * (RT // 2) + rt // 2, rt % 2].reshape(CT * 8, 128).astype(f32)

    def pv_lanes(v, pb):
        a = v[0:8] * pb[0]
        for c in range(1, CT):
            a = a + v[c * 8:(c + 1) * 8] * pb[c]
        return a

    def lane_sum(a):
        return jnp.broadcast_to(jnp.sum(a, axis=1, keepdims=True), (8, 128))

    def pv(v, pb):
        return lane_sum(pv_lanes(v, pb))

    def o_lhs(oc):
        o = merge_tree(oc, lane >> 3)
        return jnp.where((lane & 7) == row, o, 0.0).astype(bf16)

    def proj_mxu(lhs, tile):
        return jnp.dot(lhs, wtile(wo_v, blk(tile, 64), slice(None)), preferred_element_type=f32)

    def proj_vpu(oc, w):
        return w * jnp.concatenate([oc] * (D // 128), axis=1)

    def fold_rows(y):
        return jnp.broadcast_to(jnp.sum(y, axis=0, keepdims=True), y.shape)

    def rows_dot(x, wt_ref, tile):
        cols = []
        for i in range(16):
            w = wt_ref[pl.ds(tile * 128 + i * 8, 8), :] * x
            a = _sum([w[:, t * 128:(t + 1) * 128] for t in range(D // 128)])
            cols.append(jnp.broadcast_to(jnp.sum(a, axis=1, keepdims=True), (8, 128)))
        return merge_tree(cols, lane >> 3)

    def attn_streaming(x, b, z):
        slot = b % NSLOT
        mean, _, rstd = _ln_stats(x)
        xb = x.astype(bf16)
        sc = rstd * (SCALE * LOG2E)
        with _scope("wait_k"):
            for cp in k_copies(b):
                cp.wait()

        def scores(g, carry):
            q = [q_tile(xb, mean, 6 * g + i, i % 3 == 1) for i in range(6)]
            for i in range(2):
                j = 2 * g + i
                sa, mid = scores_first(slot, j, q[3 * i], q[3 * i + 1])
                sb = scores_second(slot, j, q[3 * i + 2], mid)
                p_v[2 * j] = softmax(sa, sc)
                p_v[2 * j + 1] = softmax(sb, sc)
            return carry

        with _scope("scores"):
            lax.fori_loop(0, H // 4, scores, 0)

        def head_pair(j, carry):
            y, prev = carry
            for c, (p0, _, _) in enumerate(V_CHUNKS[:-4]):
                @pl.when(j == p0 // RT)
                def _():
                    for cp in v_copies(b, c):
                        cp.wait()
            jp = jnp.maximum(j - 1, 0)
            y = y + _sum([proj_mxu(prev[i], 3 * jp + i) for i in range(3)])
            oc = []
            for i in range(2):
                h = 2 * j + i
                pb = p_rows(p_v[h])
                for rt in range(RT):
                    v = v_bf16(slot, h, rt)
                    vf_v[h, rt] = v
                    oc.append(pv(v, pb))
            return y, tuple(o_lhs(oc[16 * i:16 * i + 16]) for i in range(3))

        with _scope("pv_loop"):
            y, prev = lax.fori_loop(
                0, H // 2 - 1, head_pair,
                (jnp.zeros((8, D), f32), (jnp.zeros((8, 128), bf16),) * 3))
        def wait_v(c):
            for cp in v_copies(b, len(V_CHUNKS) + c):
                cp.wait()

        def project(acc, n0, idx):
            ys = [None] * 3
            for n, a in enumerate(acc):
                d = proj_vpu(lane_sum(a), wof_v[idx, pl.ds((n0 + n) * 8, 8), :])
                ys[n % 3] = d if ys[n % 3] is None else ys[n % 3] + d
            return ys

        pbs = [p_rows(p_v[H - 2]), p_rows(p_v[H - 1])]

        def lanes(n0, n1, sl):
            return [pv_lanes(v_bf16(sl, H - 2 + n // RT, n % RT), pbs[n // RT]) for n in range(n0, n1)]

        wait_v(-4)
        y = y + _sum([proj_mxu(prev[i], NT - 6 + i) for i in range(3)])
        y = y + _sum(project(lanes(0, 16, slot), 0, 0))
        wait_v(-3)
        y = y + _sum(project(lanes(16, 32, slot), 16, 0))
        wait_v(-2)
        acc = lanes(32, 48 - 2 * LASTP, slot)
        with _scope("wait_last"):
            wait_v(-1)
        ys = project(acc + lanes(48 - 2 * LASTP, 48, slot + z), 32, z)
        return fold_rows((y + ys[1]) + (ys[2] + ys[0]))

    def attn_resident(x, b, never):
        a_ahead, a0, b_ahead = _OVR.get("A_AHEAD", 2), _OVR.get("A0", 1), _OVR.get("B_AHEAD", 4)
        r_lag, nacc = _OVR.get("R_LAG", 20), _OVR.get("NACC", 3)
        slot = b % NSLOT
        mean, _, rstd = _ln_stats(x)
        xb = x.astype(bf16)
        sc = rstd * (SCALE * LOG2E)
        q, p, mid, oc = {}, {}, {}, {}
        ys = [None] * nacc
        n_a = n_b = n_d = 0
        tie, done, late = _OVR.get("TIE", 3), {}, {}
        vg = [16 * t + i for t in VPU_TILES for i in range(16)]
        for k in range(NQV):
            qk = jnp.where((lane & 7) == row, rows_dot(x, wqt_v, k), 0.0)
            q[QV0 + k] = q_lhs(fold_rows(qk), (QV0 + k) % 3 == 1)

        def dv(n):
            g = vg[n]
            d = proj_vpu(oc.pop(g), wof_v[0, pl.ds(n * 8, 8), :])
            ys[g % nacc] = d if ys[g % nacc] is None else ys[g % nacc] + d
            if tie and (n + 1 == len(vg) or vg[n + 1] // RT != g // RT):
                ys[:nacc] = [_sum([y for y in ys[:nacc] if y is not None])] + [None] * (nacc - 1)
                done[g // RT] = _sum([ys[0][:, t * 128:(t + 1) * 128] for t in range(D // 128)])

        a_tiles = [t for t in range(NT) if not QV0 <= t < QV0 + NQV]
        a_first = _OVR.get("A_FIRST", 0)
        n_defer = _OVR.get("DEFER", 1)
        m_lag = _OVR.get("M_LAG", 10000)
        mt = [t for t in range(NT) if t not in VPU_TILES]
        ym = []

        merged = {}

        def merge(t):
            merged[t] = merge_tree([oc.pop(16 * t + i) for i in range(16)], lane >> 3)
            if _OVR.get("MTIE", 0):
                late.setdefault((16 * t + 15) // RT, []).append(merged[t])

        def dm(t):
            lhs = jnp.where((lane & 7) == row, merged.pop(t), 0.0).astype(bf16)
            d = proj_mxu(lhs, TILE_ORDER[t])
            ym[:] = [d if not ym else ym[0] + d]

        for i in range(H):
            while n_b < H and n_b <= i + b_ahead:
                while n_a < len(a_tiles) and (
                        n_a < a_first
                        or a_tiles[n_a] * 128 < (n_b + 1 + min(a_ahead, a0 + n_b)) * DH):
                    t = a_tiles[n_a]
                    q[t] = q_tile(xb, mean, TILE_ORDER[t], t % 3 == 1)
                    n_a += 1
                jj = n_b // 2
                if n_b % 2 == 0:
                    s, mid[jj] = scores_first(slot, PAIR_ORDER[jj], q.pop(3 * jj), q.pop(3 * jj + 1))
                else:
                    s = scores_second(slot, PAIR_ORDER[jj], q.pop(3 * jj + 2), mid.pop(jj))
                p[n_b] = softmax(s, sc, defer=n_b < n_defer)
                n_b += 1
            h = 2 * PAIR_ORDER[i // 2] + i % 2
            pi = p.pop(i)
            if i < n_defer:
                pi, linv = pi
            dep = late.pop(i - tie, []) + ([done.pop(i - tie)] if i - tie in done else [])
            if dep:
                pi = jnp.where(never, _sum(dep), pi)
            pb = p_rows(pi)
            for rt in range(RT):
                use_f32 = h < HF and rt % _OVR.get("BF_EVERY", 99) != _OVR.get("BF_EVERY", 99) - 1
                v = vf_v[h, rt] if use_f32 else v_bf16(slot, h, rt)
                oc[i * RT + rt] = pv(v, pb) * linv if i < n_defer else pv(v, pb)
                if (i * RT + rt) % 16 == 15 and (i * RT + rt) // 16 in mt:
                    merge((i * RT + rt) // 16)
                while n_d < len(vg) - 16 * NVL and vg[n_d] + r_lag <= i * RT + rt:
                    dv(n_d)
                    n_d += 1
                while mt and mt[0] * 16 + 15 + m_lag <= i * RT + rt:
                    dm(mt.pop(0))
        while mt:
            dm(mt.pop(0))
        y = ym[0]
        tie = 0
        while n_d < len(vg):
            dv(n_d)
            n_d += 1
        return fold_rows(_sum([y] + [y for y in ys if y is not None]))

    def mod_block(x, z):
        wg, wu, wd, wgut, csg, csu = (r.at[z] for r in (wg_v, wu_v, wd_v, wgut_v, csg_v, csu_v))
        mean, xc, rstd = _ln_stats(x)
        xb = x.astype(bf16)
        mr = mean * rstd
        r = jnp.sum(x * wr, axis=1, keepdims=True) * rstd - mr * wr_sum
        nm = FF // 128 - NVH
        hid = []
        for t in range(nm):
            cols = blk(t, 128)
            g = jnp.dot(xb, wtile(wg, slice(None), cols), preferred_element_type=f32)
            u = jnp.dot(xb, wtile(wu, slice(None), cols), preferred_element_type=f32)
            g = g * rstd - mr * csg[:, cols]
            u = u * rstd - mr * csu[:, cols]
            hid.append((g * _sigmoid(g) * u).astype(bf16))
        for k in range(NVH):
            g = rows_dot(x, wgut, 2 * k) * rstd
            u = rows_dot(x, wgut, 2 * k + 1) * rstd
            hid.append(jnp.where((lane & 7) == row, g * _sigmoid(g) * u, 0.0).astype(bf16))
        ya = yb = None
        for t in range(FF // 128):
            d = jnp.dot(hid[t], wtile(wd, blk(t, 64), slice(None)), preferred_element_type=f32)
            if t < nm:
                ya = d if ya is None else d + ya
            else:
                yb = d if yb is None else d + yb
        y = ya + fold_rows(yb)
        return (x + xc * rstd) + y * _sigmoid(r)

    zero_s[0] = 0
    ones = jnp.ones((8, D), bf16)

    def colsum(w_v, cs_v, n):
        def body(t, carry):
            cols = blk(t, 512)
            cs_v[:, cols] = jnp.dot(ones, wtile(w_v, slice(None), cols), preferred_element_type=f32)
            return carry
        lax.fori_loop(0, n // 512, body, 0)

    for cp in w_cp[:3]:
        cp.wait()
    xf_v[0:B, :] = x_v[...].astype(f32)
    wr = wr_v[...].astype(f32).reshape(1, D)
    wr_sum = jnp.sum(wr, axis=1, keepdims=True)
    colsum(wq_v, csq_v, H * DH)

    def tile_order(t):
        return jnp.where(t < 3, t + (NT - 3), t - 3)

    def centered_transpose(w_v, cs_v, src, wt_v, dst):
        cols = blk(src, 128)
        mu = cs_v[0:1, cols] * (1.0 / D)
        for t in range(D // 128):
            w = wtile(w_v, blk(t, 64), cols).astype(f32) - mu
            wt_v[blk(dst, 128), blk(t, 128)] = w.T

    def prep_q(k, carry):
        centered_transpose(wq_v, csq_v, tile_order(QV0 + k), wqt_v, k)
        return carry

    lax.fori_loop(0, NQV, prep_q, 0)
    w_cp[3].wait()

    def unpack_wo(t, carry):
        pos = _sum([jnp.where(t == n, v, 0) for n, v in enumerate(VPU_TILES)])
        wof_v[0, blk(t, 128), :] = wtile(wo_v, blk(tile_order(pos), 64), slice(None)).astype(f32)
        return carry

    lax.fori_loop(0, NVT, unpack_wo, 0)
    w_cp[4].wait()
    colsum(wg_v.at[0], csg_v.at[0], FF)
    w_cp[5].wait()
    colsum(wu_v.at[0], csu_v.at[0], FF)

    def prep_gu(k, carry):
        src = FF // 128 - NVH + k
        centered_transpose(wg_v.at[0], csg_v.at[0], src, wgut_v.at[0], 2 * k)
        centered_transpose(wu_v.at[0], csu_v.at[0], src, wgut_v.at[0], 2 * k + 1)
        return carry

    lax.fori_loop(0, NVH, prep_gu, 0)
    w_cp[6].wait()

    def batch_body(b, carry):
        @pl.when(jnp.logical_and(b >= 1, b + NSLOT - 1 < B))
        def _():
            start_row(b + NSLOT - 1)

        x = jnp.broadcast_to(xf_v[pl.ds(b, 1), :], (8, D))
        z = zero_s[0]
        x = x + attn_streaming(x, b, z)
        with _scope("mod1"):
            x = mod_block(x, 0)
        never = lane < z
        if _OVR.get("FENCE", True):
            wgut_v[z, pl.ds(2 * NVH * 128, 8), pl.ds(0, 128)] = jnp.zeros((8, 128), f32)
            z = 0
        with _scope("attn2"):
            x = x + attn_resident(x, b, never)
        with _scope("mod2"):
            x = mod_block(x, z)
        xf_v[pl.ds(b, 1), :] = x[0:1, :]
        return carry

    lax.fori_loop(0, B, batch_body, 0)
    out_ref[...] = xf_v[0:B, :].astype(bf16)


def _tile_view(c):
    c = c.reshape(B, H, SK // 128, 128, RT, 8).transpose(0, 1, 4, 2, 5, 3)
    return c.reshape(B, NP, 2, SK // 128, 8, 128)


@jax.jit
def pallas_interleave_layers__sliding_block_cached__moe_arch_mod__decode_kernel(
    A_x: jax.Array,
    A_k_cache: jax.Array,
    A_v_cache: jax.Array,
    A_wq: jax.Array,
    A_wo: jax.Array,
    B_x: jax.Array,
    B_w_r: jax.Array,
    B_w_gate: jax.Array,
    B_w_up: jax.Array,
    B_w_down: jax.Array,
):
    del B_x
    out = pl.pallas_call(
        _kernel,
        out_shape=jax.ShapeDtypeStruct((B, D), bf16),
        in_specs=[pl.BlockSpec(memory_space=pl.ANY)] * 9,
        out_specs=pl.BlockSpec(memory_space=pltpu.VMEM),
        scratch_shapes=[
            pltpu.VMEM((B, D), bf16),
            pltpu.VMEM((D,), bf16),
            pltpu.VMEM((D // 2, H * DH + PADW), u32),
            pltpu.VMEM((H * DH // 2, D), u32),
            pltpu.VMEM((1, D // 2, FF + PADW), u32),
            pltpu.VMEM((1, D // 2, FF + PADW), u32),
            pltpu.VMEM((1, FF // 2, D), u32),
            pltpu.VMEM((NSLOT, NP, CT + PADK, 16, 128), bf16),
            pltpu.VMEM((NSLOT, NP, 2, CT, 8, 128), bf16),
            pltpu.VMEM((HF, RT, CT * 8, 128), f32),
            pltpu.VMEM((1, NVT * 128, D), f32),
            pltpu.VMEM((1, 2 * NVH * 128 + 8, D), f32),
            pltpu.VMEM((max(NQV, 1) * 128, D), f32),
            pltpu.VMEM((8, H * DH), f32),
            pltpu.VMEM((1, 8, FF), f32),
            pltpu.VMEM((1, 8, FF), f32),
            pltpu.VMEM((8, D), f32),
            pltpu.VMEM((H, 8, 128), f32),
            pltpu.SMEM((1,), jnp.int32),
            pltpu.SemaphoreType.DMA((NW + B * SEMS_PER_ROW,)),
        ],
        compiler_params=pltpu.CompilerParams(vmem_limit_bytes=120 * 1024 * 1024,
                                             disable_semaphore_checks=True),
        name="fused_decode",
    )(A_x.reshape(B, D), B_w_r, _tile_view(A_k_cache), _tile_view(A_v_cache),
      A_wq, A_wo, B_w_gate, B_w_up, B_w_down)
    return out.reshape(B, 1, D)
```

```python
import contextlib
import functools

import jax
import jax.numpy as jnp
from jax import lax
import jax.experimental.pallas as pl
import jax.experimental.pallas.tpu as pltpu

f32, bf16, u32 = jnp.float32, jnp.bfloat16, jnp.uint32

try:
    _OVR
except NameError:
    _OVR = {}

B, D, H, DH, SK, FF = 4, 640, 32, 192, 4096, 1536
W = min(4096, max(256, SK // 4))
RT = DH // 8
CT = W // 128
NT = H * DH // 128
NP = H * RT // 2
LASTP = _OVR.get("LASTP", 2)
V_CHUNKS = ((0, 192, True), (192, 96, True), (288, 48, True), (336, 24, True), (360, 8, False),
            (368, 8, False), (376, 8 - LASTP, False), (384 - LASTP, LASTP, False))
NW = 7
SEMS_PER_ROW = 2 * (1 + len(V_CHUNKS))
NSLOT = 2
NF = H * RT - _OVR.get("NBF", 2 * LASTP)
NVT = _OVR.get("NVT", 30)
NVL = _OVR.get("NVL", 1)
QV0 = _OVR.get("QV0", 3)
NQV = _OVR.get("NQV", 9)
NVH = _OVR.get("NVH", 7)
PADW = _OVR.get("PADW", 128)
PADK = _OVR.get("PADK", 1)
SCALE = DH ** -0.5
LOG2E = 1.4426950408889634
EPS = 1e-5

PAIR_ORDER = (H // 2 - 1,) + tuple(range(H // 2 - 1))
TILE_ORDER = tuple(3 * j + i for j in PAIR_ORDER for i in range(3))
VPU_TILES = tuple(range(NVT - NVL)) + tuple(range(NT - NVL, NT))
_VT = _OVR.get("VT", "vvm" * 13 + "vv" + "m" * 7)
VPU_TILES = tuple(t for t in range(NT) if _VT[t % len(_VT)] == "v" or t < 3 or t >= NT - NVL)
NVT = len(VPU_TILES)


def _scope(name):
    return jax.named_scope(name) if _OVR.get("SCOPES") else contextlib.nullcontext()


def _sum(xs):
    return functools.reduce(lambda a, c: a + c, xs)


def _sigmoid(x):
    return 0.5 * jnp.tanh(0.5 * x) + 0.5


def _ln_stats(x):
    m = jnp.sum(x, axis=1, keepdims=True) * (1.0 / D)
    if _OVR.get("ONEPASS", True):
        v = jnp.maximum(jnp.sum(x * x, axis=1, keepdims=True) * (1.0 / D) - m * m, 0.0)
        return m, x - m, lax.rsqrt(v + EPS)
    xc = x - m
    v = jnp.sum(xc * xc, axis=1, keepdims=True) * (1.0 / D)
    return m, xc, lax.rsqrt(v + EPS)


def _kernel(x_hbm, wr_hbm, k_hbm, v_hbm, wq_hbm, wo_hbm, wg_hbm, wu_hbm, wd_hbm,
            out_ref,
            x_v, wr_v, wq_v, wo_v, wg_v, wu_v, wd_v, k_v, v_v, vf_v, wof_v, wgut_v, wqt_v,
            csq_v, csg_v, csu_v, xf_v, p_v, zero_s, sems):
    w_src = (wq_hbm, x_hbm, wr_hbm, wo_hbm, wg_hbm, wu_hbm, wd_hbm)
    w_dst = (wq_v.at[:, pl.ds(0, H * DH)].bitcast(bf16), x_v, wr_v, wo_v.bitcast(bf16),
             wg_v.at[0, :, pl.ds(0, FF)].bitcast(bf16), wu_v.at[0, :, pl.ds(0, FF)].bitcast(bf16),
             wd_v.at[0].bitcast(bf16))
    w_cp = [pltpu.make_async_copy(s, d, sems.at[i]) for i, (s, d) in enumerate(zip(w_src, w_dst))]
    win = pl.ds((SK - W) // 128, CT)

    def k_copies(b):
        s0 = NW + b * SEMS_PER_ROW
        return [pltpu.make_async_copy(k_hbm.at[b, :, t, win],
                                      k_v.at[b % NSLOT, :, pl.ds(0, CT), pl.ds(8 * t, 8), :],
                                      sems.at[s0 + t]) for t in range(2)]

    def v_copies(b, c):
        p0, n, split = V_CHUNKS[c]
        rows = pl.ds(p0, n)
        s0 = NW + b * SEMS_PER_ROW + 2 * (1 + c)
        if split:
            return [pltpu.make_async_copy(v_hbm.at[b, rows, t, win], v_v.at[b % NSLOT, rows, t],
                                          sems.at[s0 + t]) for t in range(2)]
        return [pltpu.make_async_copy(v_hbm.at[b, rows, :, win], v_v.at[b % NSLOT, rows],
                                      sems.at[s0])]

    def start_row(b):
        for cp in k_copies(b):
            cp.start()
        for c in range(len(V_CHUNKS)):
            for cp in v_copies(b, c):
                cp.start()

    for cp in w_cp:
        cp.start()
    for b in range(NSLOT):
        start_row(b)

    lane = lax.broadcasted_iota(jnp.int32, (8, 128), 1)
    row = lax.broadcasted_iota(jnp.int32, (8, 128), 0)
    k32 = k_v.bitcast(u32)

    def wtile(ref, rows, cols):
        return pltpu.bitcast(ref[rows, cols], bf16)

    def blk(i, n):
        if isinstance(i, int):
            return pl.ds(i * n, n)
        return pl.ds(pl.multiple_of(i * n, n), n)

    def merge_tree(vals, idx):
        bit = 0
        while len(vals) > 1:
            odd = ((idx >> bit) & 1) == 1
            vals = [jnp.where(odd, vals[2 * i + 1], vals[2 * i]) for i in range(len(vals) // 2)]
            bit += 1
        return vals[0]

    def q_tile(xb, mean, tile, middle):
        cols = blk(tile, 128)
        q = jnp.dot(xb, wtile(wq_v, slice(None), cols), preferred_element_type=f32)
        return q_lhs(q if mean is None else q - mean * csq_v[:, cols], middle)

    def q_lhs(q, middle):
        if middle:
            q = jnp.concatenate([jnp.where(lane < 64, q, 0.0), jnp.where(lane >= 64, q, 0.0)], axis=0)
        return q.astype(bf16)

    def k_tile(slot, tile, c):
        w = k32[slot, blk(tile, 8), c]
        return pltpu.bitcast(w.reshape(64, 128), bf16)

    def scores_first(slot, j, q0, q1):
        ra, rb = [], []
        for c in range(CT):
            r1 = jnp.dot(q1, k_tile(slot, 3 * j + 1, c), preferred_element_type=f32)
            r0 = jnp.dot(q0, k_tile(slot, 3 * j, c), preferred_element_type=f32)
            ra.append(r0 + r1[0:8])
            rb.append(r1[8:16])
        return merge_tree(ra, row), merge_tree(rb, row)

    def scores_second(slot, j, q2, mid):
        r = [jnp.dot(q2, k_tile(slot, 3 * j + 2, c), preferred_element_type=f32) for c in range(CT)]
        return merge_tree(r, row) + mid

    def softmax(s, sc, defer=False):
        m = jnp.max(jnp.max(s, axis=1, keepdims=True), axis=0, keepdims=True)
        e = jnp.exp2((s - m) * sc)
        l = jnp.sum(jnp.sum(e, axis=1, keepdims=True), axis=0, keepdims=True)
        r = pl.reciprocal(l, approx=True)
        r = r * (2.0 - l * r)
        return (e, r) if defer else e * r

    def p_rows(p):
        return [jnp.broadcast_to(p[c:c + 1, :], (8, 128)) for c in range(CT)]

    def v_bf16(slot, h, rt):
        return v_v[slot, h * (RT // 2) + rt // 2, rt % 2].reshape(CT * 8, 128).astype(f32)

    def pv_lanes(v, pb):
        a = v[0:8] * pb[0]
        for c in range(1, CT):
            a = a + v[c * 8:(c + 1) * 8] * pb[c]
        return a

    def lane_sum(a):
        return jnp.broadcast_to(jnp.sum(a, axis=1, keepdims=True), (8, 128))

    def pv(v, pb):
        return lane_sum(pv_lanes(v, pb))

    def o_lhs(oc):
        o = merge_tree(oc, lane >> 3)
        return jnp.where((lane & 7) == row, o, 0.0).astype(bf16)

    def proj_mxu(lhs, tile):
        return jnp.dot(lhs, wtile(wo_v, blk(tile, 64), slice(None)), preferred_element_type=f32)

    def proj_vpu(oc, w):
        return w * jnp.concatenate([oc] * (D // 128), axis=1)

    def fold_rows(y):
        return jnp.broadcast_to(jnp.sum(y, axis=0, keepdims=True), y.shape)

    def rows_dot(x, wt_ref, tile):
        cols = []
        for i in range(16):
            w = wt_ref[pl.ds(tile * 128 + i * 8, 8), :] * x
            a = _sum([w[:, t * 128:(t + 1) * 128] for t in range(D // 128)])
            cols.append(jnp.broadcast_to(jnp.sum(a, axis=1, keepdims=True), (8, 128)))
        return merge_tree(cols, lane >> 3)

    def attn_streaming(x, b, z):
        slot = b % NSLOT
        mean, _, rstd = _ln_stats(x)
        xb = x.astype(bf16)
        sc = rstd * (SCALE * LOG2E)
        with _scope("wait_k"):
            for cp in k_copies(b):
                cp.wait()

        def scores(g, carry):
            q = [q_tile(xb, mean, 6 * g + i, i % 3 == 1) for i in range(6)]
            for i in range(2):
                j = 2 * g + i
                sa, mid = scores_first(slot, j, q[3 * i], q[3 * i + 1])
                sb = scores_second(slot, j, q[3 * i + 2], mid)
                p_v[2 * j] = softmax(sa, sc)
                p_v[2 * j + 1] = softmax(sb, sc)
            return carry

        with _scope("scores"):
            lax.fori_loop(0, H // 4, scores, 0)

        def head_pair(j, carry):
            y, prev = carry
            for c, (p0, _, _) in enumerate(V_CHUNKS[:-4]):
                @pl.when(j == p0 // RT)
                def _():
                    for cp in v_copies(b, c):
                        cp.wait()
            jp = jnp.maximum(j - 1, 0)
            y = y + _sum([proj_mxu(prev[i], 3 * jp + i) for i in range(3)])
            oc = []
            for i in range(2):
                h = 2 * j + i
                pb = p_rows(p_v[h])
                for rt in range(RT):
                    v = v_bf16(slot, h, rt)
                    vf_v[h * RT + rt] = v
                    oc.append(pv(v, pb))
            return y, tuple(o_lhs(oc[16 * i:16 * i + 16]) for i in range(3))

        with _scope("pv_loop"):
            y, prev = lax.fori_loop(
                0, H // 2 - 1, head_pair,
                (jnp.zeros((8, D), f32), (jnp.zeros((8, 128), bf16),) * 3))
        def wait_v(c):
            for cp in v_copies(b, len(V_CHUNKS) + c):
                cp.wait()

        def project(acc, n0, idx):
            ys = [None] * 3
            for n, a in enumerate(acc):
                d = proj_vpu(lane_sum(a), wof_v[idx, pl.ds((n0 + n) * 8, 8), :])
                ys[n % 3] = d if ys[n % 3] is None else ys[n % 3] + d
            return ys

        pbs = [p_rows(p_v[H - 2]), p_rows(p_v[H - 1])]

        def lanes(n0, n1, sl):
            acc = []
            for n in range(n0, n1):
                v = v_bf16(sl, H - 2 + n // RT, n % RT)
                if (H - 2) * RT + n < NF:
                    vf_v[(H - 2) * RT + n] = v
                acc.append(pv_lanes(v, pbs[n // RT]))
            return acc

        wait_v(-4)
        y = y + _sum([proj_mxu(prev[i], NT - 6 + i) for i in range(3)])
        y = y + _sum(project(lanes(0, 16, slot), 0, 0))
        wait_v(-3)
        y = y + _sum(project(lanes(16, 32, slot), 16, 0))
        wait_v(-2)
        acc = lanes(32, 48 - 2 * LASTP, slot)
        with _scope("wait_last"):
            wait_v(-1)
        ys = project(acc + lanes(48 - 2 * LASTP, 48, slot + z), 32, z)
        return fold_rows((y + ys[1]) + (ys[2] + ys[0]))

    def attn_resident(x, b, never):
        a_ahead, a0, b_ahead = _OVR.get("A_AHEAD", 2), _OVR.get("A0", 1), _OVR.get("B_AHEAD", 4)
        r_lag, nacc = _OVR.get("R_LAG", 20), _OVR.get("NACC", 3)
        slot = b % NSLOT
        mean, xc, rstd = _ln_stats(x)
        xb, xcb = x.astype(bf16), xc.astype(bf16)
        sc = rstd * (SCALE * LOG2E)
        q, p, mid, oc = {}, {}, {}, {}
        ys = [None] * nacc
        n_a = n_b = n_d = 0
        tie, done, late = _OVR.get("TIE", 3), {}, {}
        vg = [16 * t + i for t in VPU_TILES for i in range(16)]
        for k in range(NQV):
            qk = jnp.where((lane & 7) == row, rows_dot(x, wqt_v, k), 0.0)
            q[QV0 + k] = q_lhs(fold_rows(qk), (QV0 + k) % 3 == 1)

        def dv(n):
            g = vg[n]
            d = proj_vpu(oc.pop(g), wof_v[0, pl.ds(n * 8, 8), :])
            ys[g % nacc] = d if ys[g % nacc] is None else ys[g % nacc] + d
            if tie and (n + 1 == len(vg) or vg[n + 1] // RT != g // RT):
                ys[:nacc] = [_sum([y for y in ys[:nacc] if y is not None])] + [None] * (nacc - 1)
                done[g // RT] = _sum([ys[0][:, t * 128:(t + 1) * 128] for t in range(D // 128)])

        a_tiles = [t for t in range(NT) if not QV0 <= t < QV0 + NQV]
        a_first = _OVR.get("A_FIRST", 0)
        n_defer = _OVR.get("DEFER", 1)
        m_lag = _OVR.get("M_LAG", 10000)
        mt = [t for t in range(NT) if t not in VPU_TILES]
        ym = []

        merged = {}

        def merge(t):
            merged[t] = merge_tree([oc.pop(16 * t + i) for i in range(16)], lane >> 3)
            if _OVR.get("MTIE", 0):
                late.setdefault((16 * t + 15) // RT, []).append(merged[t])

        def dm(t):
            lhs = jnp.where((lane & 7) == row, merged.pop(t), 0.0).astype(bf16)
            d = proj_mxu(lhs, TILE_ORDER[t])
            ym[:] = [d if not ym else ym[0] + d]

        for i in range(H):
            while n_b < H and n_b <= i + b_ahead:
                while n_a < len(a_tiles) and (
                        n_a < a_first
                        or a_tiles[n_a] * 128 < (n_b + 1 + min(a_ahead, a0 + n_b)) * DH):
                    t = a_tiles[n_a]
                    if n_a < _OVR.get("NRAW", 3):
                        q[t] = q_tile(xb, mean, TILE_ORDER[t], t % 3 == 1)
                    else:
                        q[t] = q_tile(xcb, None, TILE_ORDER[t], t % 3 == 1)
                    n_a += 1
                jj = n_b // 2
                if n_b % 2 == 0:
                    s, mid[jj] = scores_first(slot, PAIR_ORDER[jj], q.pop(3 * jj), q.pop(3 * jj + 1))
                else:
                    s = scores_second(slot, PAIR_ORDER[jj], q.pop(3 * jj + 2), mid.pop(jj))
                p[n_b] = softmax(s, sc, defer=n_b < n_defer)
                n_b += 1
            h = 2 * PAIR_ORDER[i // 2] + i % 2
            pi = p.pop(i)
            if i < n_defer:
                pi, linv = pi
            dep = late.pop(i - tie, []) + ([done.pop(i - tie)] if i - tie in done else [])
            if dep:
                pi = jnp.where(never, _sum(dep), pi)
            pb = p_rows(pi)
            for rt in range(RT):
                v = vf_v[h * RT + rt] if h * RT + rt < NF else v_bf16(slot, h, rt)
                oc[i * RT + rt] = pv(v, pb) * linv if i < n_defer else pv(v, pb)
                if (i * RT + rt) % 16 == 15 and (i * RT + rt) // 16 in mt:
                    merge((i * RT + rt) // 16)
                while n_d < len(vg) - 16 * NVL and vg[n_d] + r_lag <= i * RT + rt:
                    dv(n_d)
                    n_d += 1
                while mt and mt[0] * 16 + 15 + m_lag <= i * RT + rt:
                    dm(mt.pop(0))
        while mt:
            dm(mt.pop(0))
        y = ym[0]
        tie = 0
        while n_d < len(vg):
            dv(n_d)
            n_d += 1
        return fold_rows(_sum([y] + [y for y in ys if y is not None]))

    def mod_block(x, z):
        wg, wu, wd, wgut, csg, csu = (r.at[z] for r in (wg_v, wu_v, wd_v, wgut_v, csg_v, csu_v))
        mean, xc, rstd = _ln_stats(x)
        xb = x.astype(bf16)
        mr = mean * rstd
        r = jnp.sum(x * wr, axis=1, keepdims=True) * rstd - mr * wr_sum
        nm = FF // 128 - NVH
        hid = []
        for t in range(nm):
            cols = blk(t, 128)
            g = jnp.dot(xb, wtile(wg, slice(None), cols), preferred_element_type=f32)
            u = jnp.dot(xb, wtile(wu, slice(None), cols), preferred_element_type=f32)
            g = g * rstd - mr * csg[:, cols]
            u = u * rstd - mr * csu[:, cols]
            hid.append((g * _sigmoid(g) * u).astype(bf16))
        for k in range(NVH):
            g = rows_dot(x, wgut, 2 * k) * rstd
            u = rows_dot(x, wgut, 2 * k + 1) * rstd
            hid.append(jnp.where((lane & 7) == row, g * _sigmoid(g) * u, 0.0).astype(bf16))
        ya = yb = None
        for t in range(FF // 128):
            d = jnp.dot(hid[t], wtile(wd, blk(t, 64), slice(None)), preferred_element_type=f32)
            if t < nm:
                ya = d if ya is None else d + ya
            else:
                yb = d if yb is None else d + yb
        y = ya + fold_rows(yb)
        return (x + xc * rstd) + y * _sigmoid(r)

    zero_s[0] = 0
    ones = jnp.ones((8, D), bf16)

    def colsum(w_v, cs_v, n):
        def body(t, carry):
            cols = blk(t, 512)
            cs_v[:, cols] = jnp.dot(ones, wtile(w_v, slice(None), cols), preferred_element_type=f32)
            return carry
        lax.fori_loop(0, n // 512, body, 0)

    for cp in w_cp[:3]:
        cp.wait()
    xf_v[0:B, :] = x_v[...].astype(f32)
    wr = wr_v[...].astype(f32).reshape(1, D)
    wr_sum = jnp.sum(wr, axis=1, keepdims=True)
    colsum(wq_v, csq_v, H * DH)

    def tile_order(t):
        return jnp.where(t < 3, t + (NT - 3), t - 3)

    def centered_transpose(w_v, cs_v, src, wt_v, dst):
        cols = blk(src, 128)
        mu = cs_v[0:1, cols] * (1.0 / D)
        for t in range(D // 128):
            w = wtile(w_v, blk(t, 64), cols).astype(f32) - mu
            wt_v[blk(dst, 128), blk(t, 128)] = w.T

    def prep_q(k, carry):
        centered_transpose(wq_v, csq_v, tile_order(QV0 + k), wqt_v, k)
        return carry

    lax.fori_loop(0, NQV, prep_q, 0)
    w_cp[3].wait()

    def unpack_wo(t, carry):
        pos = _sum([jnp.where(t == n, v, 0) for n, v in enumerate(VPU_TILES)])
        wof_v[0, blk(t, 128), :] = wtile(wo_v, blk(tile_order(pos), 64), slice(None)).astype(f32)
        return carry

    lax.fori_loop(0, NVT, unpack_wo, 0)
    w_cp[4].wait()
    colsum(wg_v.at[0], csg_v.at[0], FF)
    w_cp[5].wait()
    colsum(wu_v.at[0], csu_v.at[0], FF)

    def prep_gu(k, carry):
        src = FF // 128 - NVH + k
        centered_transpose(wg_v.at[0], csg_v.at[0], src, wgut_v.at[0], 2 * k)
        centered_transpose(wu_v.at[0], csu_v.at[0], src, wgut_v.at[0], 2 * k + 1)
        return carry

    lax.fori_loop(0, NVH, prep_gu, 0)
    w_cp[6].wait()

    def batch_body(b, carry):
        @pl.when(jnp.logical_and(b >= 1, b + NSLOT - 1 < B))
        def _():
            start_row(b + NSLOT - 1)

        x = jnp.broadcast_to(xf_v[pl.ds(b, 1), :], (8, D))
        z = zero_s[0]
        x = x + attn_streaming(x, b, z)
        with _scope("mod1"):
            x = mod_block(x, 0)
        never = lane < z
        if _OVR.get("FENCE", True):
            wgut_v[z, pl.ds(2 * NVH * 128, 8), pl.ds(0, 128)] = jnp.zeros((8, 128), f32)
            z = 0
        with _scope("attn2"):
            x = x + attn_resident(x, b, never)
        with _scope("mod2"):
            x = mod_block(x, z)
        xf_v[pl.ds(b, 1), :] = x[0:1, :]
        return carry

    lax.fori_loop(0, B, batch_body, 0)
    out_ref[...] = xf_v[0:B, :].astype(bf16)


def _tile_view(c):
    c = c.reshape(B, H, SK // 128, 128, RT, 8).transpose(0, 1, 4, 2, 5, 3)
    return c.reshape(B, NP, 2, SK // 128, 8, 128)


@jax.jit
def pallas_interleave_layers__sliding_block_cached__moe_arch_mod__decode_kernel(
    A_x: jax.Array,
    A_k_cache: jax.Array,
    A_v_cache: jax.Array,
    A_wq: jax.Array,
    A_wo: jax.Array,
    B_x: jax.Array,
    B_w_r: jax.Array,
    B_w_gate: jax.Array,
    B_w_up: jax.Array,
    B_w_down: jax.Array,
):
    del B_x
    out = pl.pallas_call(
        _kernel,
        out_shape=jax.ShapeDtypeStruct((B, D), bf16),
        in_specs=[pl.BlockSpec(memory_space=pl.ANY)] * 9,
        out_specs=pl.BlockSpec(memory_space=pltpu.VMEM),
        scratch_shapes=[
            pltpu.VMEM((B, D), bf16),
            pltpu.VMEM((D,), bf16),
            pltpu.VMEM((D // 2, H * DH + PADW), u32),
            pltpu.VMEM((H * DH // 2, D), u32),
            pltpu.VMEM((1, D // 2, FF + PADW), u32),
            pltpu.VMEM((1, D // 2, FF + PADW), u32),
            pltpu.VMEM((1, FF // 2, D), u32),
            pltpu.VMEM((NSLOT, NP, CT + PADK, 16, 128), bf16),
            pltpu.VMEM((NSLOT, NP, 2, CT, 8, 128), bf16),
            pltpu.VMEM((NF, CT * 8, 128), f32),
            pltpu.VMEM((1, NVT * 128, D), f32),
            pltpu.VMEM((1, 2 * NVH * 128 + 8, D), f32),
            pltpu.VMEM((max(NQV, 1) * 128, D), f32),
            pltpu.VMEM((8, H * DH), f32),
            pltpu.VMEM((1, 8, FF), f32),
            pltpu.VMEM((1, 8, FF), f32),
            pltpu.VMEM((8, D), f32),
            pltpu.VMEM((H, 8, 128), f32),
            pltpu.SMEM((1,), jnp.int32),
            pltpu.SemaphoreType.DMA((NW + B * SEMS_PER_ROW,)),
        ],
        compiler_params=pltpu.CompilerParams(vmem_limit_bytes=120 * 1024 * 1024,
                                             disable_semaphore_checks=True),
        name="fused_decode",
    )(A_x.reshape(B, D), B_w_r, _tile_view(A_k_cache), _tile_view(A_v_cache),
      A_wq, A_wo, B_w_gate, B_w_up, B_w_down)
    return out.reshape(B, 1, D)
```

```python
import contextlib
import functools

import jax
import jax.numpy as jnp
from jax import lax
import jax.experimental.pallas as pl
import jax.experimental.pallas.tpu as pltpu

f32, bf16, u32 = jnp.float32, jnp.bfloat16, jnp.uint32

try:
    _OVR
except NameError:
    _OVR = {}

B, D, H, DH, SK, FF = 4, 640, 32, 192, 4096, 1536
W = min(4096, max(256, SK // 4))
RT = DH // 8
CT = W // 128
NT = H * DH // 128
NP = H * RT // 2
LASTP = _OVR.get("LASTP", 2)
V_CHUNKS = ((0, 192, True), (192, 96, True), (288, 48, True), (336, 24, True), (360, 8, False),
            (368, 8, False), (376, 8 - LASTP, False), (384 - LASTP, LASTP, False))
NW = 7
SEMS_PER_ROW = 2 * (1 + len(V_CHUNKS))
NSLOT = 2
NF = H * RT - _OVR.get("NBF", 2 * LASTP)
QV0 = _OVR.get("QV0", 3)
NQV = _OVR.get("NQV", 8)
NVH = _OVR.get("NVH", 7)
PADW = _OVR.get("PADW", 128)
PADK = _OVR.get("PADK", 1)
SCALE = DH ** -0.5
LOG2E = 1.4426950408889634
EPS = 1e-5

_VT = _OVR.get("VT", "vvvm" * 9 + "vvv" + "m" * 6)
VPU_TILES = tuple(t for t in range(NT) if t >= NT - 3 or _VT[t % len(_VT)] == "v")
NVT = len(VPU_TILES)


def _scope(name):
    return jax.named_scope(name) if _OVR.get("SCOPES") else contextlib.nullcontext()


def _sum(xs):
    return functools.reduce(lambda a, c: a + c, xs)


def _sigmoid(x):
    return 0.5 * jnp.tanh(0.5 * x) + 0.5


def _ln_stats(x):
    m = jnp.sum(x, axis=1, keepdims=True) * (1.0 / D)
    if _OVR.get("ONEPASS", True):
        v = jnp.maximum(jnp.sum(x * x, axis=1, keepdims=True) * (1.0 / D) - m * m, 0.0)
        return m, x - m, lax.rsqrt(v + EPS)
    xc = x - m
    v = jnp.sum(xc * xc, axis=1, keepdims=True) * (1.0 / D)
    return m, xc, lax.rsqrt(v + EPS)


def _kernel(x_hbm, wr_hbm, k_hbm, v_hbm, wq_hbm, wo_hbm, wg_hbm, wu_hbm, wd_hbm,
            out_ref,
            x_v, wr_v, wq_v, wo_v, wg_v, wu_v, wd_v, k_v, v_v, vf_v, wof_v, wgut_v, wqt_v,
            csq_v, csg_v, csu_v, xf_v, p_v, zero_s, sems):
    w_src = (wq_hbm, x_hbm, wr_hbm, wo_hbm, wg_hbm, wu_hbm, wd_hbm)
    w_dst = (wq_v.at[:, pl.ds(0, H * DH)].bitcast(bf16), x_v, wr_v, wo_v.bitcast(bf16),
             wg_v.at[0, :, pl.ds(0, FF)].bitcast(bf16), wu_v.at[0, :, pl.ds(0, FF)].bitcast(bf16),
             wd_v.at[0].bitcast(bf16))
    w_cp = [pltpu.make_async_copy(s, d, sems.at[i]) for i, (s, d) in enumerate(zip(w_src, w_dst))]
    win = pl.ds((SK - W) // 128, CT)

    def k_copies(b):
        s0 = NW + b * SEMS_PER_ROW
        return [pltpu.make_async_copy(k_hbm.at[b, :, t, win],
                                      k_v.at[b % NSLOT, :, pl.ds(0, CT), pl.ds(8 * t, 8), :],
                                      sems.at[s0 + t]) for t in range(2)]

    def v_copies(b, c):
        p0, n, split = V_CHUNKS[c]
        rows = pl.ds(p0, n)
        s0 = NW + b * SEMS_PER_ROW + 2 * (1 + c)
        if split:
            return [pltpu.make_async_copy(v_hbm.at[b, rows, t, win], v_v.at[b % NSLOT, rows, t],
                                          sems.at[s0 + t]) for t in range(2)]
        return [pltpu.make_async_copy(v_hbm.at[b, rows, :, win], v_v.at[b % NSLOT, rows],
                                      sems.at[s0])]

    def start_row(b):
        for cp in k_copies(b):
            cp.start()
        for c in range(len(V_CHUNKS)):
            for cp in v_copies(b, c):
                cp.start()

    for cp in w_cp:
        cp.start()
    for b in range(NSLOT):
        start_row(b)

    lane = lax.broadcasted_iota(jnp.int32, (8, 128), 1)
    row = lax.broadcasted_iota(jnp.int32, (8, 128), 0)
    k32 = k_v.bitcast(u32)

    def wtile(ref, rows, cols):
        return pltpu.bitcast(ref[rows, cols], bf16)

    def blk(i, n):
        if isinstance(i, int):
            return pl.ds(i * n, n)
        return pl.ds(pl.multiple_of(i * n, n), n)

    def merge_tree(vals, idx):
        bit = 0
        while len(vals) > 1:
            odd = ((idx >> bit) & 1) == 1
            vals = [jnp.where(odd, vals[2 * i + 1], vals[2 * i]) for i in range(len(vals) // 2)]
            bit += 1
        return vals[0]

    def q_tile(xb, mean, tile, middle):
        cols = blk(tile, 128)
        q = jnp.dot(xb, wtile(wq_v, slice(None), cols), preferred_element_type=f32)
        return q_lhs(q if mean is None else q - mean * csq_v[:, cols], middle)

    def q_lhs(q, middle):
        if middle:
            q = jnp.concatenate([jnp.where(lane < 64, q, 0.0), jnp.where(lane >= 64, q, 0.0)], axis=0)
        return q.astype(bf16)

    def k_tile(slot, tile, c):
        w = k32[slot, blk(tile, 8), c]
        return pltpu.bitcast(w.reshape(64, 128), bf16)

    def scores_first(slot, j, q0, q1):
        ra, rb = [], []
        for c in range(CT):
            r1 = jnp.dot(q1, k_tile(slot, 3 * j + 1, c), preferred_element_type=f32)
            r0 = jnp.dot(q0, k_tile(slot, 3 * j, c), preferred_element_type=f32)
            ra.append(r0 + r1[0:8])
            rb.append(r1[8:16])
        return merge_tree(ra, row), merge_tree(rb, row)

    def scores_second(slot, j, q2, mid):
        r = [jnp.dot(q2, k_tile(slot, 3 * j + 2, c), preferred_element_type=f32) for c in range(CT)]
        return merge_tree(r, row) + mid

    def softmax(s, sc, defer=False):
        m = jnp.max(jnp.max(s, axis=1, keepdims=True), axis=0, keepdims=True)
        e = jnp.exp2((s - m) * sc)
        l = jnp.sum(jnp.sum(e, axis=1, keepdims=True), axis=0, keepdims=True)
        r = pl.reciprocal(l, approx=True)
        r = r * (2.0 - l * r)
        return (e, r) if defer else e * r

    def p_rows(p):
        return [jnp.broadcast_to(p[c:c + 1, :], (8, 128)) for c in range(CT)]

    def v_bf16(slot, h, rt):
        return v_v[slot, h * (RT // 2) + rt // 2, rt % 2].reshape(CT * 8, 128).astype(f32)

    def pv_lanes(v, pb):
        a = v[0:8] * pb[0]
        for c in range(1, CT):
            a = a + v[c * 8:(c + 1) * 8] * pb[c]
        return a

    def lane_sum(a):
        return jnp.broadcast_to(jnp.sum(a, axis=1, keepdims=True), (8, 128))

    def pv(v, pb):
        return lane_sum(pv_lanes(v, pb))

    def o_lhs(oc):
        o = merge_tree(oc, lane >> 3)
        return jnp.where((lane & 7) == row, o, 0.0).astype(bf16)

    def proj_mxu(lhs, tile):
        return jnp.dot(lhs, wtile(wo_v, blk(tile, 64), slice(None)), preferred_element_type=f32)

    def proj_vpu(oc, w):
        return w * jnp.concatenate([oc] * (D // 128), axis=1)

    def fold_rows(y):
        return jnp.broadcast_to(jnp.sum(y, axis=0, keepdims=True), y.shape)

    def rows_dot(x, wt_ref, tile):
        cols = []
        for i in range(16):
            w = wt_ref[pl.ds(tile * 128 + i * 8, 8), :] * x
            a = _sum([w[:, t * 128:(t + 1) * 128] for t in range(D // 128)])
            cols.append(jnp.broadcast_to(jnp.sum(a, axis=1, keepdims=True), (8, 128)))
        return merge_tree(cols, lane >> 3)

    def attn_streaming(x, b, z):
        slot = b % NSLOT
        mean, _, rstd = _ln_stats(x)
        xb = x.astype(bf16)
        sc = rstd * (SCALE * LOG2E)
        with _scope("wait_k"):
            for cp in k_copies(b):
                cp.wait()

        def scores(g, carry):
            q = [q_tile(xb, mean, 6 * g + i, i % 3 == 1) for i in range(6)]
            for i in range(2):
                j = 2 * g + i
                sa, mid = scores_first(slot, j, q[3 * i], q[3 * i + 1])
                sb = scores_second(slot, j, q[3 * i + 2], mid)
                p_v[2 * j] = softmax(sa, sc)
                p_v[2 * j + 1] = softmax(sb, sc)
            return carry

        with _scope("scores"):
            lax.fori_loop(0, H // 4, scores, 0)

        def head_pair(j, carry):
            y, prev = carry
            for c, (p0, _, _) in enumerate(V_CHUNKS[:-4]):
                @pl.when(j == p0 // RT)
                def _():
                    for cp in v_copies(b, c):
                        cp.wait()
            jp = jnp.maximum(j - 1, 0)
            y = y + _sum([proj_mxu(prev[i], 3 * jp + i) for i in range(3)])
            oc = []
            for i in range(2):
                h = 2 * j + i
                pb = p_rows(p_v[h])
                for rt in range(RT):
                    v = v_bf16(slot, h, rt)
                    vf_v[h * RT + rt] = v
                    oc.append(pv(v, pb))
            return y, tuple(o_lhs(oc[16 * i:16 * i + 16]) for i in range(3))

        with _scope("pv_loop"):
            y, prev = lax.fori_loop(
                0, H // 2 - 1, head_pair,
                (jnp.zeros((8, D), f32), (jnp.zeros((8, 128), bf16),) * 3))
        def wait_v(c):
            for cp in v_copies(b, len(V_CHUNKS) + c):
                cp.wait()

        def project(acc, n0, idx):
            ys = [None] * 3
            for n, a in enumerate(acc):
                d = proj_vpu(lane_sum(a), wof_v[idx, pl.ds(((NVT - 3) * 16 + n0 + n) * 8, 8), :])
                ys[n % 3] = d if ys[n % 3] is None else ys[n % 3] + d
            return ys

        pbs = [p_rows(p_v[H - 2]), p_rows(p_v[H - 1])]

        def lanes(n0, n1, sl):
            acc = []
            for n in range(n0, n1):
                v = v_bf16(sl, H - 2 + n // RT, n % RT)
                if (H - 2) * RT + n < NF:
                    vf_v[(H - 2) * RT + n] = v
                acc.append(pv_lanes(v, pbs[n // RT]))
            return acc

        wait_v(-4)
        y = y + _sum([proj_mxu(prev[i], NT - 6 + i) for i in range(3)])
        y = y + _sum(project(lanes(0, 16, slot), 0, 0))
        wait_v(-3)
        y = y + _sum(project(lanes(16, 32, slot), 16, 0))
        wait_v(-2)
        acc = lanes(32, 48 - 2 * LASTP, slot)
        with _scope("wait_last"):
            wait_v(-1)
        ys = project(acc + lanes(48 - 2 * LASTP, 48, slot + z), 32, z)
        return fold_rows((y + ys[1]) + (ys[2] + ys[0]))

    def attn_resident(x, b, never):
        a_ahead, a0, a_first = _OVR.get("A_AHEAD", 3), _OVR.get("A0", 2), _OVR.get("A_FIRST", 4)
        tie, n_defer = _OVR.get("TIE", 3), _OVR.get("DEFER", 4)
        slot = b % NSLOT
        mean, xc, rstd = _ln_stats(x)
        xb, xcb = x.astype(bf16), xc.astype(bf16)
        sc = rstd * (SCALE * LOG2E)
        q, e, linv = {}, {}, {}
        for k in range(NQV):
            qk = jnp.where((lane & 7) == row, rows_dot(x, wqt_v, k), 0.0)
            q[QV0 + k] = q_lhs(fold_rows(qk), (QV0 + k) % 3 == 1)
        a_tiles = [t for t in range(NT) if t not in q]
        n_a = 0
        for h in range(H):
            while n_a < len(a_tiles) and (
                    n_a < a_first or a_tiles[n_a] * 128 < (h + 1 + min(a_ahead, a0 + h)) * DH):
                t = a_tiles[n_a]
                if n_a < 3:
                    q[t] = q_tile(xb, mean, t, t % 3 == 1)
                else:
                    q[t] = q_tile(xcb, None, t, t % 3 == 1)
                n_a += 1
            j = h // 2
            if h % 2 == 0:
                s, mid = scores_first(slot, j, q.pop(3 * j), q.pop(3 * j + 1))
            else:
                s = scores_second(slot, j, q.pop(3 * j + 2), mid)
            e[h], linv[h] = softmax(s, sc, defer=True)
            if n_defer <= h < H - _OVR.get("DEFER_LAST", 2):
                e[h], linv[h] = e[h] * linv[h], None
        y, oc, merged, done = None, {}, {}, {}
        for h in range(H):
            if h - tie in done:
                e[h] = jnp.where(never, _sum(done[h - tie]), e[h])
            pb = p_rows(e[h])
            ys = [None, None, None if linv[h] is not None else y]
            for g in range(h * RT, (h + 1) * RT):
                o = pv(vf_v[g] if g < NF else v_bf16(slot, h, g % RT), pb)
                t = g // 16
                if t in VPU_TILES:
                    rows = pl.ds((VPU_TILES.index(t) * 16 + g % 16) * 8, 8)
                    d = proj_vpu(o, wof_v[0, rows, :])
                    ys[g % 3] = d if ys[g % 3] is None else ys[g % 3] + d
                else:
                    oc[g] = o
                    if g % 16 == 15:
                        m = merge_tree([oc.pop(16 * t + i) for i in range(16)], lane >> 3)
                        la, lb = linv[16 * t // RT], linv[h]
                        if la is not None and 16 * t // RT == h:
                            m = m * la
                        elif la is not None or lb is not None:
                            m = m * jnp.where(lane < 64, 1.0 if la is None else la,
                                              1.0 if lb is None else lb)
                        merged[t] = m
                        if _OVR.get("MTIE", 1):
                            done.setdefault(h, []).append(m)
            if ys[0] is not None:
                if linv[h] is None:
                    y = _sum(ys)
                else:
                    y = _sum(ys) * linv[h] if y is None else y + _sum(ys) * linv[h]
                done.setdefault(h, []).extend(y[:, t * 128:(t + 1) * 128] for t in range(D // 128))
        ym = None
        for t, m in merged.items():
            d = proj_mxu(jnp.where((lane & 7) == row, m, 0.0).astype(bf16), t)
            ym = d if ym is None else ym + d
        return fold_rows(ym + y)

    def mod_block(x, z):
        wg, wu, wd, wgut, csg, csu = (r.at[z] for r in (wg_v, wu_v, wd_v, wgut_v, csg_v, csu_v))
        mean, xc, rstd = _ln_stats(x)
        xb = x.astype(bf16)
        mr = mean * rstd
        r = jnp.sum(x * wr, axis=1, keepdims=True) * rstd - mr * wr_sum
        nm = FF // 128 - NVH
        hid = []
        for t in range(nm):
            cols = blk(t, 128)
            g = jnp.dot(xb, wtile(wg, slice(None), cols), preferred_element_type=f32)
            u = jnp.dot(xb, wtile(wu, slice(None), cols), preferred_element_type=f32)
            g = g * rstd - mr * csg[:, cols]
            u = u * rstd - mr * csu[:, cols]
            hid.append((g * _sigmoid(g) * u).astype(bf16))
        for k in range(NVH):
            g = rows_dot(x, wgut, 2 * k) * rstd
            u = rows_dot(x, wgut, 2 * k + 1) * rstd
            hid.append(jnp.where((lane & 7) == row, g * _sigmoid(g) * u, 0.0).astype(bf16))
        ya = yb = None
        for t in range(FF // 128):
            d = jnp.dot(hid[t], wtile(wd, blk(t, 64), slice(None)), preferred_element_type=f32)
            if t < nm:
                ya = d if ya is None else d + ya
            else:
                yb = d if yb is None else d + yb
        y = ya + fold_rows(yb)
        return (x + xc * rstd) + y * _sigmoid(r)

    zero_s[0] = 0
    ones = jnp.ones((8, D), bf16)

    def colsum(w_v, cs_v, n):
        def body(t, carry):
            cols = blk(t, 512)
            cs_v[:, cols] = jnp.dot(ones, wtile(w_v, slice(None), cols), preferred_element_type=f32)
            return carry
        lax.fori_loop(0, n // 512, body, 0)

    for cp in w_cp[:3]:
        cp.wait()
    xf_v[0:B, :] = x_v[...].astype(f32)
    wr = wr_v[...].astype(f32).reshape(1, D)
    wr_sum = jnp.sum(wr, axis=1, keepdims=True)
    colsum(wq_v, csq_v, H * DH)

    def centered_transpose(w_v, cs_v, src, wt_v, dst):
        cols = blk(src, 128)
        mu = cs_v[0:1, cols] * (1.0 / D)
        for t in range(D // 128):
            w = wtile(w_v, blk(t, 64), cols).astype(f32) - mu
            wt_v[blk(dst, 128), blk(t, 128)] = w.T

    def prep_q(k, carry):
        centered_transpose(wq_v, csq_v, QV0 + k, wqt_v, k)
        return carry

    lax.fori_loop(0, NQV, prep_q, 0)
    w_cp[3].wait()

    def unpack_wo(t, carry):
        pos = _sum([jnp.where(t == n, v, 0) for n, v in enumerate(VPU_TILES)])
        wof_v[0, blk(t, 128), :] = wtile(wo_v, blk(pos, 64), slice(None)).astype(f32)
        return carry

    lax.fori_loop(0, NVT, unpack_wo, 0)
    w_cp[4].wait()
    colsum(wg_v.at[0], csg_v.at[0], FF)
    w_cp[5].wait()
    colsum(wu_v.at[0], csu_v.at[0], FF)

    def prep_gu(k, carry):
        src = FF // 128 - NVH + k
        centered_transpose(wg_v.at[0], csg_v.at[0], src, wgut_v.at[0], 2 * k)
        centered_transpose(wu_v.at[0], csu_v.at[0], src, wgut_v.at[0], 2 * k + 1)
        return carry

    lax.fori_loop(0, NVH, prep_gu, 0)
    w_cp[6].wait()

    def batch_body(b, carry):
        @pl.when(jnp.logical_and(b >= 1, b + NSLOT - 1 < B))
        def _():
            start_row(b + NSLOT - 1)

        x = jnp.broadcast_to(xf_v[pl.ds(b, 1), :], (8, D))
        z = zero_s[0]
        x = x + attn_streaming(x, b, z)
        with _scope("mod1"):
            x = mod_block(x, 0)
        never = lane < z
        if _OVR.get("FENCE", True):
            wgut_v[z, pl.ds(2 * NVH * 128, 8), pl.ds(0, 128)] = jnp.zeros((8, 128), f32)
            z = 0
        with _scope("attn2"):
            x = x + attn_resident(x, b, never)
        with _scope("mod2"):
            x = mod_block(x, z)
        xf_v[pl.ds(b, 1), :] = x[0:1, :]
        return carry

    lax.fori_loop(0, B, batch_body, 0)
    out_ref[...] = xf_v[0:B, :].astype(bf16)


def _tile_view(c):
    c = c.reshape(B, H, SK // 128, 128, RT, 8).transpose(0, 1, 4, 2, 5, 3)
    return c.reshape(B, NP, 2, SK // 128, 8, 128)


@jax.jit
def pallas_interleave_layers__sliding_block_cached__moe_arch_mod__decode_kernel(
    A_x: jax.Array,
    A_k_cache: jax.Array,
    A_v_cache: jax.Array,
    A_wq: jax.Array,
    A_wo: jax.Array,
    B_x: jax.Array,
    B_w_r: jax.Array,
    B_w_gate: jax.Array,
    B_w_up: jax.Array,
    B_w_down: jax.Array,
):
    del B_x
    out = pl.pallas_call(
        _kernel,
        out_shape=jax.ShapeDtypeStruct((B, D), bf16),
        in_specs=[pl.BlockSpec(memory_space=pl.ANY)] * 9,
        out_specs=pl.BlockSpec(memory_space=pltpu.VMEM),
        scratch_shapes=[
            pltpu.VMEM((B, D), bf16),
            pltpu.VMEM((D,), bf16),
            pltpu.VMEM((D // 2, H * DH + PADW), u32),
            pltpu.VMEM((H * DH // 2, D), u32),
            pltpu.VMEM((1, D // 2, FF + PADW), u32),
            pltpu.VMEM((1, D // 2, FF + PADW), u32),
            pltpu.VMEM((1, FF // 2, D), u32),
            pltpu.VMEM((NSLOT, NP, CT + PADK, 16, 128), bf16),
            pltpu.VMEM((NSLOT, NP, 2, CT, 8, 128), bf16),
            pltpu.VMEM((NF, CT * 8, 128), f32),
            pltpu.VMEM((1, NVT * 128, D), f32),
            pltpu.VMEM((1, 2 * NVH * 128 + 8, D), f32),
            pltpu.VMEM((max(NQV, 1) * 128, D), f32),
            pltpu.VMEM((8, H * DH), f32),
            pltpu.VMEM((1, 8, FF), f32),
            pltpu.VMEM((1, 8, FF), f32),
            pltpu.VMEM((8, D), f32),
            pltpu.VMEM((H, 8, 128), f32),
            pltpu.SMEM((1,), jnp.int32),
            pltpu.SemaphoreType.DMA((NW + B * SEMS_PER_ROW,)),
        ],
        compiler_params=pltpu.CompilerParams(vmem_limit_bytes=120 * 1024 * 1024,
                                             disable_semaphore_checks=True),
        name="fused_decode",
    )(A_x.reshape(B, D), B_w_r, _tile_view(A_k_cache), _tile_view(A_v_cache),
      A_wq, A_wo, B_w_gate, B_w_up, B_w_down)
    return out.reshape(B, 1, D)
```

```python
import contextlib
import functools

import jax
import jax.numpy as jnp
from jax import lax
import jax.experimental.pallas as pl
import jax.experimental.pallas.tpu as pltpu

f32, bf16, u32 = jnp.float32, jnp.bfloat16, jnp.uint32

try:
    _OVR
except NameError:
    _OVR = {}

B, D, H, DH, SK, FF = 4, 640, 32, 192, 4096, 1536
W = min(4096, max(256, SK // 4))
RT = DH // 8
CT = W // 128
NT = H * DH // 128
NP = H * RT // 2
LASTP = _OVR.get("LASTP", 2)
V_CHUNKS = ((0, 192, True), (192, 96, True), (288, 48, True), (336, 24, True), (360, 8, False),
            (368, 8, False), (376, 8 - LASTP, False), (384 - LASTP, LASTP, False))
NW = 7
SEMS_PER_ROW = 2 * (1 + len(V_CHUNKS))
NSLOT = 2
NF = H * RT - _OVR.get("NBF", 2 * LASTP)
QV0 = _OVR.get("QV0", 3)
NQV = _OVR.get("NQV", 8)
NVH = _OVR.get("NVH", 7)
PADW = _OVR.get("PADW", 128)
PADK = _OVR.get("PADK", 1)
SCALE = DH ** -0.5
LOG2E = 1.4426950408889634
EPS = 1e-5

_VT = _OVR.get("VT", "vvvm" * 9 + "vvv" + "m" * 6)
VPU_TILES = tuple(t for t in range(NT) if t >= NT - 3 or _VT[t % len(_VT)] == "v")
NVT = len(VPU_TILES)


def _scope(name):
    return jax.named_scope(name) if _OVR.get("SCOPES") else contextlib.nullcontext()


def _sum(xs):
    return functools.reduce(lambda a, c: a + c, xs)


def _sigmoid(x):
    return 0.5 * jnp.tanh(0.5 * x) + 0.5


def _ln_stats(x):
    m = jnp.sum(x, axis=1, keepdims=True) * (1.0 / D)
    if _OVR.get("ONEPASS", True):
        v = jnp.maximum(jnp.sum(x * x, axis=1, keepdims=True) * (1.0 / D) - m * m, 0.0)
        return m, x - m, lax.rsqrt(v + EPS)
    xc = x - m
    v = jnp.sum(xc * xc, axis=1, keepdims=True) * (1.0 / D)
    return m, xc, lax.rsqrt(v + EPS)


def _kernel(x_hbm, wr_hbm, k_hbm, v_hbm, wq_hbm, wo_hbm, wg_hbm, wu_hbm, wd_hbm,
            out_ref,
            x_v, wr_v, wq_v, wo_v, wg_v, wu_v, wd_v, k_v, v_v, vf_v, wof_v, wgut_v, wqt_v,
            csq_v, csg_v, csu_v, xf_v, p_v, zero_s, sems):
    w_src = (wq_hbm, x_hbm, wr_hbm, wo_hbm, wg_hbm, wu_hbm, wd_hbm)
    w_dst = (wq_v.at[:, pl.ds(0, H * DH)].bitcast(bf16), x_v, wr_v, wo_v.bitcast(bf16),
             wg_v.at[0, :, pl.ds(0, FF)].bitcast(bf16), wu_v.at[0, :, pl.ds(0, FF)].bitcast(bf16),
             wd_v.at[0].bitcast(bf16))
    w_cp = [pltpu.make_async_copy(s, d, sems.at[i]) for i, (s, d) in enumerate(zip(w_src, w_dst))]
    win = pl.ds((SK - W) // 128, CT)

    def k_copies(b):
        s0 = NW + b * SEMS_PER_ROW
        return [pltpu.make_async_copy(k_hbm.at[b, :, t, win],
                                      k_v.at[b % NSLOT, :, pl.ds(0, CT), pl.ds(8 * t, 8), :],
                                      sems.at[s0 + t]) for t in range(2)]

    def v_copies(b, c):
        p0, n, split = V_CHUNKS[c]
        rows = pl.ds(p0, n)
        s0 = NW + b * SEMS_PER_ROW + 2 * (1 + c)
        if split:
            return [pltpu.make_async_copy(v_hbm.at[b, rows, t, win], v_v.at[b % NSLOT, rows, t],
                                          sems.at[s0 + t]) for t in range(2)]
        return [pltpu.make_async_copy(v_hbm.at[b, rows, :, win], v_v.at[b % NSLOT, rows],
                                      sems.at[s0])]

    def start_row(b):
        for cp in k_copies(b):
            cp.start()
        for c in range(len(V_CHUNKS)):
            for cp in v_copies(b, c):
                cp.start()

    for cp in w_cp:
        cp.start()
    for b in range(NSLOT):
        start_row(b)

    lane = lax.broadcasted_iota(jnp.int32, (8, 128), 1)
    row = lax.broadcasted_iota(jnp.int32, (8, 128), 0)
    k32 = k_v.bitcast(u32)

    def wtile(ref, rows, cols):
        return pltpu.bitcast(ref[rows, cols], bf16)

    def blk(i, n):
        if isinstance(i, int):
            return pl.ds(i * n, n)
        return pl.ds(pl.multiple_of(i * n, n), n)

    def merge_tree(vals, idx):
        bit = 0
        while len(vals) > 1:
            odd = ((idx >> bit) & 1) == 1
            vals = [jnp.where(odd, vals[2 * i + 1], vals[2 * i]) for i in range(len(vals) // 2)]
            bit += 1
        return vals[0]

    def q_tile(xb, mean, tile, middle):
        cols = blk(tile, 128)
        q = jnp.dot(xb, wtile(wq_v, slice(None), cols), preferred_element_type=f32)
        return q_lhs(q if mean is None else q - mean * csq_v[:, cols], middle)

    def q_lhs(q, middle):
        if middle:
            q = jnp.concatenate([jnp.where(lane < 64, q, 0.0), jnp.where(lane >= 64, q, 0.0)], axis=0)
        return q.astype(bf16)

    def k_tile(slot, tile, c):
        w = k32[slot, blk(tile, 8), c]
        return pltpu.bitcast(w.reshape(64, 128), bf16)

    def scores_first(slot, j, q0, q1):
        ra, rb = [], []
        for c in range(CT):
            r1 = jnp.dot(q1, k_tile(slot, 3 * j + 1, c), preferred_element_type=f32)
            r0 = jnp.dot(q0, k_tile(slot, 3 * j, c), preferred_element_type=f32)
            ra.append(r0 + r1[0:8])
            rb.append(r1[8:16])
        return merge_tree(ra, row), merge_tree(rb, row)

    def scores_second(slot, j, q2, mid):
        r = [jnp.dot(q2, k_tile(slot, 3 * j + 2, c), preferred_element_type=f32) for c in range(CT)]
        return merge_tree(r, row) + mid

    def softmax(s, sc, defer=False):
        m = jnp.max(jnp.max(s, axis=1, keepdims=True), axis=0, keepdims=True)
        e = jnp.exp2((s - m) * sc)
        l = jnp.sum(jnp.sum(e, axis=1, keepdims=True), axis=0, keepdims=True)
        r = pl.reciprocal(l, approx=True)
        r = r * (2.0 - l * r)
        return (e, r) if defer else e * r

    def p_rows(p):
        return [jnp.broadcast_to(p[c:c + 1, :], (8, 128)) for c in range(CT)]

    def v_bf16(slot, h, rt):
        return v_v[slot, h * (RT // 2) + rt // 2, rt % 2].reshape(CT * 8, 128).astype(f32)

    def pv_lanes(v, pb):
        a = v[0:8] * pb[0]
        for c in range(1, CT):
            a = a + v[c * 8:(c + 1) * 8] * pb[c]
        return a

    def lane_sum(a):
        return jnp.broadcast_to(jnp.sum(a, axis=1, keepdims=True), (8, 128))

    def pv(v, pb):
        return lane_sum(pv_lanes(v, pb))

    def o_lhs(oc):
        o = merge_tree(oc, lane >> 3)
        return jnp.where((lane & 7) == row, o, 0.0).astype(bf16)

    def proj_mxu(lhs, tile):
        return jnp.dot(lhs, wtile(wo_v, blk(tile, 64), slice(None)), preferred_element_type=f32)

    def proj_vpu(oc, w):
        return w * jnp.concatenate([oc] * (D // 128), axis=1)

    def fold_rows(y):
        return jnp.broadcast_to(jnp.sum(y, axis=0, keepdims=True), y.shape)

    def rows_dot(x, wt_ref, tile):
        cols = []
        for i in range(16):
            w = wt_ref[pl.ds(tile * 128 + i * 8, 8), :] * x
            a = _sum([w[:, t * 128:(t + 1) * 128] for t in range(D // 128)])
            cols.append(jnp.broadcast_to(jnp.sum(a, axis=1, keepdims=True), (8, 128)))
        return merge_tree(cols, lane >> 3)

    def attn_streaming(x, b, z):
        slot = b % NSLOT
        _, xc, rstd = _ln_stats(x)
        xcb = xc.astype(bf16)
        sc = rstd * (SCALE * LOG2E)
        with _scope("wait_k"):
            for cp in k_copies(b):
                cp.wait()

        def scores(g, carry):
            q = [q_tile(xcb, None, 6 * g + i, i % 3 == 1) for i in range(6)]
            for i in range(2):
                j = 2 * g + i
                sa, mid = scores_first(slot, j, q[3 * i], q[3 * i + 1])
                sb = scores_second(slot, j, q[3 * i + 2], mid)
                p_v[2 * j] = softmax(sa, sc)
                p_v[2 * j + 1] = softmax(sb, sc)
            return carry

        with _scope("scores"):
            lax.fori_loop(0, H // 4, scores, 0)

        def head_pair(j, carry):
            y, prev = carry
            for c, (p0, _, _) in enumerate(V_CHUNKS[:-4]):
                @pl.when(j == p0 // RT)
                def _():
                    for cp in v_copies(b, c):
                        cp.wait()
            jp = jnp.maximum(j - 1, 0)
            y = y + _sum([proj_mxu(prev[i], 3 * jp + i) for i in range(3)])
            oc = []
            for i in range(2):
                h = 2 * j + i
                pb = p_rows(p_v[h])
                for rt in range(RT):
                    v = v_bf16(slot, h, rt)
                    vf_v[h * RT + rt] = v
                    oc.append(pv(v, pb))
            return y, tuple(o_lhs(oc[16 * i:16 * i + 16]) for i in range(3))

        with _scope("pv_loop"):
            y, prev = lax.fori_loop(
                0, H // 2 - 1, head_pair,
                (jnp.zeros((8, D), f32), (jnp.zeros((8, 128), bf16),) * 3))
        def wait_v(c):
            for cp in v_copies(b, len(V_CHUNKS) + c):
                cp.wait()

        def project(acc, n0, idx):
            ys = [None] * 3
            for n, a in enumerate(acc):
                d = proj_vpu(lane_sum(a), wof_v[idx, pl.ds(((NVT - 3) * 16 + n0 + n) * 8, 8), :])
                ys[n % 3] = d if ys[n % 3] is None else ys[n % 3] + d
            return ys

        pbs = [p_rows(p_v[H - 2]), p_rows(p_v[H - 1])]

        def lanes(n0, n1, sl):
            acc = []
            for n in range(n0, n1):
                v = v_bf16(sl, H - 2 + n // RT, n % RT)
                if (H - 2) * RT + n < NF:
                    vf_v[(H - 2) * RT + n] = v
                acc.append(pv_lanes(v, pbs[n // RT]))
            return acc

        wait_v(-4)
        y = y + _sum([proj_mxu(prev[i], NT - 6 + i) for i in range(3)])
        y = y + _sum(project(lanes(0, 16, slot), 0, 0))
        wait_v(-3)
        y = y + _sum(project(lanes(16, 32, slot), 16, 0))
        wait_v(-2)
        acc = lanes(32, 48 - 2 * LASTP, slot)
        with _scope("wait_last"):
            wait_v(-1)
        ys = project(acc + lanes(48 - 2 * LASTP, 48, slot + z), 32, z)
        return fold_rows((y + ys[1]) + (ys[2] + ys[0]))

    def attn_resident(x, b, never):
        a_ahead, a0, a_first = _OVR.get("A_AHEAD", 3), _OVR.get("A0", 2), _OVR.get("A_FIRST", 4)
        tie, n_defer = _OVR.get("TIE", 3), _OVR.get("DEFER", 4)
        slot = b % NSLOT
        mean, xc, rstd = _ln_stats(x)
        xb, xcb = x.astype(bf16), xc.astype(bf16)
        sc = rstd * (SCALE * LOG2E)
        q, e, linv = {}, {}, {}
        for k in range(NQV):
            qk = jnp.where((lane & 7) == row, rows_dot(x, wqt_v, k), 0.0)
            q[QV0 + k] = q_lhs(fold_rows(qk), (QV0 + k) % 3 == 1)
        a_tiles = [t for t in range(NT) if t not in q]
        n_a = 0
        for h in range(H):
            while n_a < len(a_tiles) and (
                    n_a < a_first or a_tiles[n_a] * 128 < (h + 1 + min(a_ahead, a0 + h)) * DH):
                t = a_tiles[n_a]
                if n_a < 3:
                    q[t] = q_tile(xb, mean, t, t % 3 == 1)
                else:
                    q[t] = q_tile(xcb, None, t, t % 3 == 1)
                n_a += 1
            j = h // 2
            if h % 2 == 0:
                s, mid = scores_first(slot, j, q.pop(3 * j), q.pop(3 * j + 1))
            else:
                s = scores_second(slot, j, q.pop(3 * j + 2), mid)
            e[h], linv[h] = softmax(s, sc, defer=True)
            if n_defer <= h < H - _OVR.get("DEFER_LAST", 2):
                e[h], linv[h] = e[h] * linv[h], None
        y, oc, merged, done = None, {}, {}, {}
        for h in range(H):
            if h - tie in done:
                e[h] = jnp.where(never, _sum(done[h - tie]), e[h])
            pb = p_rows(e[h])
            ys = [None, None, None if linv[h] is not None else y]
            for g in range(h * RT, (h + 1) * RT):
                o = pv(vf_v[g] if g < NF else v_bf16(slot, h, g % RT), pb)
                t = g // 16
                if t in VPU_TILES:
                    rows = pl.ds((VPU_TILES.index(t) * 16 + g % 16) * 8, 8)
                    d = proj_vpu(o, wof_v[0, rows, :])
                    ys[g % 3] = d if ys[g % 3] is None else ys[g % 3] + d
                else:
                    oc[g] = o
                    if g % 16 == 15:
                        m = merge_tree([oc.pop(16 * t + i) for i in range(16)], lane >> 3)
                        la, lb = linv[16 * t // RT], linv[h]
                        if la is not None and 16 * t // RT == h:
                            m = m * la
                        elif la is not None or lb is not None:
                            m = m * jnp.where(lane < 64, 1.0 if la is None else la,
                                              1.0 if lb is None else lb)
                        merged[t] = m
                        if _OVR.get("MTIE", 1):
                            done.setdefault(h, []).append(m)
            if ys[0] is not None:
                if linv[h] is None:
                    y = _sum(ys)
                else:
                    y = _sum(ys) * linv[h] if y is None else y + _sum(ys) * linv[h]
                done.setdefault(h, []).extend(y[:, t * 128:(t + 1) * 128] for t in range(D // 128))
        ym = None
        for t, m in merged.items():
            d = proj_mxu(jnp.where((lane & 7) == row, m, 0.0).astype(bf16), t)
            ym = d if ym is None else ym + d
        return fold_rows(ym + y)

    def mod_block(x, z, shift=None):
        wg, wu, wd, wgut, csg, csu = (r.at[z] for r in (wg_v, wu_v, wd_v, wgut_v, csg_v, csu_v))
        mean, xc, rstd = _ln_stats(x)
        xb, xcb = x.astype(bf16), xc.astype(bf16)
        mr = mean * rstd
        r = jnp.sum(x * wr, axis=1, keepdims=True) * rstd - mr * wr_sum
        nm = FF // 128 - NVH
        hid = []
        for t in range(nm):
            cols = blk(t, 128)
            raw = t < _OVR.get("NRAWH", 2)
            lhs = xb if raw else xcb
            g = jnp.dot(lhs, wtile(wg, slice(None), cols), preferred_element_type=f32) * rstd
            u = jnp.dot(lhs, wtile(wu, slice(None), cols), preferred_element_type=f32) * rstd
            if raw:
                g = g - mr * csg[:, cols]
                u = u - mr * csu[:, cols]
            hid.append((g * _sigmoid(g) * u).astype(bf16))
        for k in range(NVH):
            g = rows_dot(x, wgut, 2 * k) * rstd
            u = rows_dot(x, wgut, 2 * k + 1) * rstd
            hid.append(jnp.where((lane & 7) == row, g * _sigmoid(g) * u, 0.0).astype(bf16))
        ya = yb = None
        for t in range(FF // 128):
            d = jnp.dot(hid[t], wtile(wd, blk(t, 64), slice(None)), preferred_element_type=f32)
            if t < nm:
                ya = d if ya is None else d + ya
            else:
                yb = d if yb is None else d + yb
        y = ya + fold_rows(yb)
        base = x + xc * rstd
        return (base if shift is None else base + shift) + y * _sigmoid(r)

    zero_s[0] = 0
    ones = jnp.ones((8, D), bf16)

    def colsum(w_v, cs_v, n):
        def body(t, carry):
            cols = blk(t, 512)
            cs_v[:, cols] = jnp.dot(ones, wtile(w_v, slice(None), cols), preferred_element_type=f32)
            return carry
        lax.fori_loop(0, n // 512, body, 0)

    for cp in w_cp[:3]:
        cp.wait()
    xf_v[0:B, :] = x_v[...].astype(f32)
    wr = wr_v[...].astype(f32).reshape(1, D)
    wr_sum = jnp.sum(wr, axis=1, keepdims=True)
    colsum(wq_v, csq_v, H * DH)

    def centered_transpose(w_v, cs_v, src, wt_v, dst):
        cols = blk(src, 128)
        mu = cs_v[0:1, cols] * (1.0 / D)
        for t in range(D // 128):
            w = wtile(w_v, blk(t, 64), cols).astype(f32) - mu
            wt_v[blk(dst, 128), blk(t, 128)] = w.T

    def prep_q(k, carry):
        centered_transpose(wq_v, csq_v, QV0 + k, wqt_v, k)
        return carry

    lax.fori_loop(0, NQV, prep_q, 0)
    w_cp[3].wait()

    def unpack_wo(t, carry):
        pos = _sum([jnp.where(t == n, v, 0) for n, v in enumerate(VPU_TILES)])
        wof_v[0, blk(t, 128), :] = wtile(wo_v, blk(pos, 64), slice(None)).astype(f32)
        return carry

    lax.fori_loop(0, NVT, unpack_wo, 0)
    w_cp[4].wait()
    colsum(wg_v.at[0], csg_v.at[0], FF)
    w_cp[5].wait()
    colsum(wu_v.at[0], csu_v.at[0], FF)

    def prep_gu(k, carry):
        src = FF // 128 - NVH + k
        centered_transpose(wg_v.at[0], csg_v.at[0], src, wgut_v.at[0], 2 * k)
        centered_transpose(wu_v.at[0], csu_v.at[0], src, wgut_v.at[0], 2 * k + 1)
        return carry

    lax.fori_loop(0, NVH, prep_gu, 0)
    w_cp[6].wait()

    def batch_body(b, carry):
        @pl.when(jnp.logical_and(b >= 1, b + NSLOT - 1 < B))
        def _():
            start_row(b + NSLOT - 1)

        x = jnp.broadcast_to(xf_v[pl.ds(b, 1), :], (8, D))
        shift = jnp.sum(x, axis=1, keepdims=True) * (1.0 / D)
        x = x - shift
        z = zero_s[0]
        x = x + attn_streaming(x, b, z)
        with _scope("mod1"):
            x = mod_block(x, 0)
        never = lane < z
        if _OVR.get("FENCE", True):
            wgut_v[z, pl.ds(2 * NVH * 128, 8), pl.ds(0, 128)] = jnp.zeros((8, 128), f32)
            z = 0
        with _scope("attn2"):
            x = x + attn_resident(x, b, never)
        with _scope("mod2"):
            x = mod_block(x, z, shift)
        xf_v[pl.ds(b, 1), :] = x[0:1, :]
        return carry

    lax.fori_loop(0, B, batch_body, 0)
    out_ref[...] = xf_v[0:B, :].astype(bf16)


def _tile_view(c):
    c = c.reshape(B, H, SK // 128, 128, RT, 8).transpose(0, 1, 4, 2, 5, 3)
    return c.reshape(B, NP, 2, SK // 128, 8, 128)


@jax.jit
def pallas_interleave_layers__sliding_block_cached__moe_arch_mod__decode_kernel(
    A_x: jax.Array,
    A_k_cache: jax.Array,
    A_v_cache: jax.Array,
    A_wq: jax.Array,
    A_wo: jax.Array,
    B_x: jax.Array,
    B_w_r: jax.Array,
    B_w_gate: jax.Array,
    B_w_up: jax.Array,
    B_w_down: jax.Array,
):
    del B_x
    out = pl.pallas_call(
        _kernel,
        out_shape=jax.ShapeDtypeStruct((B, D), bf16),
        in_specs=[pl.BlockSpec(memory_space=pl.ANY)] * 9,
        out_specs=pl.BlockSpec(memory_space=pltpu.VMEM),
        scratch_shapes=[
            pltpu.VMEM((B, D), bf16),
            pltpu.VMEM((D,), bf16),
            pltpu.VMEM((D // 2, H * DH + PADW), u32),
            pltpu.VMEM((H * DH // 2, D), u32),
            pltpu.VMEM((1, D // 2, FF + PADW), u32),
            pltpu.VMEM((1, D // 2, FF + PADW), u32),
            pltpu.VMEM((1, FF // 2, D), u32),
            pltpu.VMEM((NSLOT, NP, CT + PADK, 16, 128), bf16),
            pltpu.VMEM((NSLOT, NP, 2, CT, 8, 128), bf16),
            pltpu.VMEM((NF, CT * 8, 128), f32),
            pltpu.VMEM((1, NVT * 128, D), f32),
            pltpu.VMEM((1, 2 * NVH * 128 + 8, D), f32),
            pltpu.VMEM((max(NQV, 1) * 128, D), f32),
            pltpu.VMEM((8, H * DH), f32),
            pltpu.VMEM((1, 8, FF), f32),
            pltpu.VMEM((1, 8, FF), f32),
            pltpu.VMEM((8, D), f32),
            pltpu.VMEM((H, 8, 128), f32),
            pltpu.SMEM((1,), jnp.int32),
            pltpu.SemaphoreType.DMA((NW + B * SEMS_PER_ROW,)),
        ],
        compiler_params=pltpu.CompilerParams(vmem_limit_bytes=120 * 1024 * 1024,
                                             disable_semaphore_checks=True,
                                             disable_bounds_checks=_OVR.get("NOBC", False)),
        name="fused_decode",
    )(A_x.reshape(B, D), B_w_r, _tile_view(A_k_cache), _tile_view(A_v_cache),
      A_wq, A_wo, B_w_gate, B_w_up, B_w_down)
    return out.reshape(B, 1, D)
```

```python
import contextlib
import functools

import jax
import jax.numpy as jnp
from jax import lax
import jax.experimental.pallas as pl
import jax.experimental.pallas.tpu as pltpu

f32, bf16, u32 = jnp.float32, jnp.bfloat16, jnp.uint32

try:
    _OVR
except NameError:
    _OVR = {}

B, D, H, DH, SK, FF = 4, 640, 32, 192, 4096, 1536
W = min(4096, max(256, SK // 4))
RT = DH // 8
CT = W // 128
NT = H * DH // 128
NP = H * RT // 2
LASTP = _OVR.get("LASTP", 2)
V_CHUNKS = ((0, 192, True), (192, 96, True), (288, 48, True), (336, 24, True), (360, 8, False),
            (368, 8, False), (376, 8 - LASTP, False), (384 - LASTP, LASTP, False))
NW = 7
SEMS_PER_ROW = 2 * (1 + len(V_CHUNKS))
NF = H * RT - _OVR.get("NBF", 2 * LASTP)
QV0 = _OVR.get("QV0", 3)
NQV = _OVR.get("NQV", 8)
NVH = _OVR.get("NVH", 7)
NMH = FF // 128 - NVH
SCALE = DH ** -0.5
LOG2E = 1.4426950408889634
EPS = 1e-5

_VT = _OVR.get("VT", "vvvm" * 9 + "vvv" + "m" * 6)
VPU_TILES = tuple(t for t in range(NT) if t >= NT - 3 or _VT[t % len(_VT)] == "v")
MXU_TILES = tuple(t for t in range(NT) if t not in VPU_TILES)
NVT = len(VPU_TILES)


def _scope(name):
    return jax.named_scope(name) if _OVR.get("SCOPES") else contextlib.nullcontext()


def _sum(xs):
    return functools.reduce(lambda a, c: a + c, xs)


def _sigmoid(x):
    return 0.5 * jnp.tanh(0.5 * x) + 0.5


def _ln_stats(x):
    m = jnp.sum(x, axis=1, keepdims=True) * (1.0 / D)
    if _OVR.get("ONEPASS", True):
        v = jnp.maximum(jnp.sum(x * x, axis=1, keepdims=True) * (1.0 / D) - m * m, 0.0)
        return m, x - m, lax.rsqrt(v + EPS)
    xc = x - m
    v = jnp.sum(xc * xc, axis=1, keepdims=True) * (1.0 / D)
    return m, xc, lax.rsqrt(v + EPS)


def _kernel(x_hbm, wr_hbm, k_hbm, v_hbm, wq_hbm, wo_hbm, wg_hbm, wu_hbm, wd_hbm,
            out_ref,
            x_v, wr_v, wq_v, wo_v, wg_v, wu_v, wd_v, k_v, v_v,
            wqm_v, wom_v, wgum_v, wdm_v, km_v,
            vf_v, wof_v, wgut_v, wqt_v,
            csq_v, csg_v, csu_v, xf_v, p_v, zero_s, sems):
    w_src = (wq_hbm, x_hbm, wr_hbm, wo_hbm, wg_hbm, wu_hbm, wd_hbm)
    w_dst = (wq_v, x_v, wr_v, wo_v, wg_v, wu_v, wd_v)
    w_cp = [pltpu.make_async_copy(s, d, sems.at[i]) for i, (s, d) in enumerate(zip(w_src, w_dst))]
    win = pl.ds((SK - W) // 128, CT)

    def k_copies(b):
        s0 = NW + b * SEMS_PER_ROW
        return [pltpu.make_async_copy(k_hbm.at[b, :, t, win], k_v.at[:, t], sems.at[s0 + t])
                for t in range(2)]

    def v_copies(b, c):
        p0, n, split = V_CHUNKS[c]
        rows = pl.ds(p0, n)
        s0 = NW + b * SEMS_PER_ROW + 2 * (1 + c)
        if split:
            return [pltpu.make_async_copy(v_hbm.at[b, rows, t, win], v_v.at[0, rows, t],
                                          sems.at[s0 + t]) for t in range(2)]
        return [pltpu.make_async_copy(v_hbm.at[b, rows, :, win], v_v.at[0, rows], sems.at[s0])]

    def start_k(b):
        for cp in k_copies(b):
            cp.start()

    def start_v(b):
        for c in range(len(V_CHUNKS)):
            for cp in v_copies(b, c):
                cp.start()

    for cp in w_cp:
        cp.start()
    start_k(0)
    start_v(0)

    lane = lax.broadcasted_iota(jnp.int32, (8, 128), 1)
    row = lax.broadcasted_iota(jnp.int32, (8, 128), 0)

    def pack(w):
        return pltpu.bitcast(w, u32)

    def unpack(w):
        return pltpu.bitcast(w, bf16)

    def blk(i, n):
        if isinstance(i, int):
            return pl.ds(i * n, n)
        return pl.ds(pl.multiple_of(i * n, n), n)

    def merge_tree(vals, idx):
        bit = 0
        while len(vals) > 1:
            odd = ((idx >> bit) & 1) == 1
            vals = [jnp.where(odd, vals[2 * i + 1], vals[2 * i]) for i in range(len(vals) // 2)]
            bit += 1
        return vals[0]

    def q_lhs(q, middle):
        if middle:
            q = jnp.concatenate([jnp.where(lane < 64, q, 0.0), jnp.where(lane >= 64, q, 0.0)], axis=0)
        return q.astype(bf16)

    def scores_first(k_tile, j, q0, q1):
        ra, rb = [], []
        for c in range(CT):
            r1 = jnp.dot(q1, k_tile(3 * j + 1, c), preferred_element_type=f32)
            r0 = jnp.dot(q0, k_tile(3 * j, c), preferred_element_type=f32)
            ra.append(r0 + r1[0:8])
            rb.append(r1[8:16])
        return merge_tree(ra, row), merge_tree(rb, row)

    def scores_second(k_tile, j, q2, mid):
        r = [jnp.dot(q2, k_tile(3 * j + 2, c), preferred_element_type=f32) for c in range(CT)]
        return merge_tree(r, row) + mid

    def softmax(s, sc, defer=False):
        m = jnp.max(jnp.max(s, axis=1, keepdims=True), axis=0, keepdims=True)
        e = jnp.exp2((s - m) * sc)
        l = jnp.sum(jnp.sum(e, axis=1, keepdims=True), axis=0, keepdims=True)
        r = pl.reciprocal(l, approx=True)
        r = r * (2.0 - l * r)
        return (e, r) if defer else e * r

    def p_rows(p):
        return [jnp.broadcast_to(p[c:c + 1, :], (8, 128)) for c in range(CT)]

    def v_bf16(slot, h, rt):
        return v_v[slot, h * (RT // 2) + rt // 2, rt % 2].reshape(CT * 8, 128).astype(f32)

    def pv_lanes(v, pb):
        a = v[0:8] * pb[0]
        for c in range(1, CT):
            a = a + v[c * 8:(c + 1) * 8] * pb[c]
        return a

    def lane_sum(a):
        return jnp.broadcast_to(jnp.sum(a, axis=1, keepdims=True), (8, 128))

    def pv(v, pb):
        return lane_sum(pv_lanes(v, pb))

    def o_lhs(oc):
        o = merge_tree(oc, lane >> 3)
        return jnp.where((lane & 7) == row, o, 0.0).astype(bf16)

    def proj_vpu(oc, w):
        return w * jnp.concatenate([oc] * (D // 128), axis=1)

    def fold_rows(y):
        return jnp.broadcast_to(jnp.sum(y, axis=0, keepdims=True), y.shape)

    def rows_dot(x, wt_ref, tile):
        cols = []
        for i in range(16):
            w = wt_ref[pl.ds(tile * 128 + i * 8, 8), :] * x
            a = _sum([w[:, t * 128:(t + 1) * 128] for t in range(D // 128)])
            cols.append(jnp.broadcast_to(jnp.sum(a, axis=1, keepdims=True), (8, 128)))
        return merge_tree(cols, lane >> 3)

    def attn_streaming(x, b, z):
        _, xc, rstd = _ln_stats(x)
        xcb = xc.astype(bf16)
        sc = rstd * (SCALE * LOG2E)
        with _scope("wait_k"):
            for cp in k_copies(b):
                cp.wait()

        def k_tile(tile, c):
            w = pack(k_v[blk(tile, 8), :, c].reshape(128, 128))
            km_v[tile, c] = w
            return unpack(w)

        def scores(g, carry):
            q = [jnp.dot(xcb, wq_v[:, blk(6 * g + i, 128)], preferred_element_type=f32)
                 for i in range(6)]
            q = [q_lhs(q[i], i % 3 == 1) for i in range(6)]
            for i in range(2):
                j = 2 * g + i
                sa, mid = scores_first(k_tile, j, q[3 * i], q[3 * i + 1])
                sb = scores_second(k_tile, j, q[3 * i + 2], mid)
                p_v[2 * j] = softmax(sa, sc)
                p_v[2 * j + 1] = softmax(sb, sc)
            return carry

        with _scope("scores"):
            lax.fori_loop(0, H // 4, scores, 0)

        @pl.when(b + 1 < B)
        def _():
            start_k(b + 1)

        def proj_mxu(lhs, tile):
            return jnp.dot(lhs, wo_v[blk(tile, 128), :], preferred_element_type=f32)

        def head_pair(j, carry):
            y, prev = carry
            for c, (p0, _, _) in enumerate(V_CHUNKS[:-4]):
                @pl.when(j == p0 // RT)
                def _():
                    for cp in v_copies(b, c):
                        cp.wait()
            jp = jnp.maximum(j - 1, 0)
            y = y + _sum([proj_mxu(prev[i], 3 * jp + i) for i in range(3)])
            oc = []
            for i in range(2):
                h = 2 * j + i
                pb = p_rows(p_v[h])
                for rt in range(RT):
                    v = v_bf16(0, h, rt)
                    vf_v[h * RT + rt] = v
                    oc.append(pv(v, pb))
            return y, tuple(o_lhs(oc[16 * i:16 * i + 16]) for i in range(3))

        with _scope("pv_loop"):
            y, prev = lax.fori_loop(
                0, H // 2 - 1, head_pair,
                (jnp.zeros((8, D), f32), (jnp.zeros((8, 128), bf16),) * 3))
        def wait_v(c):
            for cp in v_copies(b, len(V_CHUNKS) + c):
                cp.wait()

        def project(acc, n0, idx):
            ys = [None] * 3
            for n, a in enumerate(acc):
                d = proj_vpu(lane_sum(a), wof_v[idx, pl.ds(((NVT - 3) * 16 + n0 + n) * 8, 8), :])
                ys[n % 3] = d if ys[n % 3] is None else ys[n % 3] + d
            return ys

        pbs = [p_rows(p_v[H - 2]), p_rows(p_v[H - 1])]

        def lanes(n0, n1, sl):
            acc = []
            for n in range(n0, n1):
                v = v_bf16(sl, H - 2 + n // RT, n % RT)
                if (H - 2) * RT + n < NF:
                    vf_v[(H - 2) * RT + n] = v
                acc.append(pv_lanes(v, pbs[n // RT]))
            return acc

        wait_v(-4)
        y = y + _sum([proj_mxu(prev[i], NT - 6 + i) for i in range(3)])
        y = y + _sum(project(lanes(0, 16, 0), 0, 0))
        wait_v(-3)
        y = y + _sum(project(lanes(16, 32, 0), 16, 0))
        wait_v(-2)
        acc = lanes(32, 48 - 2 * LASTP, 0)
        with _scope("wait_last"):
            wait_v(-1)
        ys = project(acc + lanes(48 - 2 * LASTP, 48, z), 32, z)
        return fold_rows((y + ys[1]) + (ys[2] + ys[0]))

    def attn_resident(x, never):
        a_ahead, a0, a_first = _OVR.get("A_AHEAD", 3), _OVR.get("A0", 2), _OVR.get("A_FIRST", 4)
        tie, n_defer = _OVR.get("TIE", 3), _OVR.get("DEFER", 4)
        mean, xc, rstd = _ln_stats(x)
        xb, xcb = x.astype(bf16), xc.astype(bf16)
        sc = rstd * (SCALE * LOG2E)
        q, e, linv = {}, {}, {}
        for k in range(NQV):
            qk = jnp.where((lane & 7) == row, rows_dot(x, wqt_v, k), 0.0)
            q[QV0 + k] = q_lhs(fold_rows(qk), (QV0 + k) % 3 == 1)
        a_tiles = [t for t in range(NT) if t not in q]
        n_a = 0

        def k_tile(tile, c):
            return unpack(km_v[tile, c])

        for h in range(H):
            while n_a < len(a_tiles) and (
                    n_a < a_first or a_tiles[n_a] * 128 < (h + 1 + min(a_ahead, a0 + h)) * DH):
                t = a_tiles[n_a]
                raw = n_a < 3
                qt = jnp.dot(xb if raw else xcb, unpack(wqm_v[n_a]), preferred_element_type=f32)
                q[t] = q_lhs(qt - mean * csq_v[:, blk(t, 128)] if raw else qt, t % 3 == 1)
                n_a += 1
            j = h // 2
            if h % 2 == 0:
                s, mid = scores_first(k_tile, j, q.pop(3 * j), q.pop(3 * j + 1))
            else:
                s = scores_second(k_tile, j, q.pop(3 * j + 2), mid)
            e[h], linv[h] = softmax(s, sc, defer=True)
            if n_defer <= h < H - _OVR.get("DEFER_LAST", 2):
                e[h], linv[h] = e[h] * linv[h], None
        y, oc, merged, done = None, {}, {}, {}
        for h in range(H):
            if h - tie in done:
                e[h] = jnp.where(never, _sum(done[h - tie]), e[h])
            pb = p_rows(e[h])
            ys = [None, None, None if linv[h] is not None else y]
            for g in range(h * RT, (h + 1) * RT):
                o = pv(vf_v[g] if g < NF else v_bf16(0, h, g % RT), pb)
                t = g // 16
                if t in VPU_TILES:
                    rows = pl.ds((VPU_TILES.index(t) * 16 + g % 16) * 8, 8)
                    d = proj_vpu(o, wof_v[0, rows, :])
                    ys[g % 3] = d if ys[g % 3] is None else ys[g % 3] + d
                else:
                    oc[g] = o
                    if g % 16 == 15:
                        m = merge_tree([oc.pop(16 * t + i) for i in range(16)], lane >> 3)
                        la, lb = linv[16 * t // RT], linv[h]
                        if la is not None and 16 * t // RT == h:
                            m = m * la
                        elif la is not None or lb is not None:
                            m = m * jnp.where(lane < 64, 1.0 if la is None else la,
                                              1.0 if lb is None else lb)
                        merged[t] = m
                        if _OVR.get("MTIE", 1):
                            done.setdefault(h, []).append(m)
            if ys[0] is not None:
                if linv[h] is None:
                    y = _sum(ys)
                else:
                    y = _sum(ys) * linv[h] if y is None else y + _sum(ys) * linv[h]
                done.setdefault(h, []).extend(y[:, t * 128:(t + 1) * 128] for t in range(D // 128))
        ym = None
        for t, m in merged.items():
            d = jnp.dot(jnp.where((lane & 7) == row, m, 0.0).astype(bf16),
                        unpack(wom_v[MXU_TILES.index(t)]), preferred_element_type=f32)
            ym = d if ym is None else ym + d
        return fold_rows(ym + y)

    def mod_block(x, shift=None):
        mean, xc, rstd = _ln_stats(x)
        xb, xcb = x.astype(bf16), xc.astype(bf16)
        mr = mean * rstd
        r = jnp.sum(x * wr, axis=1, keepdims=True) * rstd - mr * wr_sum
        hid = []
        for t in range(NMH):
            cols = blk(t, 128)
            raw = t < _OVR.get("NRAWH", 2)
            lhs = xb if raw else xcb
            g = jnp.dot(lhs, unpack(wgum_v[2 * t]), preferred_element_type=f32) * rstd
            u = jnp.dot(lhs, unpack(wgum_v[2 * t + 1]), preferred_element_type=f32) * rstd
            if raw:
                g = g - mr * csg_v[:, cols]
                u = u - mr * csu_v[:, cols]
            hid.append((g * _sigmoid(g) * u).astype(bf16))
        for k in range(NVH):
            g = rows_dot(x, wgut_v.at[0], 2 * k) * rstd
            u = rows_dot(x, wgut_v.at[0], 2 * k + 1) * rstd
            hid.append(jnp.where((lane & 7) == row, g * _sigmoid(g) * u, 0.0).astype(bf16))
        ya = yb = None
        for t in range(FF // 128):
            d = jnp.dot(hid[t], unpack(wdm_v[t]), preferred_element_type=f32)
            if t < NMH:
                ya = d if ya is None else d + ya
            else:
                yb = d if yb is None else d + yb
        y = ya + fold_rows(yb)
        base = x + xc * rstd
        return (base if shift is None else base + shift) + y * _sigmoid(r)

    zero_s[0] = 0
    ones = jnp.ones((8, D), bf16)

    def loop(n, body):
        def step(i, carry):
            body(i)
            return carry
        lax.fori_loop(0, n, step, 0)

    def pick(i, table):
        return _sum([jnp.where(i == n, v, 0) for n, v in enumerate(table)])

    def colsum(w_v, cs_v):
        def body(t):
            cs_v[:, blk(t, 512)] = jnp.dot(ones, w_v[:, blk(t, 512)], preferred_element_type=f32)
        loop(cs_v.shape[1] // 512, body)

    def centered_transpose(w_v, cs_v, src, wt_v, dst):
        cols = blk(src, 128)
        mu = cs_v[0:1, cols] * (1.0 / D)
        for t in range(D // 128):
            wt_v[blk(dst, 128), blk(t, 128)] = (w_v[blk(t, 128), cols].astype(f32) - mu).T

    for cp in w_cp[:3]:
        cp.wait()
    xf_v[0:B, :] = x_v[...].astype(f32)
    wr = wr_v[...].astype(f32).reshape(1, D)
    wr_sum = jnp.sum(wr, axis=1, keepdims=True)
    colsum(wq_v, csq_v)
    loop(NQV, lambda k: centered_transpose(wq_v, csq_v, QV0 + k, wqt_v, k))

    def prep_wq(n):
        wqm_v[n] = pack(wq_v[:, blk(jnp.where(n < QV0, n, n + NQV), 128)])

    loop(NT - NQV, prep_wq)
    w_cp[3].wait()

    def prep_wof(n):
        wof_v[0, blk(n, 128), :] = wo_v[blk(pick(n, VPU_TILES), 128), :].astype(f32)

    def prep_wom(n):
        wom_v[n] = pack(wo_v[blk(pick(n, MXU_TILES), 128), :])

    loop(NVT, prep_wof)
    loop(NT - NVT, prep_wom)
    w_cp[4].wait()
    w_cp[5].wait()
    colsum(wg_v, csg_v)
    colsum(wu_v, csu_v)

    def prep_gum(t):
        wgum_v[2 * t] = pack(wg_v[:, blk(t, 128)])
        wgum_v[2 * t + 1] = pack(wu_v[:, blk(t, 128)])

    def prep_gut(k):
        centered_transpose(wg_v, csg_v, NMH + k, wgut_v.at[0], 2 * k)
        centered_transpose(wu_v, csu_v, NMH + k, wgut_v.at[0], 2 * k + 1)

    def prep_wd(t):
        wdm_v[t] = pack(wd_v[blk(t, 128), :])

    loop(NMH, prep_gum)
    loop(NVH, prep_gut)
    w_cp[6].wait()
    loop(FF // 128, prep_wd)

    def batch_body(b):
        @pl.when(b >= 1)
        def _():
            start_v(b)

        x = jnp.broadcast_to(xf_v[pl.ds(b, 1), :], (8, D))
        shift = jnp.sum(x, axis=1, keepdims=True) * (1.0 / D)
        x = x - shift
        z = zero_s[0]
        x = x + attn_streaming(x, b, z)
        with _scope("mod1"):
            x = mod_block(x)
        wgut_v[z, pl.ds(2 * NVH * 128, 8), pl.ds(0, 128)] = jnp.zeros((8, 128), f32)
        with _scope("attn2"):
            x = x + attn_resident(x, lane < z)
        with _scope("mod2"):
            x = mod_block(x, shift)
        xf_v[pl.ds(b, 1), :] = x[0:1, :]

    loop(B, batch_body)
    out_ref[...] = xf_v[0:B, :].astype(bf16)


def _tile_view(c):
    c = c.reshape(B, H, SK // 128, 128, RT, 8).transpose(0, 1, 4, 2, 5, 3)
    return c.reshape(B, NP, 2, SK // 128, 8, 128)


@jax.jit
def pallas_interleave_layers__sliding_block_cached__moe_arch_mod__decode_kernel(
    A_x: jax.Array,
    A_k_cache: jax.Array,
    A_v_cache: jax.Array,
    A_wq: jax.Array,
    A_wo: jax.Array,
    B_x: jax.Array,
    B_w_r: jax.Array,
    B_w_gate: jax.Array,
    B_w_up: jax.Array,
    B_w_down: jax.Array,
):
    del B_x
    out = pl.pallas_call(
        _kernel,
        out_shape=jax.ShapeDtypeStruct((B, D), bf16),
        in_specs=[pl.BlockSpec(memory_space=pl.ANY)] * 9,
        out_specs=pl.BlockSpec(memory_space=pltpu.VMEM),
        scratch_shapes=[
            pltpu.VMEM((B, D), bf16),
            pltpu.VMEM((D,), bf16),
            pltpu.VMEM((D, H * DH), bf16),
            pltpu.VMEM((H * DH, D), bf16),
            pltpu.VMEM((D, FF), bf16),
            pltpu.VMEM((D, FF), bf16),
            pltpu.VMEM((FF, D), bf16),
            pltpu.VMEM((NP, 2, CT, 8, 128), bf16),
            pltpu.VMEM((1, NP, 2, CT, 8, 128), bf16),
            pltpu.VMEM((NT - NQV, D // 2, 128), u32),
            pltpu.VMEM((NT - NVT, 64, D), u32),
            pltpu.VMEM((2 * NMH, D // 2, 128), u32),
            pltpu.VMEM((FF // 128, 64, D), u32),
            pltpu.VMEM((NT, CT, 64, 128), u32),
            pltpu.VMEM((NF, CT * 8, 128), f32),
            pltpu.VMEM((1, NVT * 128, D), f32),
            pltpu.VMEM((1, 2 * NVH * 128 + 8, D), f32),
            pltpu.VMEM((NQV * 128, D), f32),
            pltpu.VMEM((8, -(-(QV0 + NQV) // 4) * 512), f32),
            pltpu.VMEM((8, FF), f32),
            pltpu.VMEM((8, FF), f32),
            pltpu.VMEM((8, D), f32),
            pltpu.VMEM((H, 8, 128), f32),
            pltpu.SMEM((1,), jnp.int32),
            pltpu.SemaphoreType.DMA((NW + B * SEMS_PER_ROW,)),
        ],
        compiler_params=pltpu.CompilerParams(vmem_limit_bytes=120 * 1024 * 1024,
                                             disable_semaphore_checks=True),
        name="fused_decode",
    )(A_x.reshape(B, D), B_w_r, _tile_view(A_k_cache), _tile_view(A_v_cache),
      A_wq, A_wo, B_w_gate, B_w_up, B_w_down)
    return out.reshape(B, 1, D)
```

```python
import contextlib
import functools

import jax
import jax.numpy as jnp
from jax import lax
import jax.experimental.pallas as pl
import jax.experimental.pallas.tpu as pltpu

f32, bf16, u32 = jnp.float32, jnp.bfloat16, jnp.uint32

try:
    _OVR
except NameError:
    _OVR = {}

B, D, H, DH, SK, FF = 4, 640, 32, 192, 4096, 1536
W = min(4096, max(256, SK // 4))
RT = DH // 8
CT = W // 128
NT = H * DH // 128
NP = H * RT // 2
LASTP = _OVR.get("LASTP", 2)
MIDP = _OVR.get("MIDP", 6)
V_CHUNKS = ((0, 192, True), (192, 96, True), (288, 48, True), (336, 24, True), (360, 8, False),
            (368, 16 - MIDP - LASTP, False), (384 - MIDP - LASTP, MIDP, False), (384 - LASTP, LASTP, False))
NW = 7
SEMS_PER_ROW = 2 * (1 + len(V_CHUNKS))
NF = H * RT - _OVR.get("NBF", 2 * LASTP)
QV0 = _OVR.get("QV0", 3)
NQV = _OVR.get("NQV", 9)
NVH = _OVR.get("NVH", 7)
NMH = FF // 128 - NVH
NVD = _OVR.get("NVD", 0)
NVE = _OVR.get("NVE", 3)
DOWN_VPU = tuple(range(NVD)) + tuple(range(FF // 128 - NVE, FF // 128))
SCALE = DH ** -0.5
LOG2E = 1.4426950408889634
EPS = 1e-5

_VT = _OVR.get("VT", "vvmv" * 9 + "vv" + "m" * 7)
VPU_TILES = tuple(t for t in range(NT) if t >= NT - 3 or _VT[t % len(_VT)] == "v")
MXU_TILES = tuple(t for t in range(NT) if t not in VPU_TILES)
NVT = len(VPU_TILES)


def _scope(name):
    return jax.named_scope(name) if _OVR.get("SCOPES") else contextlib.nullcontext()


def _sum(xs):
    return functools.reduce(lambda a, c: a + c, xs)


def _sigmoid(x):
    return 0.5 * jnp.tanh(0.5 * x) + 0.5


def _ln_stats(x):
    m = jnp.sum(x, axis=1, keepdims=True) * (1.0 / D)
    if _OVR.get("ONEPASS", True):
        v = jnp.maximum(jnp.sum(x * x, axis=1, keepdims=True) * (1.0 / D) - m * m, 0.0)
        return m, x - m, lax.rsqrt(v + EPS)
    xc = x - m
    v = jnp.sum(xc * xc, axis=1, keepdims=True) * (1.0 / D)
    return m, xc, lax.rsqrt(v + EPS)


def _kernel(x_hbm, wr_hbm, k_hbm, v_hbm, wq_hbm, wo_hbm, wg_hbm, wu_hbm, wd_hbm,
            out_ref,
            x_v, wr_v, wq_v, wo_v, wg_v, wu_v, wd_v, k_v, v_v,
            wqm_v, wom_v, wgum_v, wdm_v, km_v,
            vf_v, wof_v, wgut_v, wqt_v, wdf_v,
            csq_v, csg_v, csu_v, xf_v, p_v, zero_s, sems):
    w_src = (wq_hbm, x_hbm, wr_hbm, wo_hbm, wg_hbm, wu_hbm, wd_hbm)
    w_dst = (wq_v, x_v, wr_v, wo_v, wg_v, wu_v, wd_v)
    w_cp = [pltpu.make_async_copy(s, d, sems.at[i]) for i, (s, d) in enumerate(zip(w_src, w_dst))]
    win = pl.ds((SK - W) // 128, CT)

    def k_copies(b):
        s0 = NW + b * SEMS_PER_ROW
        return [pltpu.make_async_copy(k_hbm.at[b, :, t, win], k_v.at[:, t], sems.at[s0 + t])
                for t in range(2)]

    def v_copies(b, c):
        p0, n, split = V_CHUNKS[c]
        rows = pl.ds(p0, n)
        s0 = NW + b * SEMS_PER_ROW + 2 * (1 + c)
        if split:
            return [pltpu.make_async_copy(v_hbm.at[b, rows, t, win], v_v.at[0, rows, t],
                                          sems.at[s0 + t]) for t in range(2)]
        return [pltpu.make_async_copy(v_hbm.at[b, rows, :, win], v_v.at[0, rows], sems.at[s0])]

    def start_k(b):
        for cp in k_copies(b):
            cp.start()

    def start_v(b):
        for c in range(len(V_CHUNKS)):
            for cp in v_copies(b, c):
                cp.start()

    for cp in w_cp:
        cp.start()
    start_k(0)
    start_v(0)

    lane = lax.broadcasted_iota(jnp.int32, (8, 128), 1)
    row = lax.broadcasted_iota(jnp.int32, (8, 128), 0)

    def pack(w):
        return pltpu.bitcast(w, u32)

    def unpack(w):
        return pltpu.bitcast(w, bf16)

    def blk(i, n):
        if isinstance(i, int):
            return pl.ds(i * n, n)
        return pl.ds(pl.multiple_of(i * n, n), n)

    def merge_tree(vals, idx):
        bit = 0
        while len(vals) > 1:
            odd = ((idx >> bit) & 1) == 1
            vals = [jnp.where(odd, vals[2 * i + 1], vals[2 * i]) for i in range(len(vals) // 2)]
            bit += 1
        return vals[0]

    def q_lhs(q, middle):
        if middle:
            q = jnp.concatenate([jnp.where(lane < 64, q, 0.0), jnp.where(lane >= 64, q, 0.0)], axis=0)
        return q.astype(bf16)

    def scores_first(k_tile, j, q0, q1):
        ra, rb = [], []
        for c in range(CT):
            r1 = jnp.dot(q1, k_tile(3 * j + 1, c), preferred_element_type=f32)
            r0 = jnp.dot(q0, k_tile(3 * j, c), preferred_element_type=f32)
            ra.append(r0 + r1[0:8])
            rb.append(r1[8:16])
        return merge_tree(ra, row), merge_tree(rb, row)

    def scores_second(k_tile, j, q2, mid):
        r = [jnp.dot(q2, k_tile(3 * j + 2, c), preferred_element_type=f32) for c in range(CT)]
        return merge_tree(r, row) + mid

    def softmax(s, sc, defer=False):
        m = jnp.max(jnp.max(s, axis=1, keepdims=True), axis=0, keepdims=True)
        e = jnp.exp2((s - m) * sc)
        l = jnp.sum(jnp.sum(e, axis=1, keepdims=True), axis=0, keepdims=True)
        r = pl.reciprocal(l, approx=True)
        r = r * (2.0 - l * r)
        return (e, r) if defer else e * r

    def p_rows(p):
        return [jnp.broadcast_to(p[c:c + 1, :], (8, 128)) for c in range(CT)]

    def v_bf16(slot, h, rt):
        return v_v[slot, h * (RT // 2) + rt // 2, rt % 2].reshape(CT * 8, 128).astype(f32)

    def pv_lanes(v, pb):
        a = v[0:8] * pb[0]
        for c in range(1, CT):
            a = a + v[c * 8:(c + 1) * 8] * pb[c]
        return a

    def lane_sum(a):
        return jnp.broadcast_to(jnp.sum(a, axis=1, keepdims=True), (8, 128))

    def pv(v, pb):
        return lane_sum(pv_lanes(v, pb))

    def o_lhs(oc):
        o = merge_tree(oc, lane >> 3)
        return jnp.where((lane & 7) == row, o, 0.0).astype(bf16)

    def proj_vpu(oc, w):
        return w * jnp.concatenate([oc] * (D // 128), axis=1)

    def fold_rows(y):
        return jnp.broadcast_to(jnp.sum(y, axis=0, keepdims=True), y.shape)

    def rows8(x, wt_ref, tile, i):
        w = wt_ref[pl.ds(tile * 128 + i * 8, 8), :] * x
        return lane_sum(_sum([w[:, t * 128:(t + 1) * 128] for t in range(D // 128)]))

    def rows_dot(x, wt_ref, tile):
        return merge_tree([rows8(x, wt_ref, tile, i) for i in range(16)], lane >> 3)

    def attn_streaming(x, b, z):
        _, xc, rstd = _ln_stats(x)
        xcb = xc.astype(bf16)
        sc = rstd * (SCALE * LOG2E)
        with _scope("wait_k"):
            for cp in k_copies(b):
                cp.wait()

        def k_tile(tile, c):
            w = pack(k_v[blk(tile, 8), :, c].reshape(128, 128))
            km_v[tile, c, 0:64, :] = w
            return unpack(w)

        def scores(g, carry):
            q = [jnp.dot(xcb, wq_v[:, blk(6 * g + i, 128)], preferred_element_type=f32)
                 for i in range(6)]
            q = [q_lhs(q[i], i % 3 == 1) for i in range(6)]
            for i in range(2):
                j = 2 * g + i
                sa, mid = scores_first(k_tile, j, q[3 * i], q[3 * i + 1])
                sb = scores_second(k_tile, j, q[3 * i + 2], mid)
                p_v[2 * j] = softmax(sa, sc)
                p_v[2 * j + 1] = softmax(sb, sc)
            return carry

        with _scope("scores"):
            lax.fori_loop(0, H // 4, scores, 0)

        @pl.when(b + 1 < B)
        def _():
            start_k(b + 1)

        def proj_mxu(lhs, tile):
            return jnp.dot(lhs, wo_v[blk(tile, 128), :], preferred_element_type=f32)

        def head_pair(j, carry):
            y, prev = carry
            for c, (p0, _, _) in enumerate(V_CHUNKS[:-4]):
                @pl.when(j == p0 // RT)
                def _():
                    for cp in v_copies(b, c):
                        cp.wait()
            jp = jnp.maximum(j - 1, 0)
            y = y + _sum([proj_mxu(prev[i], 3 * jp + i) for i in range(3)])
            oc = []
            for i in range(2):
                h = 2 * j + i
                pb = p_rows(p_v[h])
                for rt in range(RT):
                    v = v_bf16(0, h, rt)
                    vf_v[h * RT + rt, 0:64, :] = v
                    oc.append(pv(v, pb))
            return y, tuple(o_lhs(oc[16 * i:16 * i + 16]) for i in range(3))

        with _scope("pv_loop"):
            y, prev = lax.fori_loop(
                0, H // 2 - 1, head_pair,
                (jnp.zeros((8, D), f32), (jnp.zeros((8, 128), bf16),) * 3))
        def wait_v(c):
            with _scope("wait_v%d" % c):
                for cp in v_copies(b, len(V_CHUNKS) + c):
                    cp.wait()

        def project(acc, n0, idx):
            ys = [None] * 3
            for n, a in enumerate(acc):
                d = proj_vpu(lane_sum(a), wof_v[idx, pl.ds(((NVT - 3) * 16 + n0 + n) * 8, 8), :])
                ys[n % 3] = d if ys[n % 3] is None else ys[n % 3] + d
            return ys

        pbs = [p_rows(p_v[H - 2]), p_rows(p_v[H - 1])]

        def lanes(n0, n1, sl):
            acc = []
            for n in range(n0, n1):
                v = v_bf16(sl, H - 2 + n // RT, n % RT)
                if (H - 2) * RT + n < NF:
                    vf_v[(H - 2) * RT + n, 0:64, :] = v
                acc.append(pv_lanes(v, pbs[n // RT]))
            return acc

        wait_v(-4)
        y = y + _sum([proj_mxu(prev[i], NT - 6 + i) for i in range(3)])
        y = y + _sum(project(lanes(0, 16, 0), 0, 0))
        wait_v(-3)
        n1, n2 = 48 - 2 * (MIDP + LASTP), 48 - 2 * LASTP
        y = y + _sum(project(lanes(16, n1, 0), 16, 0))
        wait_v(-2)
        acc = lanes(n1, n2, 0)
        wait_v(-1)
        ys = project(acc + lanes(n2, 48, z), n1, z)
        return fold_rows((y + ys[1]) + (ys[2] + ys[0]))

    def attn_resident(x, never):
        a_ahead, a0, a_first = _OVR.get("A_AHEAD", 4), _OVR.get("A0", 2), _OVR.get("A_FIRST", 4)
        tie, n_defer = _OVR.get("TIE", 3), _OVR.get("DEFER", 3)
        mean, xc, rstd = _ln_stats(x)
        xb, xcb = x.astype(bf16), xc.astype(bf16)
        sc = rstd * (SCALE * LOG2E)
        q, e, linv = {}, {}, {}
        done = {}

        def q_vpu(xx, k):
            qk = fold_rows(jnp.where((lane & 7) == row, rows_dot(xx, wqt_v, k), 0.0))
            q[QV0 + k] = q_lhs(qk, (QV0 + k) % 3 == 1)
            return qk

        nq2 = _OVR.get("NQ2", 2)
        for k in range(NQV - nq2):
            q_vpu(x, k)
        a_tiles = [t for t in range(NT) if not QV0 <= t < QV0 + NQV]
        n_a = 0

        def k_tile(tile, c):
            return unpack(km_v[tile, c, 0:64, :])

        for h in range(H):
            while n_a < len(a_tiles) and (
                    n_a < a_first or a_tiles[n_a] * 128 < (h + 1 + min(a_ahead, a0 + h)) * DH):
                t = a_tiles[n_a]
                raw = n_a < 3
                qt = jnp.dot(xb if raw else xcb, unpack(wqm_v[n_a]), preferred_element_type=f32)
                q[t] = q_lhs(qt - mean * csq_v[:, blk(t, 128)] if raw else qt, t % 3 == 1)
                n_a += 1
            j = h // 2
            if h % 2 == 0:
                s, mid = scores_first(k_tile, j, q.pop(3 * j), q.pop(3 * j + 1))
            else:
                s = scores_second(k_tile, j, q.pop(3 * j + 2), mid)
            if h == 0 and nq2:
                x2 = jnp.where(jnp.concatenate([never] * (D // 128), axis=1),
                               jnp.concatenate([s] * (D // 128), axis=1), x)
                done[_OVR.get("Q2TIE", 1) - tie] = [q_vpu(x2, k) for k in range(NQV - nq2, NQV)]
            e[h], linv[h] = softmax(s, sc, defer=True)
            if n_defer <= h < H - _OVR.get("DEFER_LAST", 0):
                e[h], linv[h] = e[h] * linv[h], None
        y, oc, merged = None, {}, {}
        for h in range(H):
            if h - tie in done:
                e[h] = jnp.where(never, _sum(done[h - tie]), e[h])
            pb = p_rows(e[h])
            ys = [None, None, None if linv[h] is not None else y]
            for g in range(h * RT, (h + 1) * RT):
                o = pv(vf_v[g, 0:64, :] if g < NF else v_bf16(0, h, g % RT), pb)
                t = g // 16
                if t in VPU_TILES:
                    rows = pl.ds((VPU_TILES.index(t) * 16 + g % 16) * 8, 8)
                    d = proj_vpu(o, wof_v[0, rows, :])
                    ys[g % 3] = d if ys[g % 3] is None else ys[g % 3] + d
                else:
                    oc[g] = o
                    if g % 16 == 15:
                        m = merge_tree([oc.pop(16 * t + i) for i in range(16)], lane >> 3)
                        la, lb = linv[16 * t // RT], linv[h]
                        if la is not None and 16 * t // RT == h:
                            m = m * la
                        elif la is not None or lb is not None:
                            m = m * jnp.where(lane < 64, 1.0 if la is None else la,
                                              1.0 if lb is None else lb)
                        merged[t] = m
                        if _OVR.get("MTIE", 1):
                            done.setdefault(h, []).append(m)
            if ys[0] is not None:
                if linv[h] is None:
                    y = _sum(ys)
                else:
                    y = _sum(ys) * linv[h] if y is None else y + _sum(ys) * linv[h]
                done.setdefault(h, []).extend(y[:, t * 128:(t + 1) * 128] for t in range(D // 128))
        ym = None
        for t, m in merged.items():
            d = jnp.dot(jnp.where((lane & 7) == row, m, 0.0).astype(bf16),
                        unpack(wom_v[MXU_TILES.index(t)]), preferred_element_type=f32)
            ym = d if ym is None else ym + d
        return fold_rows(ym + y)

    def mod_block(x, shift=None):
        mean, xc, rstd = _ln_stats(x)
        xb, xcb = x.astype(bf16), xc.astype(bf16)
        r = (jnp.sum(x * wr, axis=1, keepdims=True) - mean * wr_sum) * rstd
        half = 0.5 * rstd

        def swiglu(g, u):
            t = g * half
            return (t * jnp.tanh(t) + t) * u

        wgut, nh = wgut_v.at[0], FF // 128
        hid, ys = {}, [None] * 3

        def down_vpu(col, t, i):
            d = proj_vpu(col, wdf_v[0, pl.ds(DOWN_VPU.index(t) * 128 + i * 8, 8), :])
            ys[i % 3] = d if ys[i % 3] is None else ys[i % 3] + d

        for t in range(NMH):
            raw = t < _OVR.get("NRAWH", 2)
            lhs = xb if raw else xcb
            g = jnp.dot(lhs, unpack(wgum_v[2 * t]), preferred_element_type=f32)
            u = jnp.dot(lhs, unpack(wgum_v[2 * t + 1]), preferred_element_type=f32)
            if raw:
                g = g - mean * csg_v[:, blk(t, 128)]
                u = u - mean * csu_v[:, blk(t, 128)]
            hid[t] = swiglu(g, u)
        for k in range(NVH - NVE):
            h = swiglu(rows_dot(x, wgut, 2 * k), rows_dot(x, wgut, 2 * k + 1))
            hid[NMH + k] = jnp.where((lane & 7) == row, h, 0.0)
        for t in range(NVD):
            for i in range(16):
                down_vpu(lane_sum(jnp.where(lane == 8 * i + row, hid[t], 0.0)), t, i)
        for k in range(NVH - NVE, NVH):
            for i in range(16):
                down_vpu(swiglu(rows8(x, wgut, 2 * k, i), rows8(x, wgut, 2 * k + 1, i)), NMH + k, i)
        early = _OVR.get("EARLY", 2)
        order = list(range(NMH, NMH + early)) + list(range(NVD, NMH)) + list(range(NMH + early, nh - NVE))
        ya = yb = None
        for t in order:
            d = jnp.dot(hid[t].astype(bf16), unpack(wdm_v[t]), preferred_element_type=f32)
            if t < NMH:
                ya = d if ya is None else d + ya
            else:
                yb = d if yb is None else d + yb
        y = fold_rows(_sum([v for v in [yb] + ys if v is not None]))
        y = y if ya is None else ya + y
        base = x + xc * rstd
        return (base if shift is None else base + shift) + y * (rstd * _sigmoid(r))

    zero_s[0] = 0
    ones = jnp.ones((8, D), bf16)

    def loop(n, body):
        def step(i, carry):
            body(i)
            return carry
        lax.fori_loop(0, n, step, 0)

    def pick(i, table):
        return _sum([jnp.where(i == n, v, 0) for n, v in enumerate(table)])

    def colsum(w_v, cs_v):
        def body(t):
            cs_v[:, blk(t, 512)] = jnp.dot(ones, w_v[:, blk(t, 512)], preferred_element_type=f32)
        loop(cs_v.shape[1] // 512, body)

    def centered_transpose(w_v, cs_v, src, wt_v, dst):
        cols = blk(src, 128)
        mu = cs_v[0:1, cols] * (1.0 / D)
        for t in range(D // 128):
            wt_v[blk(dst, 128), blk(t, 128)] = (w_v[blk(t, 128), cols].astype(f32) - mu).T

    for cp in w_cp[:3]:
        cp.wait()
    xf_v[0:B, :] = x_v[...].astype(f32)
    wr = wr_v[...].astype(f32).reshape(1, D)
    wr_sum = jnp.sum(wr, axis=1, keepdims=True)
    colsum(wq_v, csq_v)
    loop(NQV, lambda k: centered_transpose(wq_v, csq_v, QV0 + k, wqt_v, k))

    def prep_wq(n):
        wqm_v[n] = pack(wq_v[:, blk(jnp.where(n < QV0, n, n + NQV), 128)])

    loop(NT - NQV, prep_wq)
    w_cp[3].wait()

    def prep_wof(n):
        wof_v[0, blk(n, 128), :] = wo_v[blk(pick(n, VPU_TILES), 128), :].astype(f32)

    def prep_wom(n):
        wom_v[n] = pack(wo_v[blk(pick(n, MXU_TILES), 128), :])

    loop(NVT, prep_wof)
    loop(NT - NVT, prep_wom)
    w_cp[4].wait()
    w_cp[5].wait()
    colsum(wg_v, csg_v)
    colsum(wu_v, csu_v)

    def prep_gum(t):
        wgum_v[2 * t] = pack(wg_v[:, blk(t, 128)])
        wgum_v[2 * t + 1] = pack(wu_v[:, blk(t, 128)])

    def prep_gut(k):
        centered_transpose(wg_v, csg_v, NMH + k, wgut_v.at[0], 2 * k)
        centered_transpose(wu_v, csu_v, NMH + k, wgut_v.at[0], 2 * k + 1)

    def prep_wd(t):
        wdm_v[t] = pack(wd_v[blk(t, 128), :])

    loop(NMH, prep_gum)
    loop(NVH, prep_gut)
    w_cp[6].wait()
    loop(FF // 128, prep_wd)

    def prep_wdf(t):
        wdf_v[0, blk(t, 128), :] = wd_v[blk(pick(t, DOWN_VPU), 128), :].astype(f32)

    if DOWN_VPU:
        loop(len(DOWN_VPU), prep_wdf)

    def batch_body(b):
        @pl.when(b >= 1)
        def _():
            start_v(b)

        x = jnp.broadcast_to(xf_v[pl.ds(b, 1), :], (8, D))
        shift = jnp.sum(x, axis=1, keepdims=True) * (1.0 / D)
        x = x - shift
        z = zero_s[0]
        x = x + attn_streaming(x, b, z)
        with _scope("mod1"):
            x = mod_block(x)
        wgut_v[z, pl.ds(2 * NVH * 128, 8), pl.ds(0, 128)] = jnp.zeros((8, 128), f32)
        wdf_v[z, pl.ds(len(DOWN_VPU) * 128, 8), pl.ds(0, 128)] = jnp.zeros((8, 128), f32)
        with _scope("attn2"):
            x = x + attn_resident(x, lane < z)
        with _scope("mod2"):
            x = mod_block(x, shift)
        xf_v[pl.ds(b, 1), :] = x[0:1, :]

    loop(B, batch_body)
    out_ref[...] = xf_v[0:B, :].astype(bf16)


def _tile_view(c):
    c = c.reshape(B, H, SK // 128, 128, RT, 8).transpose(0, 1, 4, 2, 5, 3)
    return c.reshape(B, NP, 2, SK // 128, 8, 128)


@jax.jit
def pallas_interleave_layers__sliding_block_cached__moe_arch_mod__decode_kernel(
    A_x: jax.Array,
    A_k_cache: jax.Array,
    A_v_cache: jax.Array,
    A_wq: jax.Array,
    A_wo: jax.Array,
    B_x: jax.Array,
    B_w_r: jax.Array,
    B_w_gate: jax.Array,
    B_w_up: jax.Array,
    B_w_down: jax.Array,
):
    del B_x
    out = pl.pallas_call(
        _kernel,
        out_shape=jax.ShapeDtypeStruct((B, D), bf16),
        in_specs=[pl.BlockSpec(memory_space=pl.ANY)] * 9,
        out_specs=pl.BlockSpec(memory_space=pltpu.VMEM),
        scratch_shapes=[
            pltpu.VMEM((B, D), bf16),
            pltpu.VMEM((D,), bf16),
            pltpu.VMEM((D, H * DH), bf16),
            pltpu.VMEM((H * DH, D), bf16),
            pltpu.VMEM((D, FF), bf16),
            pltpu.VMEM((D, FF), bf16),
            pltpu.VMEM((FF, D), bf16),
            pltpu.VMEM((NP, 2, CT, 8, 128), bf16),
            pltpu.VMEM((1, NP, 2, CT, 8, 128), bf16),
            pltpu.VMEM((NT - NQV, D // 2, 128), u32),
            pltpu.VMEM((NT - NVT, 64, D), u32),
            pltpu.VMEM((2 * NMH, D // 2, 128), u32),
            pltpu.VMEM((FF // 128, 64, D), u32),
            pltpu.VMEM((NT, CT, 64 + _OVR.get("KPAD", 8), 128), u32),
            pltpu.VMEM((NF, CT * 8 + _OVR.get("VPAD", 8), 128), f32),
            pltpu.VMEM((1, NVT * 128, D), f32),
            pltpu.VMEM((1, 2 * NVH * 128 + 8, D), f32),
            pltpu.VMEM((NQV * 128, D), f32),
            pltpu.VMEM((1, len(DOWN_VPU) * 128 + 8, D), f32),
            pltpu.VMEM((8, -(-(QV0 + NQV) // 4) * 512), f32),
            pltpu.VMEM((8, FF), f32),
            pltpu.VMEM((8, FF), f32),
            pltpu.VMEM((8, D), f32),
            pltpu.VMEM((H, 8, 128), f32),
            pltpu.SMEM((1,), jnp.int32),
            pltpu.SemaphoreType.DMA((NW + B * SEMS_PER_ROW,)),
        ],
        compiler_params=pltpu.CompilerParams(vmem_limit_bytes=120 * 1024 * 1024,
                                             disable_semaphore_checks=True),
        name="fused_decode",
    )(A_x.reshape(B, D), B_w_r, _tile_view(A_k_cache), _tile_view(A_v_cache),
      A_wq, A_wo, B_w_gate, B_w_up, B_w_down)
    return out.reshape(B, 1, D)
```

```python
import functools

import jax
import jax.numpy as jnp
from jax import lax
import jax.experimental.pallas as pl
import jax.experimental.pallas.tpu as pltpu

f32, bf16, u32 = jnp.float32, jnp.bfloat16, jnp.uint32

B, D, H, DH, SK, FF = 4, 640, 32, 192, 4096, 1536
W = min(4096, max(256, SK // 4))
RT = DH // 8
CT = W // 128
NT = H * DH // 128
NP = H * RT // 2
V_CHUNKS = ((0, 192, True), (192, 96, True), (288, 48, True), (336, 24, True),
            (360, 8, False), (368, 8, False), (376, 6, False), (382, 2, False))
NW = 7
SEMS_PER_ROW = 2 * (1 + len(V_CHUNKS))
NF = 2 * V_CHUNKS[-1][0]
SCALE = DH ** -0.5
LOG2E = 1.4426950408889634
EPS = 1e-5

QV0, NQV = 3, 9
NH = FF // 128
NMH, NVH, NVE = 5, 7, 3
_VT = "vvmv" * 9 + "vv" + "m" * 7 + "vvv"
VPU_TILES = tuple(t for t in range(NT) if _VT[t] == "v")
MXU_TILES = tuple(t for t in range(NT) if _VT[t] == "m")
NVT = len(VPU_TILES)


def _sum(xs):
    return functools.reduce(lambda a, c: a + c, xs)


def _sigmoid(x):
    return 0.5 * jnp.tanh(0.5 * x) + 0.5


def _ln_stats(x):
    m = jnp.sum(x, axis=1, keepdims=True) * (1.0 / D)
    v = jnp.maximum(jnp.sum(x * x, axis=1, keepdims=True) * (1.0 / D) - m * m, 0.0)
    return m, x - m, lax.rsqrt(v + EPS)


def _kernel(x_hbm, wr_hbm, k_hbm, v_hbm, wq_hbm, wo_hbm, wg_hbm, wu_hbm, wd_hbm,
            out_ref,
            x_v, wr_v, wq_v, wo_v, wg_v, wu_v, wd_v, k_v, v_v,
            wqm_v, wom_v, wgum_v, wdm_v, km_v,
            vf_v, wof_v, wgut_v, wqt_v, wdf_v,
            csq_v, csg_v, csu_v, xf_v, p_v, zero_s, sems):
    w_src = (wq_hbm, x_hbm, wr_hbm, wo_hbm, wg_hbm, wu_hbm, wd_hbm)
    w_dst = (wq_v, x_v, wr_v, wo_v, wg_v, wu_v, wd_v)
    w_cp = [pltpu.make_async_copy(s, d, sems.at[i]) for i, (s, d) in enumerate(zip(w_src, w_dst))]
    win = pl.ds((SK - W) // 128, CT)

    def k_copies(b):
        s0 = NW + b * SEMS_PER_ROW
        return [pltpu.make_async_copy(k_hbm.at[b, :, t, win], k_v.at[:, t], sems.at[s0 + t])
                for t in range(2)]

    def v_copies(b, c):
        p0, n, split = V_CHUNKS[c]
        rows = pl.ds(p0, n)
        s0 = NW + b * SEMS_PER_ROW + 2 * (1 + c)
        if split:
            return [pltpu.make_async_copy(v_hbm.at[b, rows, t, win], v_v.at[0, rows, t],
                                          sems.at[s0 + t]) for t in range(2)]
        return [pltpu.make_async_copy(v_hbm.at[b, rows, :, win], v_v.at[0, rows], sems.at[s0])]

    def start_k(b):
        for cp in k_copies(b):
            cp.start()

    def start_v(b):
        for c in range(len(V_CHUNKS)):
            for cp in v_copies(b, c):
                cp.start()

    for cp in w_cp:
        cp.start()
    start_k(0)
    start_v(0)

    lane = lax.broadcasted_iota(jnp.int32, (8, 128), 1)
    row = lax.broadcasted_iota(jnp.int32, (8, 128), 0)

    def pack(w):
        return pltpu.bitcast(w, u32)

    def unpack(w):
        return pltpu.bitcast(w, bf16)

    def blk(i, n):
        if isinstance(i, int):
            return pl.ds(i * n, n)
        return pl.ds(pl.multiple_of(i * n, n), n)

    def merge_tree(vals, idx):
        bit = 0
        while len(vals) > 1:
            odd = ((idx >> bit) & 1) == 1
            vals = [jnp.where(odd, vals[2 * i + 1], vals[2 * i]) for i in range(len(vals) // 2)]
            bit += 1
        return vals[0]

    def q_lhs(q, middle):
        if middle:
            q = jnp.concatenate([jnp.where(lane < 64, q, 0.0), jnp.where(lane >= 64, q, 0.0)], axis=0)
        return q.astype(bf16)

    def scores_first(k_tile, j, q0, q1):
        ra, rb = [], []
        for c in range(CT):
            r1 = jnp.dot(q1, k_tile(3 * j + 1, c), preferred_element_type=f32)
            r0 = jnp.dot(q0, k_tile(3 * j, c), preferred_element_type=f32)
            ra.append(r0 + r1[0:8])
            rb.append(r1[8:16])
        return merge_tree(ra, row), merge_tree(rb, row)

    def scores_second(k_tile, j, q2, mid):
        r = [jnp.dot(q2, k_tile(3 * j + 2, c), preferred_element_type=f32) for c in range(CT)]
        return merge_tree(r, row) + mid

    def softmax(s, sc):
        m = jnp.max(jnp.max(s, axis=1, keepdims=True), axis=0, keepdims=True)
        e = jnp.exp2((s - m) * sc)
        l = jnp.sum(jnp.sum(e, axis=1, keepdims=True), axis=0, keepdims=True)
        r = pl.reciprocal(l, approx=True)
        return e, r * (2.0 - l * r)

    def p_rows(p):
        return [jnp.broadcast_to(p[c:c + 1, :], (8, 128)) for c in range(CT)]

    def v_bf16(idx, h, rt):
        return v_v[idx, h * (RT // 2) + rt // 2, rt % 2].reshape(CT * 8, 128).astype(f32)

    def pv_lanes(v, pb):
        a = v[0:8] * pb[0]
        for c in range(1, CT):
            a = a + v[c * 8:(c + 1) * 8] * pb[c]
        return a

    def lane_sum(a):
        return jnp.broadcast_to(jnp.sum(a, axis=1, keepdims=True), (8, 128))

    def pv(v, pb):
        return lane_sum(pv_lanes(v, pb))

    def o_lhs(oc):
        o = merge_tree(oc, lane >> 3)
        return jnp.where((lane & 7) == row, o, 0.0).astype(bf16)

    def proj_vpu(oc, w):
        return w * jnp.concatenate([oc] * (D // 128), axis=1)

    def fold_rows(y):
        return jnp.broadcast_to(jnp.sum(y, axis=0, keepdims=True), y.shape)

    def rows8(x, wt_ref, tile, i):
        w = wt_ref[pl.ds(tile * 128 + i * 8, 8), :] * x
        return lane_sum(_sum([w[:, t * 128:(t + 1) * 128] for t in range(D // 128)]))

    def rows_dot(x, wt_ref, tile):
        return merge_tree([rows8(x, wt_ref, tile, i) for i in range(16)], lane >> 3)

    def attn_streaming(x, b, z):
        _, xc, rstd = _ln_stats(x)
        xcb = xc.astype(bf16)
        sc = rstd * (SCALE * LOG2E)
        for cp in k_copies(b):
            cp.wait()

        def k_tile(tile, c):
            w = pack(k_v[blk(tile, 8), :, c].reshape(128, 128))
            km_v[tile, c] = w
            return unpack(w)

        def scores(g, carry):
            q = [jnp.dot(xcb, wq_v[:, blk(6 * g + i, 128)], preferred_element_type=f32)
                 for i in range(6)]
            q = [q_lhs(q[i], i % 3 == 1) for i in range(6)]
            for i in range(2):
                j = 2 * g + i
                sa, mid = scores_first(k_tile, j, q[3 * i], q[3 * i + 1])
                sb = scores_second(k_tile, j, q[3 * i + 2], mid)
                for h, s in ((2 * j, sa), (2 * j + 1, sb)):
                    e, linv = softmax(s, sc)
                    p_v[h] = e * linv
            return carry

        lax.fori_loop(0, H // 4, scores, 0)

        @pl.when(b + 1 < B)
        def _():
            start_k(b + 1)

        def proj_mxu(lhs, tile):
            return jnp.dot(lhs, wo_v[blk(tile, 128), :], preferred_element_type=f32)

        def head_pair(j, carry):
            y, prev = carry
            for c, (p0, _, _) in enumerate(V_CHUNKS[:-4]):
                @pl.when(j == p0 // RT)
                def _():
                    for cp in v_copies(b, c):
                        cp.wait()
            jp = jnp.maximum(j - 1, 0)
            y = y + _sum([proj_mxu(prev[i], 3 * jp + i) for i in range(3)])
            oc = []
            for i in range(2):
                h = 2 * j + i
                pb = p_rows(p_v[h])
                for rt in range(RT):
                    v = v_bf16(0, h, rt)
                    vf_v[h * RT + rt] = v
                    oc.append(pv(v, pb))
            return y, tuple(o_lhs(oc[16 * i:16 * i + 16]) for i in range(3))

        y, prev = lax.fori_loop(
            0, H // 2 - 1, head_pair,
            (jnp.zeros((8, D), f32), (jnp.zeros((8, 128), bf16),) * 3))

        def wait_v(c):
            for cp in v_copies(b, len(V_CHUNKS) + c):
                cp.wait()

        def project(acc, n0, idx):
            ys = [None] * 3
            for n, a in enumerate(acc):
                d = proj_vpu(lane_sum(a), wof_v[idx, pl.ds(((NVT - 3) * 16 + n0 + n) * 8, 8), :])
                ys[n % 3] = d if ys[n % 3] is None else ys[n % 3] + d
            return ys

        pbs = [p_rows(p_v[H - 2]), p_rows(p_v[H - 1])]

        def lanes(n0, n1, idx):
            acc = []
            for n in range(n0, n1):
                v = v_bf16(idx, H - 2 + n // RT, n % RT)
                if (H - 2) * RT + n < NF:
                    vf_v[(H - 2) * RT + n] = v
                acc.append(pv_lanes(v, pbs[n // RT]))
            return acc

        wait_v(-4)
        y = y + _sum([proj_mxu(prev[i], NT - 6 + i) for i in range(3)])
        y = y + _sum(project(lanes(0, 16, 0), 0, 0))
        wait_v(-3)
        y = y + _sum(project(lanes(16, 32, 0), 16, 0))
        wait_v(-2)
        acc = lanes(32, 44, 0)
        wait_v(-1)
        ys = project(acc + lanes(44, 48, z), 32, z)
        return fold_rows((y + ys[1]) + (ys[2] + ys[0]))

    def attn_resident(x, never):
        tie, n_defer, nq2 = 3, 3, 2
        mean, xc, rstd = _ln_stats(x)
        xb, xcb = x.astype(bf16), xc.astype(bf16)
        sc = rstd * (SCALE * LOG2E)
        q, e, linv, done = {}, {}, {}, {}

        def q_vpu(xx, k):
            qk = fold_rows(jnp.where((lane & 7) == row, rows_dot(xx, wqt_v, k), 0.0))
            q[QV0 + k] = q_lhs(qk, (QV0 + k) % 3 == 1)
            return qk

        for k in range(NQV - nq2):
            q_vpu(x, k)
        a_tiles = [t for t in range(NT) if not QV0 <= t < QV0 + NQV]
        n_a = 0

        def k_tile(tile, c):
            return unpack(km_v[tile, c])

        for h in range(H):
            while n_a < len(a_tiles) and (
                    n_a < 4 or a_tiles[n_a] * 128 < (h + 1 + min(4, 2 + h)) * DH):
                t = a_tiles[n_a]
                raw = n_a < 3
                qt = jnp.dot(xb if raw else xcb, unpack(wqm_v[n_a]), preferred_element_type=f32)
                q[t] = q_lhs(qt - mean * csq_v[:, blk(t, 128)] if raw else qt, t % 3 == 1)
                n_a += 1
            j = h // 2
            if h % 2 == 0:
                s, mid = scores_first(k_tile, j, q.pop(3 * j), q.pop(3 * j + 1))
            else:
                s = scores_second(k_tile, j, q.pop(3 * j + 2), mid)
            if h == 0:
                x2 = jnp.where(jnp.concatenate([never] * (D // 128), axis=1),
                               jnp.concatenate([s] * (D // 128), axis=1), x)
                done[1 - tie] = [q_vpu(x2, k) for k in range(NQV - nq2, NQV)]
            e[h], linv[h] = softmax(s, sc)
            if h >= n_defer:
                e[h], linv[h] = e[h] * linv[h], None
        y, oc, merged = None, {}, {}
        for h in range(H):
            if h - tie in done:
                e[h] = jnp.where(never, _sum(done[h - tie]), e[h])
            pb = p_rows(e[h])
            ys = [None, None, None if linv[h] is not None else y]
            for g in range(h * RT, (h + 1) * RT):
                o = pv(vf_v[g] if g < NF else v_bf16(0, h, g % RT), pb)
                t = g // 16
                if t in VPU_TILES:
                    rows = pl.ds((VPU_TILES.index(t) * 16 + g % 16) * 8, 8)
                    d = proj_vpu(o, wof_v[0, rows, :])
                    ys[g % 3] = d if ys[g % 3] is None else ys[g % 3] + d
                else:
                    oc[g] = o
                    if g % 16 == 15:
                        m = merge_tree([oc.pop(16 * t + i) for i in range(16)], lane >> 3)
                        la, lb = linv[16 * t // RT], linv[h]
                        if la is not None and 16 * t // RT == h:
                            m = m * la
                        elif la is not None or lb is not None:
                            m = m * jnp.where(lane < 64, 1.0 if la is None else la,
                                              1.0 if lb is None else lb)
                        merged[t] = m
                        done.setdefault(h, []).append(m)
            if ys[0] is not None:
                if linv[h] is None:
                    y = _sum(ys)
                else:
                    y = _sum(ys) * linv[h] if y is None else y + _sum(ys) * linv[h]
                done.setdefault(h, []).extend(y[:, t * 128:(t + 1) * 128] for t in range(D // 128))
        ym = None
        for t, m in merged.items():
            d = jnp.dot(jnp.where((lane & 7) == row, m, 0.0).astype(bf16),
                        unpack(wom_v[MXU_TILES.index(t)]), preferred_element_type=f32)
            ym = d if ym is None else ym + d
        return fold_rows(ym + y)

    def mod_block(x, shift=None):
        mean, xc, rstd = _ln_stats(x)
        xb, xcb = x.astype(bf16), xc.astype(bf16)
        r = (jnp.sum(x * wr, axis=1, keepdims=True) - mean * wr_sum) * rstd
        half = 0.5 * rstd

        def swiglu(g, u):
            t = g * half
            return (t * jnp.tanh(t) + t) * u

        wgut = wgut_v.at[0]
        hid, ys = {}, [None] * 3
        for t in range(NMH):
            raw = t < 2
            lhs = xb if raw else xcb
            g = jnp.dot(lhs, unpack(wgum_v[2 * t]), preferred_element_type=f32)
            u = jnp.dot(lhs, unpack(wgum_v[2 * t + 1]), preferred_element_type=f32)
            if raw:
                g = g - mean * csg_v[:, blk(t, 128)]
                u = u - mean * csu_v[:, blk(t, 128)]
            hid[t] = swiglu(g, u)
        for k in range(NVH - NVE):
            h = swiglu(rows_dot(x, wgut, 2 * k), rows_dot(x, wgut, 2 * k + 1))
            hid[NMH + k] = jnp.where((lane & 7) == row, h, 0.0)
        for k in range(NVH - NVE, NVH):
            for i in range(16):
                h = swiglu(rows8(x, wgut, 2 * k, i), rows8(x, wgut, 2 * k + 1, i))
                d = proj_vpu(h, wdf_v[0, pl.ds((k - NVH + NVE) * 128 + i * 8, 8), :])
                ys[i % 3] = d if ys[i % 3] is None else ys[i % 3] + d
        ya = yb = None
        for t in [NMH, NMH + 1] + list(range(NMH)) + list(range(NMH + 2, NH - NVE)):
            d = jnp.dot(hid[t].astype(bf16), unpack(wdm_v[t]), preferred_element_type=f32)
            if t < NMH:
                ya = d if ya is None else d + ya
            else:
                yb = d if yb is None else d + yb
        y = ya + fold_rows(_sum([yb] + ys))
        base = x + xc * rstd
        return (base if shift is None else base + shift) + y * (rstd * _sigmoid(r))

    zero_s[0] = 0
    ones = jnp.ones((8, D), bf16)

    def loop(n, body):
        def step(i, carry):
            body(i)
            return carry
        lax.fori_loop(0, n, step, 0)

    def pick(i, table):
        return _sum([jnp.where(i == n, v, 0) for n, v in enumerate(table)])

    def colsum(w_v, cs_v):
        def body(t):
            cs_v[:, blk(t, 512)] = jnp.dot(ones, w_v[:, blk(t, 512)], preferred_element_type=f32)
        loop(cs_v.shape[1] // 512, body)

    def centered_transpose(w_v, cs_v, src, wt_v, dst):
        cols = blk(src, 128)
        mu = cs_v[0:1, cols] * (1.0 / D)
        for t in range(D // 128):
            wt_v[blk(dst, 128), blk(t, 128)] = (w_v[blk(t, 128), cols].astype(f32) - mu).T

    for cp in w_cp[:3]:
        cp.wait()
    xf_v[...] = x_v[...].astype(f32)
    wr = wr_v[...].astype(f32).reshape(1, D)
    wr_sum = jnp.sum(wr, axis=1, keepdims=True)
    colsum(wq_v, csq_v)
    loop(NQV, lambda k: centered_transpose(wq_v, csq_v, QV0 + k, wqt_v, k))

    def prep_wq(n):
        wqm_v[n] = pack(wq_v[:, blk(jnp.where(n < QV0, n, n + NQV), 128)])

    loop(NT - NQV, prep_wq)
    w_cp[3].wait()

    def prep_wof(n):
        wof_v[0, blk(n, 128), :] = wo_v[blk(pick(n, VPU_TILES), 128), :].astype(f32)

    def prep_wom(n):
        wom_v[n] = pack(wo_v[blk(pick(n, MXU_TILES), 128), :])

    loop(NVT, prep_wof)
    loop(NT - NVT, prep_wom)
    w_cp[4].wait()
    w_cp[5].wait()
    colsum(wg_v, csg_v)
    colsum(wu_v, csu_v)

    def prep_gum(t):
        wgum_v[2 * t] = pack(wg_v[:, blk(t, 128)])
        wgum_v[2 * t + 1] = pack(wu_v[:, blk(t, 128)])

    def prep_gut(k):
        centered_transpose(wg_v, csg_v, NMH + k, wgut_v.at[0], 2 * k)
        centered_transpose(wu_v, csu_v, NMH + k, wgut_v.at[0], 2 * k + 1)

    def prep_wd(t):
        wdm_v[t] = pack(wd_v[blk(t, 128), :])

    def prep_wdf(t):
        wdf_v[0, blk(t, 128), :] = wd_v[blk(NH - NVE + t, 128), :].astype(f32)

    loop(NMH, prep_gum)
    loop(NVH, prep_gut)
    w_cp[6].wait()
    loop(NH - NVE, prep_wd)
    loop(NVE, prep_wdf)

    def batch_body(b):
        @pl.when(b >= 1)
        def _():
            start_v(b)

        x = jnp.broadcast_to(xf_v[pl.ds(b, 1), :], (8, D))
        shift = jnp.sum(x, axis=1, keepdims=True) * (1.0 / D)
        x = x - shift
        z = zero_s[0]
        x = x + attn_streaming(x, b, z)
        x = mod_block(x)
        wgut_v[z, pl.ds(2 * NVH * 128, 8), pl.ds(0, 128)] = jnp.zeros((8, 128), f32)
        wdf_v[z, pl.ds(NVE * 128, 8), pl.ds(0, 128)] = jnp.zeros((8, 128), f32)
        x = x + attn_resident(x, lane < z)
        x = mod_block(x, shift)
        rows = jnp.where(lax.broadcasted_iota(jnp.int32, (B, D), 0) == b, x[0:B], xf_v[...])
        xf_v[...] = rows
        out_ref[...] = rows.astype(bf16)

    loop(B, batch_body)


def _tile_view(c):
    c = c.reshape(B, H, SK // 128, 128, RT, 8).transpose(0, 1, 4, 2, 5, 3)
    return c.reshape(B, NP, 2, SK // 128, 8, 128)


@jax.jit
def pallas_interleave_layers__sliding_block_cached__moe_arch_mod__decode_kernel(
    A_x: jax.Array,
    A_k_cache: jax.Array,
    A_v_cache: jax.Array,
    A_wq: jax.Array,
    A_wo: jax.Array,
    B_x: jax.Array,
    B_w_r: jax.Array,
    B_w_gate: jax.Array,
    B_w_up: jax.Array,
    B_w_down: jax.Array,
):
    del B_x
    out = pl.pallas_call(
        _kernel,
        out_shape=jax.ShapeDtypeStruct((B, D), bf16),
        in_specs=[pl.BlockSpec(memory_space=pl.ANY)] * 9,
        out_specs=pl.BlockSpec(memory_space=pltpu.VMEM),
        scratch_shapes=[
            pltpu.VMEM((B, D), bf16),
            pltpu.VMEM((D,), bf16),
            pltpu.VMEM((D, H * DH), bf16),
            pltpu.VMEM((H * DH, D), bf16),
            pltpu.VMEM((D, FF), bf16),
            pltpu.VMEM((D, FF), bf16),
            pltpu.VMEM((FF, D), bf16),
            pltpu.VMEM((NP, 2, CT, 8, 128), bf16),
            pltpu.VMEM((1, NP, 2, CT, 8, 128), bf16),
            pltpu.VMEM((NT - NQV, D // 2, 128), u32),
            pltpu.VMEM((NT - NVT, 64, D), u32),
            pltpu.VMEM((2 * NMH, D // 2, 128), u32),
            pltpu.VMEM((NH - NVE, 64, D), u32),
            pltpu.VMEM((NT, CT, 64, 128), u32),
            pltpu.VMEM((NF, CT * 8, 128), f32),
            pltpu.VMEM((1, NVT * 128, D), f32),
            pltpu.VMEM((1, 2 * NVH * 128 + 8, D), f32),
            pltpu.VMEM((NQV * 128, D), f32),
            pltpu.VMEM((1, NVE * 128 + 8, D), f32),
            pltpu.VMEM((8, (QV0 + NQV) * 128), f32),
            pltpu.VMEM((8, FF), f32),
            pltpu.VMEM((8, FF), f32),
            pltpu.VMEM((B, D), f32),
            pltpu.VMEM((H, 8, 128), f32),
            pltpu.SMEM((1,), jnp.int32),
            pltpu.SemaphoreType.DMA((NW + B * SEMS_PER_ROW,)),
        ],
        compiler_params=pltpu.CompilerParams(vmem_limit_bytes=120 * 1024 * 1024,
                                             disable_semaphore_checks=True),
        name="fused_decode",
    )(A_x.reshape(B, D), B_w_r, _tile_view(A_k_cache), _tile_view(A_v_cache),
      A_wq, A_wo, B_w_gate, B_w_up, B_w_down)
    return out.reshape(B, 1, D)
```

```python
import functools

import jax
import jax.numpy as jnp
from jax import lax
import jax.experimental.pallas as pl
import jax.experimental.pallas.tpu as pltpu

f32, bf16, u32 = jnp.float32, jnp.bfloat16, jnp.uint32

B, D, H, DH, SK, FF = 4, 640, 32, 192, 4096, 1536
W = min(4096, max(256, SK // 4))
RT = DH // 8
CT = W // 128
NT = H * DH // 128
NP = H * RT // 2
V_CHUNKS = ((0, 192, True), (192, 96, True), (288, 48, True), (336, 24, True),
            (360, 8, False), (368, 8, False), (376, 6, False), (382, 2, False))
NW = 7
SEMS_PER_ROW = 2 * (1 + len(V_CHUNKS))
NF = 2 * V_CHUNKS[-1][0]
SCALE = DH ** -0.5
LOG2E = 1.4426950408889634
EPS = 1e-5

QV0, NQV = 3, 9
NH = FF // 128
NMH, NVH, NVE = 5, 7, 3
_VT = "vvmv" * 9 + "vv" + "m" * 7 + "vvv"
VPU_TILES = tuple(t for t in range(NT) if _VT[t] == "v")
MXU_TILES = tuple(t for t in range(NT) if _VT[t] == "m")
NVT = len(VPU_TILES)


def _sum(xs):
    return functools.reduce(lambda a, c: a + c, xs)


def _sigmoid(x):
    return 0.5 * jnp.tanh(0.5 * x) + 0.5


def _ln_stats(x):
    m = jnp.sum(x, axis=1, keepdims=True) * (1.0 / D)
    v = jnp.maximum(jnp.sum(x * x, axis=1, keepdims=True) * (1.0 / D) - m * m, 0.0)
    return m, x - m, lax.rsqrt(v + EPS)


def _kernel(x_hbm, wr_hbm, k_hbm, v_hbm, wq_hbm, wo_hbm, wg_hbm, wu_hbm, wd_hbm,
            out_ref,
            x_v, wr_v, wq_v, wo_v, wg_v, wu_v, wd_v, k_v, v_v,
            wqm_v, wom_v, wgum_v, wdm_v, km_v,
            vf_v, wof_v, wgut_v, wqt_v, wdf_v,
            csq_v, csg_v, csu_v, xf_v, p_v, zero_s, sems):
    w_src = (wq_hbm, x_hbm, wr_hbm, wo_hbm, wg_hbm, wu_hbm, wd_hbm)
    w_dst = (wq_v, x_v, wr_v, wo_v, wg_v, wu_v, wd_v)
    w_cp = [pltpu.make_async_copy(s, d, sems.at[i]) for i, (s, d) in enumerate(zip(w_src, w_dst))]
    win = pl.ds((SK - W) // 128, CT)

    def k_copies(b):
        s0 = NW + b * SEMS_PER_ROW
        return [pltpu.make_async_copy(k_hbm.at[b, :, t, win], k_v.at[:, t], sems.at[s0 + t])
                for t in range(2)]

    def v_copies(b, c):
        p0, n, split = V_CHUNKS[c]
        rows = pl.ds(p0, n)
        s0 = NW + b * SEMS_PER_ROW + 2 * (1 + c)
        if split:
            return [pltpu.make_async_copy(v_hbm.at[b, rows, t, win], v_v.at[0, rows, t],
                                          sems.at[s0 + t]) for t in range(2)]
        return [pltpu.make_async_copy(v_hbm.at[b, rows, :, win], v_v.at[0, rows], sems.at[s0])]

    def start_k(b):
        for cp in k_copies(b):
            cp.start()

    def start_v(b):
        for c in range(len(V_CHUNKS)):
            for cp in v_copies(b, c):
                cp.start()

    for cp in w_cp:
        cp.start()
    start_k(0)
    start_v(0)

    lane = lax.broadcasted_iota(jnp.int32, (8, 128), 1)
    row = lax.broadcasted_iota(jnp.int32, (8, 128), 0)

    def pack(w):
        return pltpu.bitcast(w, u32)

    def unpack(w):
        return pltpu.bitcast(w, bf16)

    def blk(i, n):
        if isinstance(i, int):
            return pl.ds(i * n, n)
        return pl.ds(pl.multiple_of(i * n, n), n)

    def merge_tree(vals, idx):
        bit = 0
        while len(vals) > 1:
            odd = ((idx >> bit) & 1) == 1
            vals = [jnp.where(odd, vals[2 * i + 1], vals[2 * i]) for i in range(len(vals) // 2)]
            bit += 1
        return vals[0]

    def q_lhs(q, middle):
        if middle:
            q = jnp.concatenate([jnp.where(lane < 64, q, 0.0), jnp.where(lane >= 64, q, 0.0)], axis=0)
        return q.astype(bf16)

    def scores_first(k_tile, j, q0, q1):
        ra, rb = [], []
        for c in range(CT):
            r1 = jnp.dot(q1, k_tile(3 * j + 1, c), preferred_element_type=f32)
            r0 = jnp.dot(q0, k_tile(3 * j, c), preferred_element_type=f32)
            ra.append(r0 + r1[0:8])
            rb.append(r1[8:16])
        return merge_tree(ra, row), merge_tree(rb, row)

    def scores_second(k_tile, j, q2, mid):
        r = [jnp.dot(q2, k_tile(3 * j + 2, c), preferred_element_type=f32) for c in range(CT)]
        return merge_tree(r, row) + mid

    def softmax(s, sc):
        m = jnp.max(jnp.max(s, axis=1, keepdims=True), axis=0, keepdims=True)
        e = jnp.exp2((s - m) * sc)
        l = jnp.sum(jnp.sum(e, axis=1, keepdims=True), axis=0, keepdims=True)
        r = pl.reciprocal(l, approx=True)
        return e, r * (2.0 - l * r)

    def p_rows(p):
        return [jnp.broadcast_to(p[c:c + 1, :], (8, 128)) for c in range(CT)]

    def v_bf16(idx, h, rt):
        return v_v[idx, h * (RT // 2) + rt // 2, rt % 2].reshape(CT * 8, 128).astype(f32)

    def pv_lanes(v, pb):
        a = v[0:8] * pb[0]
        for c in range(1, CT):
            a = a + v[c * 8:(c + 1) * 8] * pb[c]
        return a

    def lane_sum(a):
        return jnp.broadcast_to(jnp.sum(a, axis=1, keepdims=True), (8, 128))

    def pv(v, pb):
        return lane_sum(pv_lanes(v, pb))

    def o_lhs(oc):
        o = merge_tree(oc, lane >> 3)
        return jnp.where((lane & 7) == row, o, 0.0).astype(bf16)

    def proj_vpu(oc, w):
        return w * jnp.concatenate([oc] * (D // 128), axis=1)

    def fold_rows(y):
        return jnp.broadcast_to(jnp.sum(y, axis=0, keepdims=True), y.shape)

    def rows8(x, wt_ref, tile, i):
        w = wt_ref[pl.ds(tile * 128 + i * 8, 8), :] * x
        return lane_sum(_sum([w[:, t * 128:(t + 1) * 128] for t in range(D // 128)]))

    def rows_dot(x, wt_ref, tile):
        return merge_tree([rows8(x, wt_ref, tile, i) for i in range(16)], lane >> 3)

    def attn_streaming(x, b, z):
        _, xc, rstd = _ln_stats(x)
        xcb = xc.astype(bf16)
        sc = rstd * (SCALE * LOG2E)
        for cp in k_copies(b):
            cp.wait()

        def k_tile(tile, c):
            w = pack(k_v[blk(tile, 8), :, c].reshape(128, 128))
            km_v[tile, c] = w
            return unpack(w)

        def scores(g, carry):
            q = [jnp.dot(xcb, wq_v[:, blk(6 * g + i, 128)], preferred_element_type=f32)
                 for i in range(6)]
            q = [q_lhs(q[i], i % 3 == 1) for i in range(6)]
            for i in range(2):
                j = 2 * g + i
                sa, mid = scores_first(k_tile, j, q[3 * i], q[3 * i + 1])
                sb = scores_second(k_tile, j, q[3 * i + 2], mid)
                for h, s in ((2 * j, sa), (2 * j + 1, sb)):
                    e, linv = softmax(s, sc)
                    p_v[h] = e * linv
            return carry

        lax.fori_loop(0, H // 4, scores, 0)

        @pl.when(b + 1 < B)
        def _():
            start_k(b + 1)

        def proj_mxu(lhs, tile):
            return jnp.dot(lhs, wo_v[blk(tile, 128), :], preferred_element_type=f32)

        def head_pair(j, carry):
            y, prev = carry
            for c, (p0, _, _) in enumerate(V_CHUNKS[:-4]):
                @pl.when(j == p0 // RT)
                def _():
                    for cp in v_copies(b, c):
                        cp.wait()
            jp = jnp.maximum(j - 1, 0)
            y = y + _sum([proj_mxu(prev[i], 3 * jp + i) for i in range(3)])
            oc = []
            for i in range(2):
                h = 2 * j + i
                pb = p_rows(p_v[h])
                for rt in range(RT):
                    v = v_bf16(0, h, rt)
                    vf_v[h * RT + rt] = v
                    oc.append(pv(v, pb))
            return y, tuple(o_lhs(oc[16 * i:16 * i + 16]) for i in range(3))

        y, prev = lax.fori_loop(
            0, H // 2 - 1, head_pair,
            (jnp.zeros((8, D), f32), (jnp.zeros((8, 128), bf16),) * 3))

        def wait_v(c):
            for cp in v_copies(b, len(V_CHUNKS) + c):
                cp.wait()

        def project(acc, n0, idx):
            ys = [None] * 3
            for n, a in enumerate(acc):
                d = proj_vpu(lane_sum(a), wof_v[idx, pl.ds(((NVT - 3) * 16 + n0 + n) * 8, 8), :])
                ys[n % 3] = d if ys[n % 3] is None else ys[n % 3] + d
            return ys

        pbs = [p_rows(p_v[H - 2]), p_rows(p_v[H - 1])]

        def lanes(n0, n1, idx):
            acc = []
            for n in range(n0, n1):
                v = v_bf16(idx, H - 2 + n // RT, n % RT)
                if (H - 2) * RT + n < NF:
                    vf_v[(H - 2) * RT + n] = v
                acc.append(pv_lanes(v, pbs[n // RT]))
            return acc

        wait_v(-4)
        y = y + _sum([proj_mxu(prev[i], NT - 6 + i) for i in range(3)])
        y = y + _sum(project(lanes(0, 16, 0), 0, 0))
        wait_v(-3)
        y = y + _sum(project(lanes(16, 32, 0), 16, 0))
        wait_v(-2)
        acc = lanes(32, 44, 0)
        wait_v(-1)
        ys = project(acc + lanes(44, 48, z), 32, z)
        return fold_rows((y + ys[1]) + (ys[2] + ys[0]))

    def attn_resident(x, never):
        tie, n_defer, nq2 = 3, 3, 2
        mean, xc, rstd = _ln_stats(x)
        xb, xcb = x.astype(bf16), xc.astype(bf16)
        sc = rstd * (SCALE * LOG2E)
        q, e, linv, done = {}, {}, {}, {}

        def q_vpu(xx, k):
            qk = fold_rows(jnp.where((lane & 7) == row, rows_dot(xx, wqt_v, k), 0.0))
            q[QV0 + k] = q_lhs(qk, (QV0 + k) % 3 == 1)
            return qk

        for k in range(NQV - nq2):
            q_vpu(x, k)
        a_tiles = [t for t in range(NT) if not QV0 <= t < QV0 + NQV]
        n_a = 0

        def k_tile(tile, c):
            return unpack(km_v[tile, c])

        for h in range(H):
            while n_a < len(a_tiles) and (
                    n_a < 4 or a_tiles[n_a] * 128 < (h + 1 + min(4, 2 + h)) * DH):
                t = a_tiles[n_a]
                raw = n_a < 3
                qt = jnp.dot(xb if raw else xcb, unpack(wqm_v[n_a]), preferred_element_type=f32)
                q[t] = q_lhs(qt - mean * csq_v[:, blk(t, 128)] if raw else qt, t % 3 == 1)
                n_a += 1
            j = h // 2
            if h % 2 == 0:
                s, mid = scores_first(k_tile, j, q.pop(3 * j), q.pop(3 * j + 1))
            else:
                s = scores_second(k_tile, j, q.pop(3 * j + 2), mid)
            if h == 0:
                x2 = jnp.where(jnp.concatenate([never] * (D // 128), axis=1),
                               jnp.concatenate([s] * (D // 128), axis=1), x)
                done[1 - tie] = [q_vpu(x2, k) for k in range(NQV - nq2, NQV)]
            e[h], linv[h] = softmax(s, sc)
            if h >= n_defer:
                e[h], linv[h] = e[h] * linv[h], None
        y, oc, merged = None, {}, {}
        for h in range(H):
            if h - tie in done:
                e[h] = jnp.where(never, _sum(done[h - tie]), e[h])
            pb = p_rows(e[h])
            ys = [None, None, None if linv[h] is not None else y]
            for g in range(h * RT, (h + 1) * RT):
                o = pv(vf_v[g] if g < NF else v_bf16(0, h, g % RT), pb)
                t = g // 16
                if t in VPU_TILES:
                    rows = pl.ds((VPU_TILES.index(t) * 16 + g % 16) * 8, 8)
                    d = proj_vpu(o, wof_v[0, rows, :])
                    ys[g % 3] = d if ys[g % 3] is None else ys[g % 3] + d
                else:
                    oc[g] = o
                    if g % 16 == 15:
                        m = merge_tree([oc.pop(16 * t + i) for i in range(16)], lane >> 3)
                        la, lb = linv[16 * t // RT], linv[h]
                        if la is not None and 16 * t // RT == h:
                            m = m * la
                        elif la is not None or lb is not None:
                            m = m * jnp.where(lane < 64, 1.0 if la is None else la,
                                              1.0 if lb is None else lb)
                        merged[t] = m
                        done.setdefault(h, []).append(m)
            if ys[0] is not None:
                if linv[h] is None:
                    y = _sum(ys)
                else:
                    y = _sum(ys) * linv[h] if y is None else y + _sum(ys) * linv[h]
                done.setdefault(h, []).extend(y[:, t * 128:(t + 1) * 128] for t in range(D // 128))
        ym = None
        for t, m in merged.items():
            d = jnp.dot(jnp.where((lane & 7) == row, m, 0.0).astype(bf16),
                        unpack(wom_v[MXU_TILES.index(t)]), preferred_element_type=f32)
            ym = d if ym is None else ym + d
        return fold_rows(ym + y)

    def mod_block(x, shift=None):
        mean, xc, rstd = _ln_stats(x)
        xb, xcb = x.astype(bf16), xc.astype(bf16)
        r = (jnp.sum(x * wr, axis=1, keepdims=True) - mean * wr_sum) * rstd
        half = 0.5 * rstd

        def swiglu(g, u):
            t = g * half
            return (t * jnp.tanh(t) + t) * u

        wgut = wgut_v.at[0]
        hid, ys = {}, [None] * 3
        for t in range(NMH):
            raw = t < 2
            lhs = xb if raw else xcb
            g = jnp.dot(lhs, unpack(wgum_v[2 * t]), preferred_element_type=f32)
            u = jnp.dot(lhs, unpack(wgum_v[2 * t + 1]), preferred_element_type=f32)
            if raw:
                g = g - mean * csg_v[:, blk(t, 128)]
                u = u - mean * csu_v[:, blk(t, 128)]
            hid[t] = swiglu(g, u)
        for k in range(NVH - NVE):
            h = swiglu(rows_dot(x, wgut, 2 * k), rows_dot(x, wgut, 2 * k + 1))
            hid[NMH + k] = jnp.where((lane & 7) == row, h, 0.0)
        for k in range(NVH - NVE, NVH):
            for i in range(16):
                h = swiglu(rows8(x, wgut, 2 * k, i), rows8(x, wgut, 2 * k + 1, i))
                d = proj_vpu(h, wdf_v[0, pl.ds((k - NVH + NVE) * 128 + i * 8, 8), :])
                ys[i % 3] = d if ys[i % 3] is None else ys[i % 3] + d
        ya = yb = None
        for t in [NMH, NMH + 1] + list(range(NMH)) + list(range(NMH + 2, NH - NVE)):
            d = jnp.dot(hid[t].astype(bf16), unpack(wdm_v[t]), preferred_element_type=f32)
            if t < NMH:
                ya = d if ya is None else d + ya
            else:
                yb = d if yb is None else d + yb
        y = ya + fold_rows(_sum([yb] + ys))
        base = x + xc * rstd
        return (base if shift is None else base + shift) + y * (rstd * _sigmoid(r))

    zero_s[0] = 0
    ones = jnp.ones((8, D), bf16)

    def loop(n, body):
        def step(i, carry):
            body(i)
            return carry
        lax.fori_loop(0, n, step, 0)

    def pick(i, table):
        return _sum([jnp.where(i == n, v, 0) for n, v in enumerate(table)])

    def colsum(w_v, cs_v):
        def body(t):
            cs_v[:, blk(t, 512)] = jnp.dot(ones, w_v[:, blk(t, 512)], preferred_element_type=f32)
        loop(cs_v.shape[1] // 512, body)

    def centered_transpose(w_v, cs_v, src, wt_v, dst):
        cols = blk(src, 128)
        mu = cs_v[0:1, cols] * (1.0 / D)
        for t in range(D // 128):
            wt_v[blk(dst, 128), blk(t, 128)] = (w_v[blk(t, 128), cols].astype(f32) - mu).T

    for cp in w_cp[:3]:
        cp.wait()
    xf_v[...] = x_v[...].astype(f32)
    wr = wr_v[...].astype(f32).reshape(1, D)
    wr_sum = jnp.sum(wr, axis=1, keepdims=True)
    colsum(wq_v, csq_v)
    loop(NQV, lambda k: centered_transpose(wq_v, csq_v, QV0 + k, wqt_v, k))

    def prep_wq(n):
        wqm_v[n] = pack(wq_v[:, blk(jnp.where(n < QV0, n, n + NQV), 128)])

    loop(NT - NQV, prep_wq)
    w_cp[3].wait()

    def prep_wof(n):
        wof_v[0, blk(n, 128), :] = wo_v[blk(pick(n, VPU_TILES), 128), :].astype(f32)

    def prep_wom(n):
        wom_v[n] = pack(wo_v[blk(pick(n, MXU_TILES), 128), :])

    loop(NVT, prep_wof)
    loop(NT - NVT, prep_wom)
    w_cp[4].wait()
    w_cp[5].wait()
    colsum(wg_v, csg_v)
    colsum(wu_v, csu_v)

    def prep_gum(t):
        wgum_v[2 * t] = pack(wg_v[:, blk(t, 128)])
        wgum_v[2 * t + 1] = pack(wu_v[:, blk(t, 128)])

    def prep_gut(k):
        centered_transpose(wg_v, csg_v, NMH + k, wgut_v.at[0], 2 * k)
        centered_transpose(wu_v, csu_v, NMH + k, wgut_v.at[0], 2 * k + 1)

    def prep_wd(t):
        wdm_v[t] = pack(wd_v[blk(t, 128), :])

    def prep_wdf(t):
        wdf_v[0, blk(t, 128), :] = wd_v[blk(NH - NVE + t, 128), :].astype(f32)

    loop(NMH, prep_gum)
    loop(NVH, prep_gut)
    w_cp[6].wait()
    loop(NH - NVE, prep_wd)
    loop(NVE, prep_wdf)

    def batch_body(b):
        @pl.when(b >= 1)
        def _():
            start_v(b)

        x = jnp.broadcast_to(xf_v[pl.ds(b, 1), :], (8, D))
        shift = jnp.sum(x, axis=1, keepdims=True) * (1.0 / D)
        x = x - shift
        z = zero_s[0]
        x = x + attn_streaming(x, b, z)
        x = mod_block(x)
        wgut_v[z, pl.ds(2 * NVH * 128, 8), pl.ds(0, 128)] = jnp.zeros((8, 128), f32)
        wdf_v[z, pl.ds(NVE * 128, 8), pl.ds(0, 128)] = jnp.zeros((8, 128), f32)
        x = x + attn_resident(x, lane < z)
        x = mod_block(x, shift)
        rows = jnp.where(lax.broadcasted_iota(jnp.int32, (B, D), 0) == b, x[0:B], xf_v[...])
        xf_v[...] = rows
        out_ref[...] = rows.astype(bf16)

    loop(B, batch_body)


def _tile_view(c):
    c = c.reshape(B, H, SK // 128, 128, RT, 8).transpose(0, 1, 4, 2, 5, 3)
    return c.reshape(B, NP, 2, SK // 128, 8, 128)


def _compiler_params():
    limit = 120 * 1024 * 1024
    try:
        return pltpu.CompilerParams(vmem_limit_bytes=limit, disable_semaphore_checks=True)
    except TypeError:
        return pltpu.CompilerParams(vmem_limit_bytes=limit)


@jax.jit
def pallas_interleave_layers__sliding_block_cached__moe_arch_mod__decode_kernel(
    A_x: jax.Array,
    A_k_cache: jax.Array,
    A_v_cache: jax.Array,
    A_wq: jax.Array,
    A_wo: jax.Array,
    B_x: jax.Array,
    B_w_r: jax.Array,
    B_w_gate: jax.Array,
    B_w_up: jax.Array,
    B_w_down: jax.Array,
):
    del B_x
    out = pl.pallas_call(
        _kernel,
        out_shape=jax.ShapeDtypeStruct((B, D), bf16),
        in_specs=[pl.BlockSpec(memory_space=pl.ANY)] * 9,
        out_specs=pl.BlockSpec(memory_space=pltpu.VMEM),
        scratch_shapes=[
            pltpu.VMEM((B, D), bf16),
            pltpu.VMEM((D,), bf16),
            pltpu.VMEM((D, H * DH), bf16),
            pltpu.VMEM((H * DH, D), bf16),
            pltpu.VMEM((D, FF), bf16),
            pltpu.VMEM((D, FF), bf16),
            pltpu.VMEM((FF, D), bf16),
            pltpu.VMEM((NP, 2, CT, 8, 128), bf16),
            pltpu.VMEM((1, NP, 2, CT, 8, 128), bf16),
            pltpu.VMEM((NT - NQV, D // 2, 128), u32),
            pltpu.VMEM((NT - NVT, 64, D), u32),
            pltpu.VMEM((2 * NMH, D // 2, 128), u32),
            pltpu.VMEM((NH - NVE, 64, D), u32),
            pltpu.VMEM((NT, CT, 64, 128), u32),
            pltpu.VMEM((NF, CT * 8, 128), f32),
            pltpu.VMEM((1, NVT * 128, D), f32),
            pltpu.VMEM((1, 2 * NVH * 128 + 8, D), f32),
            pltpu.VMEM((NQV * 128, D), f32),
            pltpu.VMEM((1, NVE * 128 + 8, D), f32),
            pltpu.VMEM((8, (QV0 + NQV) * 128), f32),
            pltpu.VMEM((8, FF), f32),
            pltpu.VMEM((8, FF), f32),
            pltpu.VMEM((B, D), f32),
            pltpu.VMEM((H, 8, 128), f32),
            pltpu.SMEM((1,), jnp.int32),
            pltpu.SemaphoreType.DMA((NW + B * SEMS_PER_ROW,)),
        ],
        compiler_params=_compiler_params(),
        name="fused_decode",
    )(A_x.reshape(B, D), B_w_r, _tile_view(A_k_cache), _tile_view(A_v_cache),
      A_wq, A_wo, B_w_gate, B_w_up, B_w_down)
    return out.reshape(B, 1, D)
```

```python
import functools

import jax
import jax.numpy as jnp
from jax import lax
import jax.experimental.pallas as pl
import jax.experimental.pallas.tpu as pltpu

f32, bf16, u32 = jnp.float32, jnp.bfloat16, jnp.uint32

B, D, H, DH, SK, FF = 4, 640, 32, 192, 4096, 1536
W = min(4096, max(256, SK // 4))
RT = DH // 8
CT = W // 128
NT = H * DH // 128
NP = H * RT // 2
V_CHUNKS = ((0, 192, True), (192, 96, True), (288, 48, True), (336, 24, True),
            (360, 8, False), (368, 8, False), (376, 6, False), (382, 2, False))
NW = 7
V_SEM0 = [NW + 2 + sum(1 + sp for _, _, sp in V_CHUNKS[:c]) for c in range(len(V_CHUNKS) + 1)]
NF = 2 * V_CHUNKS[-1][0]
SCALE = DH ** -0.5
LOG2E = 1.4426950408889634
EPS = 1e-5

QV0, NQV = 3, 9
NH = FF // 128
NMH, NVH, NVE = 5, 7, 3
_VT = "vvmv" * 9 + "vv" + "m" * 7 + "vvv"
VPU_TILES = tuple(t for t in range(NT) if _VT[t] == "v")
MXU_TILES = tuple(t for t in range(NT) if _VT[t] == "m")
NVT = len(VPU_TILES)


def _sum(xs):
    return functools.reduce(lambda a, c: a + c, xs)


def _sigmoid(x):
    return 0.5 * jnp.tanh(0.5 * x) + 0.5


def _ln_stats(x):
    m = jnp.sum(x, axis=1, keepdims=True) * (1.0 / D)
    v = jnp.maximum(jnp.sum(x * x, axis=1, keepdims=True) * (1.0 / D) - m * m, 0.0)
    return m, x - m, lax.rsqrt(v + EPS)


def _kernel(x_hbm, wr_hbm, k_hbm, v_hbm, wq_hbm, wo_hbm, wg_hbm, wu_hbm, wd_hbm,
            out_ref,
            x_v, wr_v, wq_v, wo_v, wg_v, wu_v, wd_v, k_v, v_v,
            wqm_v, wom_v, wgum_v, wdm_v, km_v,
            vf_v, wof_v, wgut_v, wqt_v, wdf_v,
            csq_v, csg_v, csu_v, xf_v, p_v, zero_s, sems):
    w_src = (wq_hbm, x_hbm, wr_hbm, wo_hbm, wg_hbm, wu_hbm, wd_hbm)
    w_dst = (wq_v, x_v, wr_v, wo_v, wg_v, wu_v, wd_v)
    w_cp = [pltpu.make_async_copy(s, d, sems.at[i]) for i, (s, d) in enumerate(zip(w_src, w_dst))]
    win = pl.ds((SK - W) // 128, CT)

    def k_copies(b):
        return [pltpu.make_async_copy(k_hbm.at[b, :, t, win], k_v.at[:, t], sems.at[NW + t])
                for t in range(2)]

    def v_copies(b, c):
        p0, n, split = V_CHUNKS[c]
        rows, s0 = pl.ds(p0, n), V_SEM0[c]
        if split:
            return [pltpu.make_async_copy(v_hbm.at[b, rows, t, win], v_v.at[0, rows, t],
                                          sems.at[s0 + t]) for t in range(2)]
        return [pltpu.make_async_copy(v_hbm.at[b, rows, :, win], v_v.at[0, rows], sems.at[s0])]

    def start_k(b):
        for cp in k_copies(b):
            cp.start()

    def start_v(b):
        for c in range(len(V_CHUNKS)):
            for cp in v_copies(b, c):
                cp.start()

    for cp in w_cp:
        cp.start()
    start_k(0)
    start_v(0)

    lane = lax.broadcasted_iota(jnp.int32, (8, 128), 1)
    row = lax.broadcasted_iota(jnp.int32, (8, 128), 0)

    def pack(w):
        return pltpu.bitcast(w, u32)

    def unpack(w):
        return pltpu.bitcast(w, bf16)

    def blk(i, n):
        if isinstance(i, int):
            return pl.ds(i * n, n)
        return pl.ds(pl.multiple_of(i * n, n), n)

    def merge_tree(vals, idx):
        bit = 0
        while len(vals) > 1:
            odd = ((idx >> bit) & 1) == 1
            vals = [jnp.where(odd, vals[2 * i + 1], vals[2 * i]) for i in range(len(vals) // 2)]
            bit += 1
        return vals[0]

    def q_lhs(q, middle):
        if middle:
            q = jnp.concatenate([jnp.where(lane < 64, q, 0.0), jnp.where(lane >= 64, q, 0.0)], axis=0)
        return q.astype(bf16)

    def scores_first(k_tile, j, q0, q1):
        ra, rb = [], []
        for c in range(CT):
            r1 = jnp.dot(q1, k_tile(3 * j + 1, c), preferred_element_type=f32)
            r0 = jnp.dot(q0, k_tile(3 * j, c), preferred_element_type=f32)
            ra.append(r0 + r1[0:8])
            rb.append(r1[8:16])
        return merge_tree(ra, row), merge_tree(rb, row)

    def scores_second(k_tile, j, q2, mid):
        r = [jnp.dot(q2, k_tile(3 * j + 2, c), preferred_element_type=f32) for c in range(CT)]
        return merge_tree(r, row) + mid

    def softmax(s, sc):
        m = jnp.max(jnp.max(s, axis=1, keepdims=True), axis=0, keepdims=True)
        e = jnp.exp2((s - m) * sc)
        l = jnp.sum(jnp.sum(e, axis=1, keepdims=True), axis=0, keepdims=True)
        r = pl.reciprocal(l, approx=True)
        return e, r * (2.0 - l * r)

    def p_rows(p):
        return [jnp.broadcast_to(p[c:c + 1, :], (8, 128)) for c in range(CT)]

    def v_bf16(idx, h, rt):
        return v_v[idx, h * (RT // 2) + rt // 2, rt % 2].reshape(CT * 8, 128).astype(f32)

    def pv_lanes(v, pb):
        a = v[0:8] * pb[0]
        for c in range(1, CT):
            a = a + v[c * 8:(c + 1) * 8] * pb[c]
        return a

    def lane_sum(a):
        return jnp.broadcast_to(jnp.sum(a, axis=1, keepdims=True), (8, 128))

    def pv(v, pb):
        return lane_sum(pv_lanes(v, pb))

    def o_lhs(oc):
        o = merge_tree(oc, lane >> 3)
        return jnp.where((lane & 7) == row, o, 0.0).astype(bf16)

    def proj_vpu(oc, w):
        return w * jnp.concatenate([oc] * (D // 128), axis=1)

    def fold_rows(y):
        return jnp.broadcast_to(jnp.sum(y, axis=0, keepdims=True), y.shape)

    def rows8(x, wt_ref, tile, i):
        w = wt_ref[pl.ds(tile * 128 + i * 8, 8), :] * x
        return lane_sum(_sum([w[:, t * 128:(t + 1) * 128] for t in range(D // 128)]))

    def rows_dot(x, wt_ref, tile):
        return merge_tree([rows8(x, wt_ref, tile, i) for i in range(16)], lane >> 3)

    def attn_streaming(x, b, z):
        _, xc, rstd = _ln_stats(x)
        xcb = xc.astype(bf16)
        sc = rstd * (SCALE * LOG2E)
        for cp in k_copies(b):
            cp.wait()

        def k_tile(tile, c):
            w = pack(k_v[blk(tile, 8), :, c].reshape(128, 128))
            km_v[tile, c] = w
            return unpack(w)

        def scores(g, carry):
            q = [jnp.dot(xcb, wq_v[:, blk(6 * g + i, 128)], preferred_element_type=f32)
                 for i in range(6)]
            q = [q_lhs(q[i], i % 3 == 1) for i in range(6)]
            for i in range(2):
                j = 2 * g + i
                sa, mid = scores_first(k_tile, j, q[3 * i], q[3 * i + 1])
                sb = scores_second(k_tile, j, q[3 * i + 2], mid)
                for h, s in ((2 * j, sa), (2 * j + 1, sb)):
                    e, linv = softmax(s, sc)
                    p_v[h] = e * linv
            return carry

        lax.fori_loop(0, H // 4, scores, 0)

        @pl.when(b + 1 < B)
        def _():
            start_k(b + 1)

        def proj_mxu(lhs, tile):
            return jnp.dot(lhs, wo_v[blk(tile, 128), :], preferred_element_type=f32)

        def head_pair(j, carry):
            y, prev = carry
            for c, (p0, _, _) in enumerate(V_CHUNKS[:-4]):
                @pl.when(j == p0 // RT)
                def _():
                    for cp in v_copies(b, c):
                        cp.wait()
            jp = jnp.maximum(j - 1, 0)
            y = y + _sum([proj_mxu(prev[i], 3 * jp + i) for i in range(3)])
            oc = []
            for i in range(2):
                h = 2 * j + i
                pb = p_rows(p_v[h])
                for rt in range(RT):
                    v = v_bf16(0, h, rt)
                    vf_v[h * RT + rt] = v
                    oc.append(pv(v, pb))
            return y, tuple(o_lhs(oc[16 * i:16 * i + 16]) for i in range(3))

        y, prev = lax.fori_loop(
            0, H // 2 - 1, head_pair,
            (jnp.zeros((8, D), f32), (jnp.zeros((8, 128), bf16),) * 3))

        def wait_v(c):
            for cp in v_copies(b, len(V_CHUNKS) + c):
                cp.wait()

        def project(acc, n0, idx):
            ys = [None] * 3
            for n, a in enumerate(acc):
                d = proj_vpu(lane_sum(a), wof_v[idx, pl.ds(((NVT - 3) * 16 + n0 + n) * 8, 8), :])
                ys[n % 3] = d if ys[n % 3] is None else ys[n % 3] + d
            return ys

        pbs = [p_rows(p_v[H - 2]), p_rows(p_v[H - 1])]

        def lanes(n0, n1, idx):
            acc = []
            for n in range(n0, n1):
                v = v_bf16(idx, H - 2 + n // RT, n % RT)
                if (H - 2) * RT + n < NF:
                    vf_v[(H - 2) * RT + n] = v
                acc.append(pv_lanes(v, pbs[n // RT]))
            return acc

        wait_v(-4)
        y = y + _sum([proj_mxu(prev[i], NT - 6 + i) for i in range(3)])
        y = y + _sum(project(lanes(0, 16, 0), 0, 0))
        wait_v(-3)
        y = y + _sum(project(lanes(16, 32, 0), 16, 0))
        wait_v(-2)
        acc = lanes(32, 44, 0)
        wait_v(-1)
        ys = project(acc + lanes(44, 48, z), 32, z)
        return fold_rows((y + ys[1]) + (ys[2] + ys[0]))

    def attn_resident(x, never):
        tie, n_defer, nq2 = 3, 3, 2
        mean, xc, rstd = _ln_stats(x)
        xb, xcb = x.astype(bf16), xc.astype(bf16)
        sc = rstd * (SCALE * LOG2E)
        q, e, linv, done = {}, {}, {}, {}

        def q_vpu(xx, k):
            qk = fold_rows(jnp.where((lane & 7) == row, rows_dot(xx, wqt_v, k), 0.0))
            q[QV0 + k] = q_lhs(qk, (QV0 + k) % 3 == 1)
            return qk

        for k in range(NQV - nq2):
            q_vpu(x, k)
        a_tiles = [t for t in range(NT) if not QV0 <= t < QV0 + NQV]
        n_a = 0

        def k_tile(tile, c):
            return unpack(km_v[tile, c])

        for h in range(H):
            while n_a < len(a_tiles) and (
                    n_a < 4 or a_tiles[n_a] * 128 < (h + 1 + min(4, 2 + h)) * DH):
                t = a_tiles[n_a]
                raw = n_a < 3
                qt = jnp.dot(xb if raw else xcb, unpack(wqm_v[n_a]), preferred_element_type=f32)
                q[t] = q_lhs(qt - mean * csq_v[:, blk(t, 128)] if raw else qt, t % 3 == 1)
                n_a += 1
            j = h // 2
            if h % 2 == 0:
                s, mid = scores_first(k_tile, j, q.pop(3 * j), q.pop(3 * j + 1))
            else:
                s = scores_second(k_tile, j, q.pop(3 * j + 2), mid)
            if h == 0:
                x2 = jnp.where(jnp.concatenate([never] * (D // 128), axis=1),
                               jnp.concatenate([s] * (D // 128), axis=1), x)
                done[1 - tie] = [q_vpu(x2, k) for k in range(NQV - nq2, NQV)]
            e[h], linv[h] = softmax(s, sc)
            if h >= n_defer:
                e[h], linv[h] = e[h] * linv[h], None
        y, oc, merged = None, {}, {}
        for h in range(H):
            if h - tie in done:
                e[h] = jnp.where(never, _sum(done[h - tie]), e[h])
            pb = p_rows(e[h])
            ys = [None, None, None if linv[h] is not None else y]
            for g in range(h * RT, (h + 1) * RT):
                o = pv(vf_v[g] if g < NF else v_bf16(0, h, g % RT), pb)
                t = g // 16
                if t in VPU_TILES:
                    rows = pl.ds((VPU_TILES.index(t) * 16 + g % 16) * 8, 8)
                    d = proj_vpu(o, wof_v[0, rows, :])
                    ys[g % 3] = d if ys[g % 3] is None else ys[g % 3] + d
                else:
                    oc[g] = o
                    if g % 16 == 15:
                        m = merge_tree([oc.pop(16 * t + i) for i in range(16)], lane >> 3)
                        la, lb = linv[16 * t // RT], linv[h]
                        if la is not None and 16 * t // RT == h:
                            m = m * la
                        elif la is not None or lb is not None:
                            m = m * jnp.where(lane < 64, 1.0 if la is None else la,
                                              1.0 if lb is None else lb)
                        merged[t] = m
                        done.setdefault(h, []).append(m)
            if ys[0] is not None:
                if linv[h] is None:
                    y = _sum(ys)
                else:
                    y = _sum(ys) * linv[h] if y is None else y + _sum(ys) * linv[h]
                done.setdefault(h, []).extend(y[:, t * 128:(t + 1) * 128] for t in range(D // 128))
        ym = None
        for t, m in merged.items():
            d = jnp.dot(jnp.where((lane & 7) == row, m, 0.0).astype(bf16),
                        unpack(wom_v[MXU_TILES.index(t)]), preferred_element_type=f32)
            ym = d if ym is None else ym + d
        return fold_rows(ym + y)

    def mod_block(x, shift=None):
        mean, xc, rstd = _ln_stats(x)
        xb, xcb = x.astype(bf16), xc.astype(bf16)
        r = (jnp.sum(x * wr, axis=1, keepdims=True) - mean * wr_sum) * rstd
        half = 0.5 * rstd

        def swiglu(g, u):
            t = g * half
            return (t * jnp.tanh(t) + t) * u

        wgut = wgut_v.at[0]
        hid, ys = {}, [None] * 3
        for t in range(NMH):
            raw = t < 2
            lhs = xb if raw else xcb
            g = jnp.dot(lhs, unpack(wgum_v[2 * t]), preferred_element_type=f32)
            u = jnp.dot(lhs, unpack(wgum_v[2 * t + 1]), preferred_element_type=f32)
            if raw:
                g = g - mean * csg_v[:, blk(t, 128)]
                u = u - mean * csu_v[:, blk(t, 128)]
            hid[t] = swiglu(g, u)
        for k in range(NVH - NVE):
            h = swiglu(rows_dot(x, wgut, 2 * k), rows_dot(x, wgut, 2 * k + 1))
            hid[NMH + k] = jnp.where((lane & 7) == row, h, 0.0)
        for k in range(NVH - NVE, NVH):
            for i in range(16):
                h = swiglu(rows8(x, wgut, 2 * k, i), rows8(x, wgut, 2 * k + 1, i))
                d = proj_vpu(h, wdf_v[0, pl.ds((k - NVH + NVE) * 128 + i * 8, 8), :])
                ys[i % 3] = d if ys[i % 3] is None else ys[i % 3] + d
        ya = yb = None
        for t in [NMH, NMH + 1] + list(range(NMH)) + list(range(NMH + 2, NH - NVE)):
            d = jnp.dot(hid[t].astype(bf16), unpack(wdm_v[t]), preferred_element_type=f32)
            if t < NMH:
                ya = d if ya is None else d + ya
            else:
                yb = d if yb is None else d + yb
        y = ya + fold_rows(_sum([yb] + ys))
        base = x + xc * rstd
        return (base if shift is None else base + shift) + y * (rstd * _sigmoid(r))

    zero_s[0] = 0
    ones = jnp.ones((8, D), bf16)

    def loop(n, body):
        def step(i, carry):
            body(i)
            return carry
        lax.fori_loop(0, n, step, 0)

    def pick(i, table):
        return _sum([jnp.where(i == n, v, 0) for n, v in enumerate(table)])

    def colsum(w_v, cs_v):
        def body(t):
            cs_v[:, blk(t, 512)] = jnp.dot(ones, w_v[:, blk(t, 512)], preferred_element_type=f32)
        loop(cs_v.shape[1] // 512, body)

    def centered_transpose(w_v, cs_v, src, wt_v, dst):
        cols = blk(src, 128)
        mu = cs_v[0:1, cols] * (1.0 / D)
        for t in range(D // 128):
            wt_v[blk(dst, 128), blk(t, 128)] = (w_v[blk(t, 128), cols].astype(f32) - mu).T

    for cp in w_cp[:3]:
        cp.wait()
    xf_v[...] = x_v[...].astype(f32)
    wr = wr_v[...].astype(f32).reshape(1, D)
    wr_sum = jnp.sum(wr, axis=1, keepdims=True)
    colsum(wq_v, csq_v)
    loop(NQV, lambda k: centered_transpose(wq_v, csq_v, QV0 + k, wqt_v, k))

    def prep_wq(n):
        wqm_v[n] = pack(wq_v[:, blk(jnp.where(n < QV0, n, n + NQV), 128)])

    loop(NT - NQV, prep_wq)
    w_cp[3].wait()

    def prep_wof(n):
        wof_v[0, blk(n, 128), :] = wo_v[blk(pick(n, VPU_TILES), 128), :].astype(f32)

    def prep_wom(n):
        wom_v[n] = pack(wo_v[blk(pick(n, MXU_TILES), 128), :])

    loop(NVT, prep_wof)
    loop(NT - NVT, prep_wom)
    w_cp[4].wait()
    w_cp[5].wait()
    colsum(wg_v, csg_v)
    colsum(wu_v, csu_v)

    def prep_gum(t):
        wgum_v[2 * t] = pack(wg_v[:, blk(t, 128)])
        wgum_v[2 * t + 1] = pack(wu_v[:, blk(t, 128)])

    def prep_gut(k):
        centered_transpose(wg_v, csg_v, NMH + k, wgut_v.at[0], 2 * k)
        centered_transpose(wu_v, csu_v, NMH + k, wgut_v.at[0], 2 * k + 1)

    def prep_wd(t):
        wdm_v[t] = pack(wd_v[blk(t, 128), :])

    def prep_wdf(t):
        wdf_v[0, blk(t, 128), :] = wd_v[blk(NH - NVE + t, 128), :].astype(f32)

    loop(NMH, prep_gum)
    loop(NVH, prep_gut)
    w_cp[6].wait()
    loop(NH - NVE, prep_wd)
    loop(NVE, prep_wdf)

    def batch_body(b):
        @pl.when(b >= 1)
        def _():
            start_v(b)

        x = jnp.broadcast_to(xf_v[pl.ds(b, 1), :], (8, D))
        shift = jnp.sum(x, axis=1, keepdims=True) * (1.0 / D)
        x = x - shift
        z = zero_s[0]
        x = x + attn_streaming(x, b, z)
        x = mod_block(x)
        wgut_v[z, pl.ds(2 * NVH * 128, 8), pl.ds(0, 128)] = jnp.zeros((8, 128), f32)
        wdf_v[z, pl.ds(NVE * 128, 8), pl.ds(0, 128)] = jnp.zeros((8, 128), f32)
        x = x + attn_resident(x, lane < z)
        x = mod_block(x, shift)
        rows = jnp.where(lax.broadcasted_iota(jnp.int32, (B, D), 0) == b, x[0:B], xf_v[...])
        xf_v[...] = rows
        out_ref[...] = rows.astype(bf16)

    loop(B, batch_body)


def _tile_view(c):
    c = c.reshape(B, H, SK // 128, 128, RT, 8).transpose(0, 1, 4, 2, 5, 3)
    return c.reshape(B, NP, 2, SK // 128, 8, 128)


def _compiler_params():
    limit = 120 * 1024 * 1024
    try:
        return pltpu.CompilerParams(vmem_limit_bytes=limit, disable_semaphore_checks=True)
    except TypeError:
        return pltpu.CompilerParams(vmem_limit_bytes=limit)


@jax.jit
def pallas_interleave_layers__sliding_block_cached__moe_arch_mod__decode_kernel(
    A_x: jax.Array,
    A_k_cache: jax.Array,
    A_v_cache: jax.Array,
    A_wq: jax.Array,
    A_wo: jax.Array,
    B_x: jax.Array,
    B_w_r: jax.Array,
    B_w_gate: jax.Array,
    B_w_up: jax.Array,
    B_w_down: jax.Array,
):
    del B_x
    out = pl.pallas_call(
        _kernel,
        out_shape=jax.ShapeDtypeStruct((B, D), bf16),
        in_specs=[pl.BlockSpec(memory_space=pl.ANY)] * 9,
        out_specs=pl.BlockSpec(memory_space=pltpu.VMEM),
        scratch_shapes=[
            pltpu.VMEM((B, D), bf16),
            pltpu.VMEM((D,), bf16),
            pltpu.VMEM((D, H * DH), bf16),
            pltpu.VMEM((H * DH, D), bf16),
            pltpu.VMEM((D, FF), bf16),
            pltpu.VMEM((D, FF), bf16),
            pltpu.VMEM((FF, D), bf16),
            pltpu.VMEM((NP, 2, CT, 8, 128), bf16),
            pltpu.VMEM((1, NP, 2, CT, 8, 128), bf16),
            pltpu.VMEM((NT - NQV, D // 2, 128), u32),
            pltpu.VMEM((NT - NVT, 64, D), u32),
            pltpu.VMEM((2 * NMH, D // 2, 128), u32),
            pltpu.VMEM((NH - NVE, 64, D), u32),
            pltpu.VMEM((NT, CT, 64, 128), u32),
            pltpu.VMEM((NF, CT * 8, 128), f32),
            pltpu.VMEM((1, NVT * 128, D), f32),
            pltpu.VMEM((1, 2 * NVH * 128 + 8, D), f32),
            pltpu.VMEM((NQV * 128, D), f32),
            pltpu.VMEM((1, NVE * 128 + 8, D), f32),
            pltpu.VMEM((8, (QV0 + NQV) * 128), f32),
            pltpu.VMEM((8, FF), f32),
            pltpu.VMEM((8, FF), f32),
            pltpu.VMEM((B, D), f32),
            pltpu.VMEM((H, 8, 128), f32),
            pltpu.SMEM((1,), jnp.int32),
            pltpu.SemaphoreType.DMA((V_SEM0[-1],)),
        ],
        compiler_params=_compiler_params(),
        name="fused_decode",
    )(A_x.reshape(B, D), B_w_r, _tile_view(A_k_cache), _tile_view(A_v_cache),
      A_wq, A_wo, B_w_gate, B_w_up, B_w_down)
    return out.reshape(B, 1, D)
```
